```python
import jax
import jax.numpy as jnp

def _softmax(x, axis=-1):
    return jax.nn.softmax(x, axis=axis)
def _gelu(x):
    return jax.nn.gelu(x, approximate=True)
def _silu(x):
    return jax.nn.silu(x)
def _sigmoid(x):
    return jax.nn.sigmoid(x)
def _layernorm(x, axis=-1, eps=1e-5):
    m = jnp.mean(x, axis=axis, keepdims=True)
    v = jnp.var(x, axis=axis, keepdims=True)
    return (x - m) / jnp.sqrt(v + eps)
def _scatter_add(tgt, idx, src, axis=0):
    return tgt.at[idx].add(src)
def _segment_sum(src, seg, n):
    return jax.ops.segment_sum(src, seg, n)
class _Rng:
    def __init__(self, key):
        self._k = key
    def _next(self):
        self._k, sub = jax.random.split(self._k)
        return sub
    def normal(self, shape):
        return jax.random.normal(self._next(), shape, dtype=jnp.bfloat16)
    def randint(self, lo, hi, shape):
        return jax.random.randint(self._next(), shape, lo, hi, dtype=jnp.int32)
    def uniform(self, shape, lo=0.0, hi=1.0):
        return jax.random.uniform(self._next(), shape, jnp.bfloat16, lo, hi)
    def permutation(self, n):
        return jax.random.permutation(self._next(), n)


kernel_name = 'recurrent_scan__sliding_local_dilated__moe_arch_mod__prompt'

def setup_inputs():
    _rng = _Rng(jax.random.key(int.from_bytes(__import__("os").urandom(4), "little")))
    _w = (lambda a: (lambda t: t.astype(jnp.bfloat16) if jnp.issubdtype(t.dtype, jnp.floating) else t)(jnp.asarray(a)))
    def _A_setup():
        B, S, D = 1, 2048, 640
        return {
            "x": _w((lambda *s: _rng.normal(s) * 0.05)(B, S, D)),
            "wqkv": _w((lambda *s: _rng.normal(s) * 0.05)(D, 3 * D)),
            "wo": _w((lambda *s: _rng.normal(s) * 0.05)(D, D)),
        }
    _A_in = _A_setup()

    def _B_setup():
        B, S, D, F, C = 1, 2048, 640, 1728, 2
        return {
            "x": _w((lambda *s: _rng.normal(s) * 0.05)(B, S, D)),
            "w_r": _w((lambda *s: _rng.normal(s) * 0.05)(D)),
            "w_gate": _w((lambda *s: _rng.normal(s) * 0.05)(D, F)),
            "w_up": _w((lambda *s: _rng.normal(s) * 0.05)(D, F)),
            "w_down": _w((lambda *s: _rng.normal(s) * 0.05)(F, D)),
        }
    _B_in = _B_setup()

    return {
        "A_x": _A_in["x"],
        "A_wqkv": _A_in["wqkv"],
        "A_wo": _A_in["wo"],
        "B_x": _B_in["x"],
        "B_w_r": _B_in["w_r"],
        "B_w_gate": _B_in["w_gate"],
        "B_w_up": _B_in["w_up"],
        "B_w_down": _B_in["w_down"],
    }

def reference(A_x, A_wqkv, A_wo, B_x, B_w_r, B_w_gate, B_w_up, B_w_down):
    def _A_ref(x, wqkv, wo):
        B, S, D = x.shape
        H = 32; Dh = D // H
        W, dil = 8, 2
        qkv = (lambda x, *d: x.transpose(*d))((x @ wqkv).reshape(B, S, 3, H, Dh), 2, 0, 3, 1, 4)
        q, k, v = qkv[0], qkv[1], qkv[2]
        scale = Dh ** -0.5
        pos = jnp.arange(S)
        off = jnp.arange(W) * dil
        idx = pos[:, None] - off[None, :]
        mask = idx >= 0
        idx_c = jnp.where(mask, idx, 0).reshape(-1)
        kg = k[:, :, idx_c, :].reshape(B, H, S, W, Dh)
        vg = v[:, :, idx_c, :].reshape(B, H, S, W, Dh)
        logits = jnp.einsum("bhsd,bhswd->bhsw", q, kg) * scale
        logits = jnp.where(mask[None, None, :, :], logits, -1e9)
        attn = _softmax(logits, axis=-1)
        o = jnp.einsum("bhsw,bhswd->bhsd", attn, vg)
        return (lambda x, *d: x.transpose(*d))(o, 0, 2, 1, 3).reshape(B, S, D) @ wo

    def _B_ref(x, w_r, w_gate, w_up, w_down):
        B, S, D = x.shape
        C = 2
        r = x @ w_r
        idx = jnp.argsort(-r, axis=-1)[:, :C]
        idx_e = jnp.repeat(idx.reshape(B, C, 1), D, axis=2)
        x_sel = jnp.take_along_axis(x, idx_e, axis=1)
        g = _silu(x_sel @ w_gate)
        u = x_sel @ w_up
        y = (g * u) @ w_down
        r_sel = _sigmoid(jnp.take_along_axis(r, idx, axis=1))
        y = y * r_sel.reshape(B, C, 1)
        b_off = (jnp.arange(B) * S).reshape(B, 1)
        flat_idx = (idx + b_off).reshape(B * C)
        zero = (x * 0.0).reshape(B * S, D)
        upd = _scatter_add(zero, flat_idx, y.reshape(B * C, D), axis=0)
        return x + upd.reshape(B, S, D)

    x = A_x
    xn = _layernorm(x, axis=-1)
    s = _A_ref(xn, A_wqkv, A_wo)
    g = _silu(_B_ref(xn, B_w_r, B_w_gate, B_w_up, B_w_down))
    return x + s * g
```

```python
import math

import jax
import jax.numpy as jnp
import numpy as np
from jax import lax
from jax.experimental import pallas as pl
from jax.experimental.pallas import tpu as pltpu

F32, BF16, U32, I32 = jnp.float32, jnp.bfloat16, jnp.uint32, jnp.int32

S, D, H, DH, F = 2048, 640, 32, 20, 1728
W, DIL = 8, 2
NT = D // 128
HALO = 16
LOG2E = math.log2(math.e)
EPS_BF16 = float(np.asarray(1e-5, dtype=jnp.bfloat16).astype(np.float32))

CFG = dict(flags=None, T=256, RA=8, RL=16, RF=16, tick=True, lag=13, span=1.0)

NT_DIMS = (((1,), (1,)), ((), ()))


def _rb(v):
    return v.astype(BF16).astype(F32)


def _rows(z, r0, n, align=8):
    return pl.ds(r0, n) if z is None else pl.ds(pl.multiple_of(z + r0, align), n)


def _pair_rows(src, c, dst_store):
    for j in range(DH // 2):
        for g in range(2):
            a = src[c, pl.ds(g * 160 + j, 8, stride=DH), :]
            b = src[c, pl.ds(g * 160 + DH // 2 + j, 8, stride=DH), :]
            lo = (a & jnp.uint32(0xFFFF)) | (b << 16)
            hi = (a >> 16) | (b & jnp.uint32(0xFFFF0000))
            dst_store((2 * j) * (H // 2) + 8 * g, lo)
            dst_store((2 * j + 1) * (H // 2) + 8 * g, hi)


def _layernorm(x):
    mean = jnp.sum(x, axis=-1, keepdims=True) * (1.0 / D)
    xc = x - mean
    var = jnp.sum(xc * xc, axis=-1, keepdims=True) * (1.0 / D)
    sd = _rb(jnp.sqrt(_rb(_rb(var) + EPS_BF16)))
    return _rb(x - _rb(mean)) * (1.0 / sd)


def _silu(z):
    h = 0.5 * z
    return h * jnp.tanh(h) + h


def _kernel(x_hbm, wqkv_hbm, wo_hbm, wr_hbm, wg_hbm, wu_hbm, wd_hbm, out_hbm,
            x_v, wqkv_v, wo_v, wg_v, wu_v, wd_v, tmp_v, wp_v, wop_v,
            xn_v, qkv_v, o_v, s_v, out_v, r_v, wr1_v, wr_v, sem_in, sem_out, sem_fix):
    T, RA, RL, RF = CFG["T"], CFG["RA"], CFG["RL"], CFG["RF"]
    NB = S // T

    def x_copy(i, lo, hi):
        return pltpu.make_async_copy(x_hbm.at[pl.ds(lo, hi - lo), :], x_v.at[pl.ds(lo, hi - lo), :], sem_in.at[i])

    def w_copy(m):
        return pltpu.make_async_copy(wqkv_hbm.at[:, pl.ds(m * D, D)], wqkv_v.at[m], sem_in.at[3 + m])

    cx = [x_copy(0, 0, T), x_copy(1, T, 3 * T), x_copy(2, 3 * T, S)]
    cw = [w_copy(m) for m in range(3)]
    cwo = pltpu.make_async_copy(wo_hbm, wo_v, sem_in.at[6])
    cg = pltpu.make_async_copy(wg_hbm, wg_v, sem_in.at[7])
    cu = pltpu.make_async_copy(wu_hbm, wu_v, sem_in.at[8])
    cd = pltpu.make_async_copy(wd_hbm, wd_v, sem_in.at[9])
    cr = pltpu.make_async_copy(wr_hbm, wr1_v, sem_in.at[10])

    def out_copy(b):
        return pltpu.make_async_copy(out_v.at[pl.ds(b * T, T), :], out_hbm.at[pl.ds(b * T, T), :], sem_out.at[b])

    lane = lax.broadcasted_iota(I32, (8, 128), 1)

    def prep_qkv(m):
        for c in range(NT):
            wt = wqkv_v[m, c * 128:(c + 1) * 128, :].T
            tmp_v[m, c] = pltpu.bitcast(wt, U32)
        for c in range(NT):
            def st(row, val, c=c):
                wp_v[m, row:row + 8, c * 128:(c + 1) * 128] = val
            _pair_rows(tmp_v.at[m], c, st)

    def prep_wo():
        for c in range(NT):
            tmp_v[3, c] = pltpu.bitcast(wo_v[:, c * 128:(c + 1) * 128], U32)
        for c in range(NT):
            def st(row, val, c=c):
                wop_v[row:row + 8, c * 128:(c + 1) * 128] = val
            _pair_rows(tmp_v.at[3], c, st)

    held = {}

    def store_packed(key, ref, row, cols, val):
        if val.shape[0] == 8:
            if row % 16 == 0:
                held[key] = val
                return
            val, row = jnp.concatenate([held.pop(key), val], axis=0), row - 8
        ref[row // 2:(row + val.shape[0]) // 2, cols] = pltpu.bitcast(val.astype(BF16), U32)

    def ln_rows(r0, racc, z=None):
        b, o = divmod(r0, T)
        xn = _rb(_layernorm(x_v[_rows(z, r0, RL), :].astype(F32)))
        store_packed("xn", xn_v[b], o, slice(None), xn)
        r = jnp.sum(xn * wr_v[...], axis=-1, keepdims=True)
        for i in range(RL // 8):
            j = r0 // 8 + i
            racc = jnp.where(lane == (j % 128), jnp.broadcast_to(r[8 * i:8 * i + 8], (8, 128)), racc)
            if j % 128 == 127:
                r_v[j // 128] = racc
        return racc, pltpu.bitcast(racc, U32)

    def proj(b, m):
        y = lax.dot_general(pltpu.bitcast(xn_v[b][...], BF16), pltpu.bitcast(wp_v[m], BF16), NT_DIMS,
                            preferred_element_type=F32)
        ys = y * (DH ** -0.5 * LOG2E) if m == 0 else y
        for c in range(NT):
            yc = ys[:, c * 128:(c + 1) * 128]
            qkv_v[b][m * NT + c, HALO:HALO + T, :] = yc
            if m > 0 and b == 0:
                qkv_v[0][m * NT + c, 0:HALO, :] = jnp.broadcast_to(yc[0:1], (HALO, 128))
            if m > 0 and b + 1 < NB:
                qkv_v[b + 1][m * NT + c, 0:HALO, :] = yc[T - HALO:]
        return y

    def attn_rows(r0, z=None):
        b, o = divmod(r0, T)
        win = qkv_v[b].at[:, _rows(z, o, HALO + RA), :]
        q = [win[c, HALO:HALO + RA, :] for c in range(NT)]
        lg = []
        for w in range(W):
            lo = HALO - DIL * w
            p = q[0] * win[NT, lo:lo + RA, :]
            for c in range(1, NT):
                p = p + q[c] * win[NT + c, lo:lo + RA, :]
            p = p + pltpu.roll(p, 64, 1)
            p = p + pltpu.roll(p, 32, 1)
            if r0 < DIL * w:
                row = lax.broadcasted_iota(I32, (RA, 128), 0)
                p = jnp.where(row >= DIL * w - r0, p, -1e9 * LOG2E)
            lg.append(p)
        mx = lg[0]
        for w in range(1, W):
            mx = jnp.maximum(mx, lg[w])
        e = [jnp.exp2(l - mx) for l in lg]
        den = e[0]
        for w in range(1, W):
            den = den + e[w]
        inv = pl.reciprocal(den, full_range=False)
        fin = None
        for c in range(NT):
            acc = e[0] * win[2 * NT + c, HALO:HALO + RA, :]
            for w in range(1, W):
                lo = HALO - DIL * w
                acc = acc + e[w] * win[2 * NT + c, lo:lo + RA, :]
            res = acc * inv
            store_packed(("o", c), o_v, r0, slice(c * 128, (c + 1) * 128), res)
            bits = pltpu.bitcast(res[-8:], U32)
            fin = bits if fin is None else fin | bits
        return fin

    def out_proj(b):
        r0 = b * T
        y = jnp.dot(pltpu.bitcast(o_v[r0 // 2:(r0 + T) // 2, :], BF16), pltpu.bitcast(wop_v[...], BF16),
                    preferred_element_type=F32)
        s_v[r0:r0 + T, :] = y
        return y

    def final_rows(r0, z=None):
        b, o = divmod(r0, T)
        g = _silu(pltpu.bitcast(xn_v[b][_rows(z, o // 2, RF // 2), :], BF16).astype(F32))
        x = x_v[_rows(z, r0, RF, 16), :].astype(F32)
        res = x + s_v[r0:r0 + RF, :] * g
        out_v[r0:r0 + RF, :] = res.astype(BF16)
        bits = pltpu.bitcast(res[-8:], U32)
        fin = bits[:, :128]
        for c in range(1, NT):
            fin = fin | bits[:, c * 128:(c + 1) * 128]
        return fin

    def top2():
        sub = lax.broadcasted_iota(I32, (8, 128), 0)
        imin = jnp.int32(-2 ** 31)
        keys, ids, vals = [], [], []
        for i in range(S // 1024):
            r = _rb(r_v[i]) + 0.0
            bits = pltpu.bitcast(r, I32)
            key = jnp.where(bits < 0, bits ^ jnp.int32(0x7FFFFFFF), bits) >> 16
            keys.append(jnp.where(r != r, jnp.int32(-2 ** 15), key))
            ids.append(i * 1024 + lane * 8 + sub)
            vals.append(r)
        comb = [k * S + (S - 1 - i) for k, i in zip(keys, ids)]
        res = []
        for _ in range(2):
            m = comb[0]
            for cmb in comb[1:]:
                m = jnp.maximum(m, cmb)
            best = jnp.max(m)
            idx = (S - 1) - (best & (S - 1))
            rv = jnp.where(comb[0] == best, vals[0], 0.0)
            for cmb, val in zip(comb[1:], vals[1:]):
                rv = rv + jnp.where(cmb == best, val, 0.0)
            res.append((idx, jnp.sum(rv, keepdims=True)))
            comb = [jnp.where(cmb == best, imin, cmb) for cmb in comb]
        return res

    def group(idx):
        return pl.multiple_of((idx >> 4) << 4, 16)

    def ffn(sel):
        row = lax.broadcasted_iota(I32, (16, D), 0)
        xs = jnp.zeros((16, D), F32)
        rs = jnp.zeros((16, 1), F32)
        normed = []
        for i, (idx, rv) in enumerate(sel):
            blk = _rb(_layernorm(x_v[pl.ds(group(idx), 16), :].astype(F32)))
            normed.append(blk)
            one = jnp.sum(jnp.where(row == (idx & 15), blk, 0.0), axis=0, keepdims=True)
            xs = jnp.where(row == i, one, xs)
            rs = jnp.where(row[:, 0:1] == i, rv, rs)
        xs = xs.astype(BF16)
        g = lax.dot_general(xs, wg_v[...], NT_DIMS, preferred_element_type=F32)
        u = lax.dot_general(xs, wu_v[...], NT_DIMS, preferred_element_type=F32)
        hh = (g * jax.nn.sigmoid(g) * u).astype(BF16)
        y = jnp.dot(hh, wd_v[...], preferred_element_type=F32) * jax.nn.sigmoid(rs)
        gates = []
        for (idx, _), blk in zip(sel, normed):
            upd = jnp.zeros((16, D), F32)
            for i, (other, _) in enumerate(sel):
                upd = jnp.where(row == other - group(idx), y[i:i + 1, :], upd)
            gates.append(_silu(blk + upd))
        return gates

    def patch(sel, gates):
        for (idx, _), g in zip(sel, gates):
            g0 = group(idx)
            out_v[pl.ds(g0, 16), :] = (x_v[pl.ds(g0, 16), :].astype(F32) + s_v[pl.ds(g0, 16), :] * g).astype(BF16)

    def tick(y, u, after):
        bits = after
        if CFG["tick"] and y is not None:
            n = y.shape[0] // 8
            c, g = divmod(int(u * NT * n), n)
            bits = pltpu.bitcast(y[8 * g:8 * g + 8, c * 128:(c + 1) * 128], U32)
            if after is not None:
                bits = bits | after
        if bits is None:
            return None
        return ((bits[0, 0] >> 31) >> 1).astype(I32)

    done = []

    racc = jnp.zeros((8, 128), F32)

    def run(tasks, ys):
        nonlocal racc
        for i, task in enumerate(tasks):
            u = CFG["span"] * i * len(ys) / len(tasks)
            lag = CFG["lag"]
            z = tick(ys[int(u)], u - int(u), done[-lag] if lag and len(done) >= lag else None)
            for kind, r in task:
                if kind == "a":
                    d = attn_rows(r, z)
                elif kind == "l":
                    racc, d = ln_rows(r, racc, z)
                else:
                    d = final_rows(r, z)
            done.append(d)

    cr.start()
    cx[0].start()
    cw[1].start()
    cr.wait()
    wr_v[...] = jnp.broadcast_to(wr1_v[...].astype(F32).reshape(1, D), (RL, D))
    cx[0].wait()
    cw[2].start()
    run([[("l", r)] for r in range(0, T, RL)], [None])
    cw[1].wait()
    cw[0].start()
    prep_qkv(1)
    cw[2].wait()
    cx[1].start()
    proj(0, 1)
    prep_qkv(2)
    cw[0].wait()
    cwo.start()
    cx[2].start()
    proj(0, 2)
    prep_qkv(0)
    cx[1].wait()
    cwo.wait()
    cg.start()
    cu.start()
    cd.start()
    y = proj(0, 0)
    prep_wo()
    run([[("l", r)] for r in range(T, 2 * T, RL)], [y])

    sel = gates = None
    for it in range(NB + 2):
        if it == 1:
            cx[2].wait()
        ys = []
        if it + 1 < NB:
            ys += [proj(it + 1, m) for m in (1, 2, 0)]
        if 1 <= it <= NB:
            ys.append(out_proj(it - 1))
        lists = []
        if it < NB:
            lists.append([("a", r) for r in range(it * T, (it + 1) * T, RA)])
        if it + 2 < NB:
            lists.append([("l", r) for r in range((it + 2) * T, (it + 3) * T, RL)])
        if it >= 2:
            lists.append([("f", r) for r in range((it - 2) * T, (it - 1) * T, RF)])
        tasks = sorted(((i + (k + 0.0) / len(lists)) / len(l), t) for k, l in enumerate(lists) for i, t in enumerate(l))
        run([[t] for _, t in tasks], ys or [None])
        if it == NB - 3:
            cg.wait()
            cu.wait()
            cd.wait()
            sel = top2()
            gates = ffn(sel)
        if 2 <= it <= NB:
            out_copy(it - 2).start()

    for b in range(NB - 1):
        out_copy(b).wait()
    patch(sel, gates)
    out_copy(NB - 1).start()
    g0, g1 = group(sel[0][0]), group(sel[1][0])

    def fix_copy(i, g):
        return pltpu.make_async_copy(out_v.at[pl.ds(g, 16), :], out_hbm.at[pl.ds(g, 16), :], sem_fix.at[i])

    do0 = g0 < S - T
    do1 = jnp.logical_and(g1 < S - T, g1 != g0)

    @pl.when(do0)
    def _():
        fix_copy(0, g0).start()

    @pl.when(do1)
    def _():
        fix_copy(1, g1).start()

    @pl.when(do0)
    def _():
        fix_copy(0, g0).wait()

    @pl.when(do1)
    def _():
        fix_copy(1, g1).wait()

    out_copy(NB - 1).wait()


@jax.jit
def pallas_recurrent_scan__sliding_local_dilated__moe_arch_mod__prompt_kernel(A_x, A_wqkv, A_wo, B_x, B_w_r, B_w_gate, B_w_up, B_w_down):
    del B_x
    T = CFG["T"]
    NB = S // T
    hbm = pl.BlockSpec(memory_space=pltpu.HBM)
    out = pl.pallas_call(
        _kernel,
        out_shape=jax.ShapeDtypeStruct((S, D), BF16),
        in_specs=[hbm] * 7,
        out_specs=hbm,
        scratch_shapes=[
            pltpu.VMEM((S, D), BF16),
            pltpu.VMEM((3, D, D), BF16),
            pltpu.VMEM((D, D), BF16),
            pltpu.VMEM((F, D), BF16),
            pltpu.VMEM((F, D), BF16),
            pltpu.VMEM((F, D), BF16),
            pltpu.VMEM((4, NT, D // 2, 128), U32),
            pltpu.VMEM((3, D // 2, D), U32),
            pltpu.VMEM((D // 2, D), U32),
            [pltpu.VMEM((T // 2, D), U32) for _ in range(NB)],
            [pltpu.VMEM((3 * NT, HALO + T, 128), F32) for _ in range(NB)],
            pltpu.VMEM((S // 2, D), U32),
            pltpu.VMEM((S, D), F32),
            pltpu.VMEM((S, D), BF16),
            pltpu.VMEM((S // 1024, 8, 128), F32),
            pltpu.VMEM((D,), BF16),
            pltpu.VMEM((CFG['RL'], D), F32),
            pltpu.SemaphoreType.DMA((11,)),
            pltpu.SemaphoreType.DMA((NB,)),
            pltpu.SemaphoreType.DMA((2,)),
        ],
        compiler_params=pltpu.CompilerParams(vmem_limit_bytes=100 * 2 ** 20, flags=CFG['flags']),
        name="fused",
    )(A_x.reshape(S, D), A_wqkv, A_wo, B_w_r, B_w_gate.T, B_w_up.T, B_w_down)
    return out.reshape(1, S, D)
```

```python
import functools
import math

import jax
import jax.numpy as jnp
import numpy as np
from jax import lax
from jax.experimental import pallas as pl
from jax.experimental.pallas import tpu as pltpu

F32, BF16, U32, I32 = jnp.float32, jnp.bfloat16, jnp.uint32, jnp.int32

S, D, H, DH, F = 2048, 640, 32, 20, 1728
W, DIL = 8, 2
NT = D // 128
HALO = 16
LOG2E = math.log2(math.e)
EPS_BF16 = float(np.asarray(1e-5, dtype=jnp.bfloat16).astype(np.float32))

CFG = dict(flags=None, B0=256, TS=256, U=1, RA=8, RL=16, lat=100, laga=4, lagl=5, tick=True, aspan=(0.0, 0.62), lspan=(0.62, 0.88), TA=512, T2=448, N2=3,
           marks=False)

NT_DIMS = (((1,), (1,)), ((), ()))


def _rb(v):
    return v.astype(BF16).astype(F32)


def _ds(r0, n, align=8):
    return pl.ds(r0 if isinstance(r0, int) else pl.multiple_of(r0, align), n)


def _half(r0):
    return r0 // 2 if isinstance(r0, int) else r0 >> 1


def _pair_rows(src, c, dst_store):
    for j in range(DH // 2):
        for g in range(2):
            a = src[c, pl.ds(g * 160 + j, 8, stride=DH), :]
            b = src[c, pl.ds(g * 160 + DH // 2 + j, 8, stride=DH), :]
            lo = (a & jnp.uint32(0xFFFF)) | (b << 16)
            hi = (a >> 16) | (b & jnp.uint32(0xFFFF0000))
            dst_store((2 * j) * (H // 2) + 8 * g, lo)
            dst_store((2 * j + 1) * (H // 2) + 8 * g, hi)


def _const(val, gate, rows):
    if gate is None:
        return val
    c = pltpu.bitcast(gate | np.float32(val).view(np.uint32), F32)
    return jnp.concatenate([c] * (rows // 8), axis=0)


def _layernorm(x, gate=None):
    tot = x[:, :128] if gate is None else x[:, :128] + _const(0.0, gate, x.shape[0])
    for c in range(1, NT):
        tot = tot + x[:, c * 128:(c + 1) * 128]
    mean = jnp.sum(tot, axis=-1, keepdims=True) * (1.0 / D)
    xc = x - mean
    var = jnp.sum(xc * xc, axis=-1, keepdims=True) * (1.0 / D)
    sd = _rb(jnp.sqrt(_rb(_rb(var) + EPS_BF16)))
    return _rb(_rb(x - _rb(mean)) * (1.0 / sd))


def _silu(z):
    h = 0.5 * z
    return h * jnp.tanh(h) + h


def _kernel(x_hbm, wqkv_hbm, wo_hbm, wr_hbm, wg_hbm, wu_hbm, wd_hbm, out_hbm,
            x_v, wqkv_v, wo_v, wg_v, wu_v, wd_v, tmp_v, wp_v, wop_v,
            xn_v, qkv_v, o_v, s_v, out_v, r_v, wr1_v, wr_v, xs_v, y_v, sem_in, sem_out, sem_fix):
    B0, TS, U, RA, RL = CFG["B0"], CFG["TS"], CFG["U"], CFG["RA"], CFG["RL"]
    A0 = B0 - TS
    N1 = (S - B0) // TS
    FC = F
    assert N1 * TS == S - B0 and A0 == 0

    def x_copy(i, lo, hi):
        return pltpu.make_async_copy(x_hbm.at[pl.ds(lo, hi - lo), :], x_v.at[pl.ds(lo, hi - lo), :], sem_in.at[i])

    def w_copy(m):
        return pltpu.make_async_copy(wqkv_hbm.at[:, pl.ds(m * D, D)], wqkv_v.at[m], sem_in.at[3 + m])

    cx = [x_copy(0, 0, B0), x_copy(1, B0, B0 + TS), x_copy(2, B0 + TS, S)]
    cw = [w_copy(m) for m in range(3)]
    cwo = pltpu.make_async_copy(wo_hbm, wo_v, sem_in.at[6])
    cg = pltpu.make_async_copy(wg_hbm, wg_v, sem_in.at[7])
    cu = pltpu.make_async_copy(wu_hbm, wu_v, sem_in.at[8])
    cd = pltpu.make_async_copy(wd_hbm, wd_v, sem_in.at[9])
    cr = pltpu.make_async_copy(wr_hbm, wr1_v, sem_in.at[10])

    def out_copy(i, r0, n):
        return pltpu.make_async_copy(out_v.at[_ds(r0, n, 16), :], out_hbm.at[_ds(r0, n, 16), :], sem_out.at[i])

    lane = lax.broadcasted_iota(I32, (8, 128), 1)

    def prep_qkv(m):
        for c in range(NT):
            wt = wqkv_v[m, c * 128:(c + 1) * 128, :].T
            tmp_v[m, c] = pltpu.bitcast(wt, U32)
        for c in range(NT):
            def st(row, val, c=c):
                wp_v[m, row:row + 8, c * 128:(c + 1) * 128] = val
            _pair_rows(tmp_v.at[m], c, st)

    def prep_wo():
        for c in range(NT):
            tmp_v[3, c] = pltpu.bitcast(wo_v[:, c * 128:(c + 1) * 128], U32)
        for c in range(NT):
            def st(row, val, c=c):
                wop_v[row:row + 8, c * 128:(c + 1) * 128] = val
            _pair_rows(tmp_v.at[3], c, st)

    def ln_rows(src, xn_out, dst, racc, gate):
        xn = _layernorm(src.astype(F32), gate)
        xn_out[pl.ds(dst // 2, RL // 2), :] = pltpu.bitcast(xn.astype(BF16), U32)
        r = jnp.sum(xn * wr_v[...], axis=-1, keepdims=True)
        acc, n = racc
        for i in range(RL // 8):
            acc = jnp.where(lane == n + i, jnp.broadcast_to(r[8 * i:8 * i + 8], (8, 128)), acc)
        return (acc, n + RL // 8), pltpu.bitcast(acc, U32)

    def gated(w, gate):
        if gate is None:
            return pltpu.bitcast(w, BF16)
        head = w[:8] | jnp.concatenate([gate] * (w.shape[1] // 128), axis=1)
        return pltpu.bitcast(jnp.concatenate([head, w[8:]], axis=0), BF16)

    def proj(xn, qkv, r0, n, mats=(1, 2, 0)):
        def col(m, c, gate):
            y = lax.dot_general(pltpu.bitcast(xn[r0 // 2:(r0 + n) // 2, :], BF16),
                                gated(wp_v[m, c * 64:(c + 1) * 64, :], gate), NT_DIMS, preferred_element_type=F32)
            qkv[m * NT + c, HALO + r0:HALO + r0 + n, :] = y
            if m > 0 and r0 == 0:
                qkv_v[m * NT + c, 0:HALO, :] = jnp.broadcast_to(y[0:1], (HALO, 128))
            return y
        return [(n, functools.partial(col, m, c)) for m in mats for c in range(NT)]

    held = {}

    def attn_rows(qkv, o, off, first, gate):
        win = qkv.at[:, pl.ds(off, HALO + RA), :]
        scale = _const(DH ** -0.5 * LOG2E, gate, RA)
        q = [win[c, HALO:HALO + RA, :] * scale for c in range(NT)]
        lg = []
        for w in range(W):
            lo = HALO - DIL * w
            p = q[0] * win[NT, lo:lo + RA, :]
            for c in range(1, NT):
                p = p + q[c] * win[NT + c, lo:lo + RA, :]
            p = p + pltpu.roll(p, 64, 1)
            p = p + pltpu.roll(p, 32, 1)
            if first is not None and off < DIL * w:
                row = lax.broadcasted_iota(I32, (RA, 128), 0)
                p = jnp.where(row >= DIL * w - off - first, p, -1e9 * LOG2E)
            lg.append(p)
        mx = lg[0]
        for w in range(1, W):
            mx = jnp.maximum(mx, lg[w])
        e = [jnp.exp2(l - mx) for l in lg]
        den = e[0]
        for w in range(1, W):
            den = den + e[w]
        inv = pl.reciprocal(den, full_range=False)
        fin = None
        for c in range(NT):
            acc = e[0] * win[2 * NT + c, HALO:HALO + RA, :]
            for w in range(1, W):
                lo = HALO - DIL * w
                acc = acc + e[w] * win[2 * NT + c, lo:lo + RA, :]
            res = acc * inv
            bits = pltpu.bitcast(res[-8:], U32)
            fin = bits if fin is None else fin | bits
            row = off
            if RA == 8:
                if off % 16 == 0:
                    held[c] = res
                    continue
                res, row = jnp.concatenate([held.pop(c), res], axis=0), off - 8
            o[pl.ds(row // 2, res.shape[0] // 2), c * 128:(c + 1) * 128] = (
                pltpu.bitcast(res.astype(BF16), U32))
        return fin

    def out_rows(o, xn, nat, r0, n):
        x, s, out = nat

        def col(c, gate):
            cols = slice(c * 128, (c + 1) * 128)
            y = jnp.dot(pltpu.bitcast(o[r0 // 2:(r0 + n) // 2, :], BF16), gated(wop_v[:, cols], gate),
                        preferred_element_type=F32)
            s[r0:r0 + n, cols] = y
            g = _silu(pltpu.bitcast(xn[r0 // 2:(r0 + n) // 2, cols], BF16).astype(F32))
            out[r0:r0 + n, cols] = (x[r0:r0 + n, cols].astype(F32) + y * g).astype(BF16)
            return y
        return [(n, functools.partial(col, c)) for c in range(NT)]

    groups = [(0, B0)] + [(B0 + i * TS, TS) for i in range(N1)]

    def top2():
        sub = lax.broadcasted_iota(I32, (8, 128), 0)
        imin = jnp.int32(-2 ** 31)
        comb, vals = [], []
        for i, (r0, n) in enumerate(groups):
            r = _rb(r_v[i]) + 0.0
            bits = pltpu.bitcast(r, I32)
            key = jnp.where(bits < 0, bits ^ jnp.int32(0x7FFFFFFF), bits) >> 16
            key = jnp.where(r != r, jnp.int32(-2 ** 15), key)
            comb.append(jnp.where(lane < n // 8, key * S + (S - 1 - r0 - lane * 8 - sub), imin))
            vals.append(r)
        res = []
        for _ in range(2):
            m = comb[0]
            for cmb in comb[1:]:
                m = jnp.maximum(m, cmb)
            best = jnp.max(m)
            rv = jnp.where(comb[0] == best, vals[0], 0.0)
            for cmb, val in zip(comb[1:], vals[1:]):
                rv = jnp.where(cmb == best, val, rv)
            res.append(((S - 1) - (best & (S - 1)), jnp.sum(rv, keepdims=True)))
            comb = [jnp.where(cmb == best, imin, cmb) for cmb in comb]
        return res

    def group(idx):
        return pl.multiple_of((idx >> 4) << 4, 16)

    def normed(g0):
        return pltpu.bitcast(xn_v[_ds(g0 >> 1, 8), :], BF16).astype(F32)

    def gather(sel):
        row = lax.broadcasted_iota(I32, (16, D), 0)
        xs = jnp.zeros((16, D), F32)
        for i, (idx, _) in enumerate(sel):
            one = jnp.sum(jnp.where(row == (idx & 15), normed(group(idx)), 0.0), axis=0, keepdims=True)
            xs = jnp.where(row == i, one, xs)
        xs_v[...] = xs.astype(BF16)
        y_v[...] = jnp.zeros((16, D), F32)

    def ffn_chunk(i):
        rows = _ds(i * FC, FC, 16)
        xs = xs_v[...]
        g = lax.dot_general(xs, wg_v[rows, :], NT_DIMS, preferred_element_type=F32)
        u = lax.dot_general(xs, wu_v[rows, :], NT_DIMS, preferred_element_type=F32)
        return (g * jax.nn.sigmoid(g) * u).astype(BF16), rows

    def ffn_down(hh, rows):
        y_v[...] += jnp.dot(hh, wd_v[rows, :], preferred_element_type=F32)

    def routed_gates(sel):
        row = lax.broadcasted_iota(I32, (16, D), 0)
        ys = [y_v[i:i + 1, :] * jax.nn.sigmoid(rv) for i, (_, rv) in enumerate(sel)]
        gates = []
        for idx, _ in sel:
            upd = jnp.zeros((16, D), F32)
            for (other, _), y in zip(sel, ys):
                upd = jnp.where(row == other - group(idx), y, upd)
            gates.append(_silu(normed(group(idx)) + upd))
        return gates

    def run(dots, attn=(), ln=(), aspan=(0.0, 1.0), lspan=(0.0, 1.0)):
        n = dots[0][0] if dots else 0
        ready = [(5 * j + 4) // 4 * n + CFG["lat"] for j in range(len(dots))]
        total = 5 * len(dots) * n // 4
        tasks = []
        for k, (_, _, _, rows, _) in enumerate(attn):
            cnt = rows // RA
            tasks += [(aspan[0] + (aspan[1] - aspan[0]) * (k + i / cnt) / len(attn), "a", k, i * RA)
                      for i in range(cnt)]
        for k, (_, _, _, rows, _) in enumerate(ln):
            cnt = rows // RL
            tasks += [(lspan[0] + (lspan[1] - lspan[0]) * (k + i / cnt) / len(ln), "l", k, i * RL)
                      for i in range(cnt)]
        tasks.sort()
        racc = [(jnp.zeros((8, 128), F32), 0) for _ in ln]
        done = {"a": [], "l": []}
        pos = 0
        y = None
        for j in range(-1, len(dots)):
            if j >= 0:
                y = dots[j][1](None)
            while pos < len(tasks):
                u, kind, k, off = tasks[pos]
                t = int(u * total)
                if j + 1 < len(dots) and t >= ready[j + 1]:
                    break
                pos += 1
                lag = CFG["lag" + kind]
                bits = done[kind][-lag] if len(done[kind]) >= lag else None
                if j >= 0 and CFG["tick"]:
                    g = min(t - ready[j], n - 8) // 8
                    mine = pltpu.bitcast(y[8 * g:8 * g + 8], U32)
                    bits = mine if bits is None else bits | mine
                gate = None if bits is None else (bits >> 31) >> 1
                if kind == "a":
                    d = attn_rows(attn[k][0], attn[k][1], attn[k][2] + off, attn[k][4], gate)
                else:
                    racc[k], d = ln_rows(ln[k][0][off:off + RL, :], ln[k][1], ln[k][2] + off, racc[k], gate)
                done[kind].append(d)
        for k, l in enumerate(ln):
            r_v[l[4]] = racc[k][0]

    scope = [None]

    def mark(name):
        if not CFG.get("marks"):
            return
        if scope[0] is not None:
            scope[0].__exit__(None, None, None)
            scope[0] = None
        if name:
            scope[0] = jax.named_scope(name)
            scope[0].__enter__()

    mark("m00_start")
    cr.start()
    cx[0].start()
    cw[1].start()
    cr.wait()
    cx[0].wait()
    mark("m01_ln0")
    cw[2].start()
    wr_v[...] = jnp.broadcast_to(wr1_v[...].astype(F32).reshape(1, D), (RL, D))
    run([], ln=[(x_v, xn_v, 0, B0, 0)])
    mark("m02_waitwk")
    cw[1].wait()
    mark("m03_prepk")
    cw[0].start()
    prep_qkv(1)
    mark("m04_waitwv")
    cw[2].wait()
    mark("m05_projk")
    cx[1].start()
    run(proj(xn_v, qkv_v, 0, B0, (1,)))
    prep_qkv(2)
    mark("m06_waitwq")
    cw[0].wait()
    mark("m07_projv")
    cwo.start()
    cx[2].start()
    run(proj(xn_v, qkv_v, 0, B0, (2,)))
    prep_qkv(0)
    mark("m08_waitx1")
    cx[1].wait()
    mark("m09_projq")
    run(proj(xn_v, qkv_v, 0, B0, (0,)), ln=[(x_v.at[B0:B0 + TS, :], xn_v, B0, TS, 1)], lspan=(0.0, 0.6))
    mark("m10_waitx2")
    cwo.wait()
    cx[2].wait()
    mark("m11_loop")
    cg.start()
    cu.start()
    cd.start()
    prep_wo()

    def main(i, carry):
        base = i * TS
        qkv = qkv_v.at[:, _ds(base, HALO + 2 * TS), :]
        xn = xn_v.at[_ds(i * (TS // 2), 3 * TS // 2), :]
        o = o_v.at[_ds(i * (TS // 2), TS // 2), :]
        nat = [ref.at[_ds(base, TS, 16), :] for ref in (x_v, s_v, out_v)]
        run(proj(xn, qkv, TS, TS) + out_rows(o, xn, nat, 0, TS), [(qkv, o, 0, TS, base)],
            [(x_v.at[_ds(jnp.minimum(base + 2 * TS, S - TS), TS, 16), :], xn, 2 * TS, TS, i + 2)], CFG["aspan"], CFG["lspan"])
        out_copy(i, base, TS).start()
        return carry

    def main_marked(i, c):
        with jax.named_scope("m11_body"):
            return main(i, c)

    lax.fori_loop(0, N1, main_marked if CFG["marks"] else main, 0)

    mark("m12_ffn")
    cg.wait()
    cu.wait()
    cd.wait()
    sel = top2()
    gather(sel)
    ffn_down(*ffn_chunk(0))
    run([], attn=[(qkv_v, o_v, S - TS, TS, None)])
    nat = (x_v, s_v, out_v)
    run(out_rows(o_v, xn_v, nat, S - TS, TS))
    gates = routed_gates(sel)
    mark("m16_tail")
    for i in range(N1):
        out_copy(i, A0 + i * TS, TS).wait()
    for (idx, _), g in zip(sel, gates):
        rows = pl.ds(group(idx), 16)
        out_v[rows, :] = (x_v[rows, :].astype(F32) + s_v[rows, :] * g).astype(BF16)
    out_copy(N1, S - TS, TS).start()
    g0, g1 = group(sel[0][0]), group(sel[1][0])

    def fix_copy(i, g):
        return pltpu.make_async_copy(out_v.at[pl.ds(g, 16), :], out_hbm.at[pl.ds(g, 16), :], sem_fix.at[i])

    def sent(g):
        return g < S - TS

    do0 = sent(g0)
    do1 = jnp.logical_and(sent(g1), g1 != g0)

    @pl.when(do0)
    def _():
        fix_copy(0, g0).start()

    @pl.when(do1)
    def _():
        fix_copy(1, g1).start()

    @pl.when(do0)
    def _():
        fix_copy(0, g0).wait()

    @pl.when(do1)
    def _():
        fix_copy(1, g1).wait()

    out_copy(N1, S - TS, TS).wait()
    mark(None)


@jax.jit
def pallas_recurrent_scan__sliding_local_dilated__moe_arch_mod__prompt_kernel(A_x, A_wqkv, A_wo, B_x, B_w_r, B_w_gate, B_w_up, B_w_down):
    del B_x
    TS = CFG["TS"]
    N1 = (S - CFG["B0"]) // TS
    hbm = pl.BlockSpec(memory_space=pltpu.HBM)
    out = pl.pallas_call(
        _kernel,
        out_shape=jax.ShapeDtypeStruct((S, D), BF16),
        in_specs=[hbm] * 7,
        out_specs=hbm,
        scratch_shapes=[
            pltpu.VMEM((S, D), BF16),
            pltpu.VMEM((3, D, D), BF16),
            pltpu.VMEM((D, D), BF16),
            pltpu.VMEM((F, D), BF16),
            pltpu.VMEM((F, D), BF16),
            pltpu.VMEM((F, D), BF16),
            pltpu.VMEM((4, NT, D // 2, 128), U32),
            pltpu.VMEM((3, D // 2, D), U32),
            pltpu.VMEM((D // 2, D), U32),
            pltpu.VMEM(((S + TS) // 2, D), U32),
            pltpu.VMEM((3 * NT + 1, HALO + S, 128), F32),
            pltpu.VMEM((S // 2, D), U32),
            pltpu.VMEM((S, D), F32),
            pltpu.VMEM((S, D), BF16),
            pltpu.VMEM((N1 + 2, 8, 128), F32),
            pltpu.VMEM((D,), BF16),
            pltpu.VMEM((CFG['RL'], D), F32),
            pltpu.VMEM((16, D), BF16),
            pltpu.VMEM((16, D), F32),
            pltpu.SemaphoreType.DMA((11,)),
            pltpu.SemaphoreType.DMA((N1 + 2,)),
            pltpu.SemaphoreType.DMA((2,)),
        ],
        compiler_params=pltpu.CompilerParams(vmem_limit_bytes=100 * 2 ** 20, flags=CFG['flags']),
        name="fused",
    )(A_x.reshape(S, D), A_wqkv, A_wo, B_w_r, B_w_gate.T, B_w_up.T, B_w_down)
    return out.reshape(1, S, D)
```

```python
import functools
import math

import jax
import jax.numpy as jnp
import numpy as np
from jax import lax
from jax.experimental import pallas as pl
from jax.experimental.pallas import tpu as pltpu

F32, BF16, U32, I32 = jnp.float32, jnp.bfloat16, jnp.uint32, jnp.int32

S, D, H, DH, F = 2048, 640, 32, 20, 1728
W, DIL = 8, 2
NT = D // 128
HALO = 16
T = 256
NB = S // T
RA, RL = 8, 16
LOG2E = math.log2(math.e)
EPS_BF16 = float(np.asarray(1e-5, dtype=jnp.bfloat16).astype(np.float32))

CFG = dict(flags=None, lat=100, laga=5, lagl=5, aspan=(0.0, 0.56), lspan=(0.55, 0.8), M=128, quota=(1, 1, 2, 2, 2, 0.5), send=4, e1=(0.0, 0.38), e2=(0.46, 0.8), ksplit=3,
           last=(256,), marks=False)

NT_DIMS = (((1,), (1,)), ((), ()))


def _rb(v):
    return v.astype(BF16).astype(F32)


def _ds(r0, n, align=8):
    return pl.ds(r0 if isinstance(r0, int) else pl.multiple_of(r0, align), n)


def _regroup(src, dst, cols):
    for j in range(DH // 2):
        for g in range(2):
            a = src[pl.ds(g * 160 + j, 8, stride=DH), :]
            b = src[pl.ds(g * 160 + DH // 2 + j, 8, stride=DH), :]
            row = j * H + 8 * g
            dst[row:row + 8, cols] = (a & jnp.uint32(0xFFFF)) | (b << 16)
            dst[row + H // 2:row + H // 2 + 8, cols] = (a >> 16) | (b & jnp.uint32(0xFFFF0000))


def _const(val, gate, rows):
    if gate is None:
        return val
    c = pltpu.bitcast(gate | np.float32(val).view(np.uint32), F32)
    return jnp.concatenate([c] * (rows // 8), axis=0)


def _layernorm(x, gate):
    tot = x[:, :128] if gate is None else x[:, :128] + _const(0.0, gate, x.shape[0])
    for c in range(1, NT):
        tot = tot + x[:, c * 128:(c + 1) * 128]
    mean = jnp.sum(tot, axis=-1, keepdims=True) * (1.0 / D)
    xc = x - mean
    var = jnp.sum(xc * xc, axis=-1, keepdims=True) * (1.0 / D)
    sd = _rb(jnp.sqrt(_rb(_rb(var) + EPS_BF16)))
    return _rb(_rb(x - _rb(mean)) * (1.0 / sd))


def _silu(z):
    h = 0.5 * z
    return h * jnp.tanh(h) + h


def _timed(fns, rows):
    return [((5 * j + 4) // 4 * rows, 5 * (j + 1) * rows // 4, rows, fn) for j, fn in enumerate(fns)]


def _kernel(x_hbm, wqkv_hbm, wo_hbm, wr_hbm, wg_hbm, wu_hbm, wd_hbm, out_hbm,
            x_v, wqkv_v, wo_v, wg_v, wu_v, wd_v, tmp_v, wp_v, wop_v,
            xn_v, qkv_v, o_v, s_v, out_v, wr_v, r_v, xs_v, fix_v, wr1_v, sem_in, sem_out, sem_fix):
    KS = CFG["ksplit"]
    sems = iter(range(sem_in.shape[0]))

    def copy_in(src, dst):
        return pltpu.make_async_copy(src, dst, sem_in.at[next(sems)])

    def x_copy(lo, hi):
        return copy_in(x_hbm.at[lo:hi, :], x_v.at[lo:hi, :])

    def w_copy(m, lo, hi):
        return copy_in(wqkv_hbm.at[lo * 128:hi * 128, m * D:(m + 1) * D], wqkv_v.at[m, lo * 128:hi * 128, :])

    cr = copy_in(wr_hbm, wr1_v)
    cx0, cx1, cx2, cx3 = x_copy(0, T), x_copy(T, 2 * T), x_copy(2 * T, 3 * T), x_copy(3 * T, S)
    cka, ckb, cva, cvb, cq = w_copy(1, 0, KS), w_copy(1, KS, NT), w_copy(2, 0, KS), w_copy(2, KS, NT), w_copy(0, 0, NT)
    cwo = copy_in(wo_hbm, wo_v)
    cg, cu, cd = copy_in(wg_hbm, wg_v), copy_in(wu_hbm, wu_v), copy_in(wd_hbm, wd_v)

    def out_copy(i, r0, n):
        return pltpu.make_async_copy(out_v.at[_ds(r0, n, 16), :], out_hbm.at[_ds(r0, n, 16), :], sem_out.at[i])

    lane = lax.broadcasted_iota(I32, (8, 128), 1)
    sub = lax.broadcasted_iota(I32, (8, 128), 0)

    def prep_qkv(m, lo, hi):
        for c in range(lo, hi):
            tmp_v[m, c] = pltpu.bitcast(wqkv_v[m, c * 128:(c + 1) * 128, :].T, U32)
        for c in range(lo, hi):
            _regroup(tmp_v.at[m, c], wp_v.at[m], slice(c * 128, (c + 1) * 128))

    def prep_wo():
        for c in range(NT):
            tmp_v[3, c] = pltpu.bitcast(wo_v[:, c * 128:(c + 1) * 128], U32)
        for c in range(NT):
            _regroup(tmp_v.at[3, c], wop_v, slice(c * 128, (c + 1) * 128))

    def ln_rows(x, xn_out, row, racc, gate):
        xn = _layernorm(x.astype(F32), gate)
        xn_out[row // 2:(row + RL) // 2, :] = pltpu.bitcast(xn.astype(BF16), U32)
        r = jnp.sum(xn * wr_v[...], axis=-1, keepdims=True)
        acc, n = racc
        for i in range(RL // 8):
            acc = jnp.where(lane == n + i, jnp.broadcast_to(r[8 * i:8 * i + 8], (8, 128)), acc)
        return (acc, n + RL // 8), pltpu.bitcast(acc, U32)

    def proj(xn, qkv, r0, n, mats=(1, 2, 0)):
        def col(m, c):
            y = lax.dot_general(pltpu.bitcast(xn[r0 // 2:(r0 + n) // 2, :], BF16),
                                pltpu.bitcast(wp_v[m, c * 64:(c + 1) * 64, :], BF16),
                                NT_DIMS, preferred_element_type=F32)
            qkv[m * NT + c, HALO + r0:HALO + r0 + n, :] = y
            if m > 0 and r0 == 0:
                qkv[m * NT + c, 0:HALO, :] = jnp.broadcast_to(y[0:1], (HALO, 128))
            return y
        return [functools.partial(col, m, c) for m in mats for c in range(NT)]

    held = {}

    def attn_rows(qkv, o, off, start, gate):
        scale = _const(DH ** -0.5 * LOG2E, gate, RA)
        q = [qkv[c, HALO + off:HALO + off + RA, :] * scale for c in range(NT)]
        lg = []
        for w in range(W):
            lo = HALO + off - DIL * w
            p = q[0] * qkv[NT, lo:lo + RA, :]
            for c in range(1, NT):
                p = p + q[c] * qkv[NT + c, lo:lo + RA, :]
            p = p + pltpu.roll(p, 64, 1)
            p = p + pltpu.roll(p, 32, 1)
            if start is not None and off < DIL * w:
                p = jnp.where(sub >= DIL * w - off - start, p, -1e9 * LOG2E)
            lg.append(p)
        mx = lg[0]
        for w in range(1, W):
            mx = jnp.maximum(mx, lg[w])
        e = [jnp.exp2(l - mx) for l in lg]
        den = e[0]
        for w in range(1, W):
            den = den + e[w]
        inv = pl.reciprocal(den, full_range=False)
        fin = None
        for c in range(NT):
            acc = e[0] * qkv[2 * NT + c, HALO + off:HALO + off + RA, :]
            for w in range(1, W):
                lo = HALO + off - DIL * w
                acc = acc + e[w] * qkv[2 * NT + c, lo:lo + RA, :]
            res = acc * inv
            bits = pltpu.bitcast(res, U32)
            fin = bits if fin is None else fin | bits
            if off % 16 == 0:
                held[c] = res
            else:
                pair = jnp.concatenate([held.pop(c), res], axis=0).astype(BF16)
                o[off // 2 - 4:off // 2 + 4, c * 128:(c + 1) * 128] = pltpu.bitcast(pair, U32)
        return fin

    def out_rows(o, xn, x, s, out, r0, n):
        def col(c):
            cols = slice(c * 128, (c + 1) * 128)
            y = jnp.dot(pltpu.bitcast(o[r0 // 2:(r0 + n) // 2, :], BF16), pltpu.bitcast(wop_v[:, cols], BF16),
                        preferred_element_type=F32)
            s[r0:r0 + n, cols] = y
            g = _silu(pltpu.bitcast(xn[r0 // 2:(r0 + n) // 2, cols], BF16).astype(F32))
            out[r0:r0 + n, cols] = (x[r0:r0 + n, cols].astype(F32) + y * g).astype(BF16)
            return y
        return [functools.partial(col, c) for c in range(NT)]

    def group(idx):
        return pl.multiple_of((idx >> 4) << 4, 16)

    def normed(idx):
        return pltpu.bitcast(xn_v[_ds((idx >> 4) << 3, 8), :], BF16).astype(F32)

    def route():
        imin = jnp.int32(-2 ** 31)
        r = r_v[0]
        for b in range(1, NB):
            if b % 4 == 0:
                first, r = r, r_v[b]
            else:
                r = jnp.where(lane >= b % 4 * 32, pltpu.roll(r_v[b], b % 4 * 32, 1), r)
        comb, vals = [], []
        for i, r in enumerate((first, r)):
            r = _rb(r) + 0.0
            bits = pltpu.bitcast(r, I32)
            key = jnp.where(bits < 0, bits ^ jnp.int32(0x7FFFFFFF), bits) >> 16
            key = jnp.where(r != r, jnp.int32(-2 ** 15), key)
            comb.append(key * S + (S - 1 - i * 1024 - lane * 8 - sub))
            vals.append(r)
        row = lax.broadcasted_iota(I32, (16, D), 0)
        xs = jnp.zeros((16, D), F32)
        sel = []
        for i in range(2):
            best = jnp.max(jnp.maximum(comb[0], comb[1]))
            rv = jnp.where(comb[0] == best, vals[0], jnp.where(comb[1] == best, vals[1], 0.0))
            comb = [jnp.where(cmb == best, imin, cmb) for cmb in comb]
            idx = (S - 1) - (best & (S - 1))
            one = jnp.sum(jnp.where(row == (idx & 15), normed(idx), 0.0), axis=0, keepdims=True)
            xs = jnp.where(row == i, one, xs)
            sel.append((idx, jnp.sum(rv, keepdims=True)))
        xs_v[...] = xs.astype(BF16)
        return sel

    def ffn():
        st = {"y": None}
        bounds = [(lo, min(lo + 128, F)) for lo in range(0, F, 128)]

        def up(name, w, j):
            st[name, j] = lax.dot_general(xs_v[...], w[bounds[j][0]:bounds[j][1], :], NT_DIMS,
                                          preferred_element_type=F32)

        def down(j):
            g = st.pop(("g", j))
            h = (g * jax.nn.sigmoid(g) * st.pop(("u", j))).astype(BF16)
            y = jnp.dot(h, wd_v[bounds[j][0]:bounds[j][1], :], preferred_element_type=F32)
            st["y"] = y if st["y"] is None else st["y"] + y

        steps = []
        for j in range(len(bounds) + 2):
            if j < len(bounds):
                steps += [functools.partial(up, "g", wg_v, j), functools.partial(up, "u", wu_v, j)]
            if j >= 2:
                steps.append(functools.partial(down, j - 2))
        return steps, st

    def routed_gates(sel, y):
        row = lax.broadcasted_iota(I32, (16, D), 0)
        ys = [y[i:i + 1, :] * jax.nn.sigmoid(rv) for i, (_, rv) in enumerate(sel)]
        gates = []
        for idx, _ in sel:
            upd = jnp.zeros((16, D), F32)
            for (other, _), yo in zip(sel, ys):
                upd = jnp.where(row == other - group(idx), yo, upd)
            gates.append(_silu(normed(idx) + upd))
        return gates

    def run(dots, attn=None, ln=None):
        tasks = []
        for first, (lo, hi) in attn[3] if attn is not None else ():
            tasks += [(lo + (hi - lo) * r / T, "a", first + r) for r in range(0, T, RA)]
        if ln is not None:
            lo, hi = ln[-1]
            tasks += [(lo + (hi - lo) * r / T, "l", r) for r in range(0, T, RL)]
        tasks.sort()
        racc = (jnp.zeros((8, 128), F32), 0)
        done = {"a": [], "l": []}
        pos = 0
        for j in range(-1, len(dots)):
            y = dots[j][3]() if j >= 0 else None
            while pos < len(tasks):
                u, kind, off = tasks[pos]
                t = int(u * dots[-1][1]) - CFG["lat"] if dots else 0
                if j + 1 < len(dots) and t >= dots[j + 1][0]:
                    break
                pos += 1
                lag = CFG["lag" + kind]
                bits = done[kind][-lag] if dots and len(done[kind]) >= lag else None
                if y is not None:
                    g = min(t - dots[j][0], dots[j][2] - 8) // 8
                    mine = pltpu.bitcast(y[8 * g:8 * g + 8], U32)
                    bits = mine if bits is None else bits | mine
                gate = None if bits is None else (bits >> 31) >> 1
                if kind == "a":
                    d = attn_rows(attn[0], attn[1], off, attn[2], gate)
                else:
                    racc, d = ln_rows(ln[0][off:off + RL, :], ln[1], ln[2] + off, racc, gate)
                done[kind].append(d)
        if ln is not None:
            r_v[ln[3]] = racc[0]

    scope = [None]

    def mark(name):
        if not CFG.get("marks"):
            return
        if scope[0] is not None:
            scope[0].__exit__(None, None, None)
            scope[0] = None
        if name:
            scope[0] = jax.named_scope(name)
            scope[0].__enter__()

    mark("m00_start")
    for c in (cr, cx0, cka, ckb, cva, cvb, cq, cx1, cwo, cx2, cx3, cg, cu, cd):
        c.start()
    cr.wait()
    cx0.wait()
    mark("m01_ln0")
    wr_v[...] = jnp.broadcast_to(wr1_v[...].astype(F32).reshape(1, D), (RL, D))
    run([], ln=(x_v, xn_v, 0, 0, (0, 0)))
    mark("m02_prepka")
    cka.wait()
    prep_qkv(1, 0, KS)
    mark("m03_prepkb")
    ckb.wait()
    prep_qkv(1, KS, NT)
    h = T // 2
    run(_timed(proj(xn_v, qkv_v, 0, h, (1,)), h))
    mark("m04_kb")
    cva.wait()
    run(_timed(proj(xn_v, qkv_v, h, h, (1,)), h))
    prep_qkv(2, 0, KS)
    mark("m05_va")
    cvb.wait()
    prep_qkv(2, KS, NT)
    run(_timed(proj(xn_v, qkv_v, 0, h, (2,)), h))
    mark("m06_vb")
    cq.wait()
    run(_timed(proj(xn_v, qkv_v, h, h, (2,)), h))
    prep_qkv(0, 0, NT)
    mark("m07_q")
    cx1.wait()
    run(_timed(proj(xn_v, qkv_v, 0, T, (0,)), T), ln=(x_v.at[T:2 * T, :], xn_v, T, 1, (0.0, 0.6)))
    mark("m08_wo")
    cwo.wait()
    prep_wo()
    cx2.wait()
    mark("m11_loop")

    def main(i, carry):
        @pl.when(i == 1)
        def _():
            cx3.wait()

        base = i * T
        qkv = qkv_v.at[:, _ds(base, HALO + 2 * T), :]
        xn = xn_v.at[_ds(i * (T // 2), 3 * T // 2), :]
        o = o_v.at[_ds(i * (T // 2), T // 2), :]
        x, s, out = [ref.at[_ds(base, T, 16), :] for ref in (x_v, s_v, out_v)]
        ahead = x_v.at[_ds(base + 2 * T, T, 16), :]
        run(_timed(proj(xn, qkv, T, T) + out_rows(o, xn, x, s, out, 0, T), T),
            (qkv, o, base, [(0, CFG["aspan"])]), (ahead, xn, 2 * T, i + 2, CFG["lspan"]))
        out_copy(i, base, T).start()
        return carry

    lax.fori_loop(0, NB - 2, main, 0)

    mark("m12_ffn")
    cg.wait()
    cu.wait()
    cd.wait()
    sel = route()
    steps, st = ffn()
    last = S - T
    M = CFG["M"]
    long = proj(xn_v, qkv_v, last, T, (1, 2))
    dots = _timed(long, T)
    mixed = [f for r in range(last, S, M) for f in proj(xn_v, qkv_v, r, M, (0,))]
    mixed += [f for r in range(last - T, S, M) for f in out_rows(o_v, xn_v, x_v, s_v, out_v, r, M)]
    quota = np.cumsum(np.repeat(CFG["quota"], NT))
    quota = np.concatenate([[0], np.round(quota * len(steps) / quota[-1])]).astype(int)

    def both(small, big, send):
        if send:
            out_copy(NB - 2, last - T, 2 * T - M).start()
        for f in small:
            f()
        return big()

    t = dots[-1][1]
    for j, big in enumerate(mixed):
        small = steps[quota[j]:quota[j + 1]]
        t += 5 * M // 4 + 50 * len(small)
        dots.append((t - M, t, M, functools.partial(both, small, big, j == len(mixed) - CFG["send"])))
    run(dots, (qkv_v, o_v, None, [(last - T, CFG["e1"]), (last, CFG["e2"])]))

    for i, ((idx, _), g) in enumerate(zip(sel, routed_gates(sel, st["y"]))):
        rows = pl.ds(group(idx), 16)
        fix_v[i] = (x_v[rows, :].astype(F32) + s_v[rows, :] * g).astype(BF16)
    mark("m16_tail")
    out_copy(NB - 1, S - M, M).start()
    tiles = [group(idx) for idx, _ in sel]
    wanted = [True, tiles[1] != tiles[0]]
    fixes = [pltpu.make_async_copy(fix_v.at[i], out_hbm.at[pl.ds(g, 16), :], sem_fix.at[i])
             for i, g in enumerate(tiles)]
    for i in range(NB - 2):
        out_copy(i, i * T, T).wait()
    for lo, hi, sent in ((0, last - T, None), (last - T, S - M, out_copy(NB - 2, last - T, 2 * T - M)),
                         (S - M, S, out_copy(NB - 1, S - M, M))):
        if sent is not None:
            sent.wait()
        for fix, g, want in zip(fixes, tiles, wanted):
            pl.when((g >= lo) & (g < hi) & want)(fix.start)
    fixes[0].wait()
    pl.when(wanted[1])(fixes[1].wait)
    mark(None)


@jax.jit
def pallas_recurrent_scan__sliding_local_dilated__moe_arch_mod__prompt_kernel(A_x, A_wqkv, A_wo, B_x, B_w_r, B_w_gate, B_w_up, B_w_down):
    del B_x
    hbm = pl.BlockSpec(memory_space=pltpu.HBM)
    out = pl.pallas_call(
        _kernel,
        out_shape=jax.ShapeDtypeStruct((S, D), BF16),
        in_specs=[hbm] * 7,
        out_specs=hbm,
        scratch_shapes=[
            pltpu.VMEM((S, D), BF16),
            pltpu.VMEM((3, D, D), BF16),
            pltpu.VMEM((D, D), BF16),
            pltpu.VMEM((F, D), BF16),
            pltpu.VMEM((F, D), BF16),
            pltpu.VMEM((F, D), BF16),
            pltpu.VMEM((4, NT, D // 2, 128), U32),
            pltpu.VMEM((3, D // 2, D), U32),
            pltpu.VMEM((D // 2, D), U32),
            pltpu.VMEM(((S + T) // 2, D), U32),
            pltpu.VMEM((3 * NT + 1, HALO + S, 128), F32),
            pltpu.VMEM((S // 2, D), U32),
            pltpu.VMEM((S, D), F32),
            pltpu.VMEM((S, D), BF16),
            pltpu.VMEM((RL, D), F32),
            pltpu.VMEM((NB + 1, 8, 128), F32),
            pltpu.VMEM((16, D), BF16),
            pltpu.VMEM((2, 16, D), BF16),
            pltpu.VMEM((D,), BF16),
            pltpu.SemaphoreType.DMA((14,)),
            pltpu.SemaphoreType.DMA((NB,)),
            pltpu.SemaphoreType.DMA((2,)),
        ],
        compiler_params=pltpu.CompilerParams(vmem_limit_bytes=100 * 2 ** 20, flags=CFG['flags']),
        name="fused",
    )(A_x.reshape(S, D), A_wqkv, A_wo, B_w_r, B_w_gate.T, B_w_up.T, B_w_down)
    return out.reshape(1, S, D)
```

```python
import functools
import math

import jax
import jax.numpy as jnp
import numpy as np
from jax import lax
from jax.experimental import pallas as pl
from jax.experimental.pallas import tpu as pltpu

F32, BF16, U32, I32 = jnp.float32, jnp.bfloat16, jnp.uint32, jnp.int32

S, D, H, DH, F = 2048, 640, 32, 20, 1728
W, DIL = 8, 2
NT = D // 128
HALO = 16
T = 256
NB = S // T
RA, RL = 8, 16
LOG2E = math.log2(math.e)
EPS_BF16 = float(np.asarray(1e-5, dtype=jnp.bfloat16).astype(np.float32))

CFG = dict(flags=None, lat=100, laga=5, lagl=5, aspan=(0.0, 0.5), lspan=(0.55, 0.8), M=128, quota=(1, 1, 1, 1, 1.5, 1.5, 1.5, 0.5), send=4, e1=(0.0, 0.42), e2=(0.5, 0.8), ksplit=3, U=2, h=128, nlong=1,
           last=(256,), marks=False)

NT_DIMS = (((1,), (1,)), ((), ()))


def _rb(v):
    return v.astype(BF16).astype(F32)


def _ds(r0, n, align=8):
    return pl.ds(r0 if isinstance(r0, int) else pl.multiple_of(r0, align), n)


def _regroup(src, dst, cols):
    for j in range(DH // 2):
        for g in range(2):
            a = src[pl.ds(g * 160 + j, 8, stride=DH), :]
            b = src[pl.ds(g * 160 + DH // 2 + j, 8, stride=DH), :]
            row = j * H + 8 * g
            dst[row:row + 8, cols] = (a & jnp.uint32(0xFFFF)) | (b << 16)
            dst[row + H // 2:row + H // 2 + 8, cols] = (a >> 16) | (b & jnp.uint32(0xFFFF0000))


def _const(val, gate, rows):
    if gate is None:
        return val
    c = pltpu.bitcast(gate | np.float32(val).view(np.uint32), F32)
    return jnp.concatenate([c] * (rows // 8), axis=0)


def _layernorm(x, gate):
    tot = x[:, :128] if gate is None else x[:, :128] + _const(0.0, gate, x.shape[0])
    for c in range(1, NT):
        tot = tot + x[:, c * 128:(c + 1) * 128]
    mean = jnp.sum(tot, axis=-1, keepdims=True) * (1.0 / D)
    xc = x - mean
    var = jnp.sum(xc * xc, axis=-1, keepdims=True) * (1.0 / D)
    sd = _rb(jnp.sqrt(_rb(_rb(var) + EPS_BF16)))
    return (_rb(x - _rb(mean)) * (1.0 / sd)).astype(BF16)


def _silu(z):
    h = 0.5 * z
    return h * jnp.tanh(h) + h


def _timed(fns, rows):
    return [((5 * j + 4) // 4 * rows, 5 * (j + 1) * rows // 4, rows, fn) for j, fn in enumerate(fns)]


def _kernel(x_hbm, wqkv_hbm, wo_hbm, wr_hbm, wg_hbm, wu_hbm, wd_hbm, out_hbm,
            x_v, wqkv_v, wo_v, wg_v, wu_v, wd_v, tmp_v, wp_v, wop_v,
            xn_v, qkv_v, o_v, s_v, out_v, wr_v, r_v, xs_v, fix_v, wr1_v, sem_in, sem_out, sem_fix):
    KS = CFG["ksplit"]
    sems = iter(range(sem_in.shape[0]))

    def copy_in(src, dst):
        return pltpu.make_async_copy(src, dst, sem_in.at[next(sems)])

    def x_copy(lo, hi):
        return copy_in(x_hbm.at[lo:hi, :], x_v.at[lo:hi, :])

    def w_copy(m, lo, hi):
        return copy_in(wqkv_hbm.at[lo * 128:hi * 128, m * D:(m + 1) * D], wqkv_v.at[m, lo * 128:hi * 128, :])

    cr = copy_in(wr_hbm, wr1_v)
    cx0, cx1, cx2, cx3 = x_copy(0, T), x_copy(T, 2 * T), x_copy(2 * T, (2 + CFG['U']) * T), x_copy((2 + CFG['U']) * T, S)
    cka, ckb, cv, cq = w_copy(1, 0, KS), w_copy(1, KS, NT), w_copy(2, 0, NT), w_copy(0, 0, NT)
    cwo = [copy_in(wo_hbm.at[:, c * 128:(c + 1) * 128], wo_v.at[c]) for c in range(NT)]
    cg, cu, cd = copy_in(wg_hbm, wg_v), copy_in(wu_hbm, wu_v), copy_in(wd_hbm, wd_v)

    def out_copy(i, r0, n):
        return pltpu.make_async_copy(out_v.at[_ds(r0, n, 16), :], out_hbm.at[_ds(r0, n, 16), :], sem_out.at[i])

    lane = lax.broadcasted_iota(I32, (8, 128), 1)
    sub = lax.broadcasted_iota(I32, (8, 128), 0)

    def prep_qkv(m, lo, hi):
        for c in range(lo, hi):
            tmp_v[m, c] = pltpu.bitcast(wqkv_v[m, c * 128:(c + 1) * 128, :].T, U32)
        for c in range(lo, hi):
            _regroup(tmp_v.at[m, c], wp_v.at[m], slice(c * 128, (c + 1) * 128))

    def prep_wo():
        for c in range(NT):
            _regroup(wo_v.bitcast(U32).at[c], wop_v, slice(c * 128, (c + 1) * 128))

    def ln_rows(x, xn_out, row, slot, scores, gate):
        xn = _layernorm(x[row:row + RL, :].astype(F32), gate)
        xn_out[row // 2:(row + RL) // 2, :] = pltpu.bitcast(xn, U32)
        r = jnp.sum(xn.astype(F32) * wr_v[...], axis=-1, keepdims=True)
        for i in range(RL // 8):
            scores = jnp.where(lane == slot + i, jnp.broadcast_to(r[8 * i:8 * i + 8], (8, 128)), scores)
        return scores

    def proj(xn, qkv, r0, n, mats=(1, 2, 0)):
        def col(m, c):
            y = lax.dot_general(pltpu.bitcast(xn[r0 // 2:(r0 + n) // 2, :], BF16),
                                pltpu.bitcast(wp_v[m, c * 64:(c + 1) * 64, :], BF16),
                                NT_DIMS, preferred_element_type=F32)
            qkv[m * NT + c, HALO + r0:HALO + r0 + n, :] = y
            if m > 0 and r0 == 0:
                qkv[m * NT + c, 0:HALO, :] = jnp.broadcast_to(y[0:1], (HALO, 128))
            return y
        return [functools.partial(col, m, c) for m in mats for c in range(NT)]

    held = {}

    def attn_rows(qkv, o, off, start, gate):
        scale = _const(DH ** -0.5 * LOG2E, gate, RA)
        q = [qkv[c, HALO + off:HALO + off + RA, :] * scale for c in range(NT)]
        lg = []
        for w in range(W):
            lo = HALO + off - DIL * w
            p = q[0] * qkv[NT, lo:lo + RA, :]
            for c in range(1, NT):
                p = p + q[c] * qkv[NT + c, lo:lo + RA, :]
            p = p + pltpu.roll(p, 64, 1)
            p = p + pltpu.roll(p, 32, 1)
            if start is not None and off < DIL * w:
                p = jnp.where(sub >= DIL * w - off - start, p, -1e9 * LOG2E)
            lg.append(p)
        mx = lg[0]
        for w in range(1, W):
            mx = jnp.maximum(mx, lg[w])
        e = [jnp.exp2(l - mx) for l in lg]
        den = e[0]
        for w in range(1, W):
            den = den + e[w]
        inv = pl.reciprocal(den, full_range=False)
        fin = None
        for c in range(NT):
            acc = e[0] * qkv[2 * NT + c, HALO + off:HALO + off + RA, :]
            for w in range(1, W):
                lo = HALO + off - DIL * w
                acc = acc + e[w] * qkv[2 * NT + c, lo:lo + RA, :]
            res = acc * inv
            bits = pltpu.bitcast(res, U32)
            fin = bits if fin is None else fin | bits
            if off % 16 == 0:
                held[c] = res
            else:
                pair = jnp.concatenate([held.pop(c), res], axis=0).astype(BF16)
                o[off // 2 - 4:off // 2 + 4, c * 128:(c + 1) * 128] = pltpu.bitcast(pair, U32)
        return fin

    def out_rows(o, xn, x, s, out, r0, n):
        def col(c):
            cols = slice(c * 128, (c + 1) * 128)
            y = jnp.dot(pltpu.bitcast(o[r0 // 2:(r0 + n) // 2, :], BF16), pltpu.bitcast(wop_v[:, cols], BF16),
                        preferred_element_type=F32)
            s[r0:r0 + n, cols] = y
            g = _silu(pltpu.bitcast(xn[r0 // 2:(r0 + n) // 2, cols], BF16).astype(F32))
            out[r0:r0 + n, cols] = (x[r0:r0 + n, cols].astype(F32) + y * g).astype(BF16)
            return y
        return [functools.partial(col, c) for c in range(NT)]

    def group(idx):
        return pl.multiple_of((idx >> 4) << 4, 16)

    def normed(idx):
        return pltpu.bitcast(xn_v[_ds((idx >> 4) << 3, 8), :], BF16).astype(F32)

    def route():
        imin = jnp.int32(-2 ** 31)
        r = r_v[0]
        for b in range(1, NB):
            if b % 4 == 0:
                first, r = r, r_v[b]
            else:
                r = jnp.where(lane >= b % 4 * 32, pltpu.roll(r_v[b], b % 4 * 32, 1), r)
        comb, vals = [], []
        for i, r in enumerate((first, r)):
            r = _rb(r) + 0.0
            bits = pltpu.bitcast(r, I32)
            key = jnp.where(bits < 0, bits ^ jnp.int32(0x7FFFFFFF), bits) >> 16
            key = jnp.where(r != r, jnp.int32(-2 ** 15), key)
            comb.append(key * S + (S - 1 - i * 1024 - lane * 8 - sub))
            vals.append(r)
        row = lax.broadcasted_iota(I32, (16, D), 0)
        xs = jnp.zeros((16, D), F32)
        sel = []
        for i in range(2):
            best = jnp.max(jnp.maximum(comb[0], comb[1]))
            rv = jnp.where(comb[0] == best, vals[0], jnp.where(comb[1] == best, vals[1], 0.0))
            comb = [jnp.where(cmb == best, imin, cmb) for cmb in comb]
            idx = (S - 1) - (best & (S - 1))
            one = jnp.sum(jnp.where(row == (idx & 15), normed(idx), 0.0), axis=0, keepdims=True)
            xs = jnp.where(row == i, one, xs)
            sel.append((idx, jnp.sum(rv, keepdims=True)))
        xs_v[...] = xs.astype(BF16)
        return sel

    def ffn():
        st = {"y": None}
        bounds = [(lo, min(lo + 128, F)) for lo in range(0, F, 128)]

        def up(name, w, j):
            st[name, j] = lax.dot_general(xs_v[...], w[bounds[j][0]:bounds[j][1], :], NT_DIMS,
                                          preferred_element_type=F32)

        def down(j):
            g = st.pop(("g", j))
            h = (g * jax.nn.sigmoid(g) * st.pop(("u", j))).astype(BF16)
            y = jnp.dot(h, wd_v[bounds[j][0]:bounds[j][1], :], preferred_element_type=F32)
            st["y"] = y if st["y"] is None else st["y"] + y

        steps = []
        for j in range(len(bounds) + 2):
            if j < len(bounds):
                steps += [functools.partial(up, "g", wg_v, j), functools.partial(up, "u", wu_v, j)]
            if j >= 2:
                steps.append(functools.partial(down, j - 2))
        return steps, st

    def routed_gates(sel, y):
        row = lax.broadcasted_iota(I32, (16, D), 0)
        ys = [y[i:i + 1, :] * jax.nn.sigmoid(rv) for i, (_, rv) in enumerate(sel)]
        gates = []
        for idx, _ in sel:
            upd = jnp.zeros((16, D), F32)
            for (other, _), yo in zip(sel, ys):
                upd = jnp.where(row == other - group(idx), yo, upd)
            gates.append(_silu(normed(idx) + upd))
        return gates

    def run(dots, attn=(), ln=()):
        tasks = []
        for kind, jobs, step in (("a", attn, RA), ("l", ln, RL)):
            for k, job in enumerate(jobs):
                lo, hi = job[-1]
                tasks += [(lo + (hi - lo) * r / T, kind, k, r) for r in range(0, T, step)]
        tasks.sort()
        done = {"a": [], "l": []}
        pos = 0
        for j in range(-1, len(dots)):
            y = dots[j][3]() if j >= 0 else None
            while pos < len(tasks):
                u, kind, k, off = tasks[pos]
                t = int(u * dots[-1][1]) - CFG["lat"] if dots else 0
                if j + 1 < len(dots) and t >= dots[j + 1][0]:
                    break
                pos += 1
                lag = CFG["lag" + kind]
                bits = done[kind][-lag] if dots and len(done[kind]) >= lag else None
                if y is not None:
                    g = min(t - dots[j][0], dots[j][2] - 8) // 8
                    mine = pltpu.bitcast(y[8 * g:8 * g + 8], U32)
                    bits = mine if bits is None else bits | mine
                gate = None if bits is None else (bits >> 31) >> 1
                if kind == "a":
                    qkv, o, first, start, _ = attn[k]
                    done[kind].append(attn_rows(qkv, o, first + off, start, gate))
                else:
                    x, xn, first, blk, _ = ln[k]
                    if off == 0:
                        scores = jnp.zeros((8, 128), F32)
                    scores = ln_rows(x, xn, first + off, off // 8, scores, gate)
                    done[kind].append(pltpu.bitcast(scores, U32))
                    if off == T - RL:
                        r_v[blk] = scores

    scope = [None]

    def mark(name):
        if not CFG.get("marks"):
            return
        if scope[0] is not None:
            scope[0].__exit__(None, None, None)
            scope[0] = None
        if name:
            scope[0] = jax.named_scope(name)
            scope[0].__enter__()

    mark("m00_start")
    for c in (cr, cx0, cka, ckb, cv, cq, cx1, *cwo, cx2, cx3, cg, cu, cd):
        c.start()
    cr.wait()
    cx0.wait()
    mark("m01_ln0")
    wr_v[...] = jnp.broadcast_to(wr1_v[...].astype(F32).reshape(1, D), (RL, D))
    run([], ln=[(x_v, xn_v, 0, 0, (0, 0))])
    mark("m02_prepka")
    cka.wait()
    prep_qkv(1, 0, KS)
    mark("m03_prepkb")
    ckb.wait()
    prep_qkv(1, KS, NT)
    h = CFG["h"]
    run(_timed(proj(xn_v, qkv_v, 0, h, (1,)), h))
    mark("m04_kb")
    cv.wait()
    run(_timed(proj(xn_v, qkv_v, h, T - h, (1,)), T - h))
    prep_qkv(2, 0, NT)
    run(_timed(proj(xn_v, qkv_v, 0, T // 2, (2,)), T // 2))
    h = T // 2
    mark("m06_vb")
    cq.wait()
    run(_timed(proj(xn_v, qkv_v, h, h, (2,)), h))
    prep_qkv(0, 0, NT)
    mark("m07_q")
    cx1.wait()
    run(_timed(proj(xn_v, qkv_v, 0, T, (0,)), T), ln=[(x_v, xn_v, T, 1, (0.0, 0.6))])
    mark("m08_wo")
    for c in cwo:
        c.wait()
    prep_wo()
    cx2.wait()
    mark("m11_loop")

    U = CFG["U"]

    def main(i, carry):
        base = i * (U * T)
        qkv = qkv_v.at[:, _ds(base, HALO + (U + 1) * T), :]
        xn = xn_v.at[_ds(i * (U * T // 2), (U + 2) * T // 2), :]
        o = o_v.at[_ds(i * (U * T // 2), U * T // 2), :]
        x = x_v.at[_ds(base, (U + 2) * T, 16), :]
        s, out = [ref.at[_ds(base, U * T, 16), :] for ref in (s_v, out_v)]
        dots, attn, ln = [], [], []
        for k in range(U):
            dots += proj(xn, qkv, (k + 1) * T, T) + out_rows(o, xn, x, s, out, k * T, T)
            attn.append((qkv, o, k * T, base, [(k + f) / U for f in CFG["aspan"]]))
            ln.append((x, xn, (k + 2) * T, i * U + k + 2, [(k + f) / U for f in CFG["lspan"]]))
        run(_timed(dots, T), attn, ln)
        out_copy(i, base, U * T).start()

        pl.when(i == 0)(cx3.wait)

        return carry

    lax.fori_loop(0, (NB - 2) // U, main, 0)

    mark("m12_ffn")
    cg.wait()
    cu.wait()
    cd.wait()
    sel = route()
    steps, st = ffn()
    last = S - T
    M = CFG["M"]
    NL = CFG["nlong"]
    long = proj(xn_v, qkv_v, last, T, (1, 2, 0)[:NL])
    dots = _timed(long, T)
    mixed = [f for m in (1, 2, 0)[NL:] for r in range(last, S, M) for f in proj(xn_v, qkv_v, r, M, (m,))]
    mixed += [f for r in range(last - T, S, M) for f in out_rows(o_v, xn_v, x_v, s_v, out_v, r, M)]
    quota = np.cumsum(np.repeat(CFG["quota"], NT))
    quota = np.concatenate([[0], np.round(quota * len(steps) / quota[-1])]).astype(int)

    def both(small, big, send):
        if send:
            out_copy(NB - 2, last - T, 2 * T - M).start()
        for f in small:
            f()
        return big()

    t = dots[-1][1]
    for j, big in enumerate(mixed):
        small = steps[quota[j]:quota[j + 1]]
        t += 5 * M // 4 + 50 * len(small)
        dots.append((t - M, t, M, functools.partial(both, small, big, j == len(mixed) - CFG["send"])))
    run(dots, [(qkv_v, o_v, last - T, None, CFG["e1"]), (qkv_v, o_v, last, None, CFG["e2"])])

    for i, ((idx, _), g) in enumerate(zip(sel, routed_gates(sel, st["y"]))):
        rows = pl.ds(group(idx), 16)
        fix_v[i] = (x_v[rows, :].astype(F32) + s_v[rows, :] * g).astype(BF16)
    mark("m16_tail")
    out_copy(NB - 1, S - M, M).start()
    tiles = [group(idx) for idx, _ in sel]
    wanted = [True, tiles[1] != tiles[0]]
    fixes = [pltpu.make_async_copy(fix_v.at[i], out_hbm.at[pl.ds(g, 16), :], sem_fix.at[i])
             for i, g in enumerate(tiles)]
    for i in range((NB - 2) // U):
        out_copy(i, i * U * T, U * T).wait()
    for lo, hi, sent in ((0, last - T, None), (last - T, S - M, out_copy(NB - 2, last - T, 2 * T - M)),
                         (S - M, S, out_copy(NB - 1, S - M, M))):
        if sent is not None:
            sent.wait()
        for fix, g, want in zip(fixes, tiles, wanted):
            pl.when((g >= lo) & (g < hi) & want)(fix.start)
    fixes[0].wait()
    pl.when(wanted[1])(fixes[1].wait)
    mark(None)


@jax.jit
def pallas_recurrent_scan__sliding_local_dilated__moe_arch_mod__prompt_kernel(A_x, A_wqkv, A_wo, B_x, B_w_r, B_w_gate, B_w_up, B_w_down):
    del B_x
    hbm = pl.BlockSpec(memory_space=pltpu.HBM)
    out = pl.pallas_call(
        _kernel,
        out_shape=jax.ShapeDtypeStruct((S, D), BF16),
        in_specs=[hbm] * 7,
        out_specs=hbm,
        scratch_shapes=[
            pltpu.VMEM((S, D), BF16),
            pltpu.VMEM((3, D, D), BF16),
            pltpu.VMEM((NT, D, 128), BF16),
            pltpu.VMEM((F, D), BF16),
            pltpu.VMEM((F, D), BF16),
            pltpu.VMEM((F, D), BF16),
            pltpu.VMEM((3, NT, D // 2, 128), U32),
            pltpu.VMEM((3, D // 2, D), U32),
            pltpu.VMEM((D // 2, D), U32),
            pltpu.VMEM((S // 2, D), U32),
            pltpu.VMEM((3 * NT + 1, HALO + S, 128), F32),
            pltpu.VMEM((S // 2, D), U32),
            pltpu.VMEM((S, D), F32),
            pltpu.VMEM((S, D), BF16),
            pltpu.VMEM((RL, D), F32),
            pltpu.VMEM((NB, 8, 128), F32),
            pltpu.VMEM((16, D), BF16),
            pltpu.VMEM((2, 16, D), BF16),
            pltpu.VMEM((D,), BF16),
            pltpu.SemaphoreType.DMA((17,)),
            pltpu.SemaphoreType.DMA((NB,)),
            pltpu.SemaphoreType.DMA((2,)),
        ],
        compiler_params=pltpu.CompilerParams(vmem_limit_bytes=100 * 2 ** 20, flags=CFG['flags']),
        name="fused",
    )(A_x.reshape(S, D), A_wqkv, A_wo, B_w_r, B_w_gate.T, B_w_up.T, B_w_down)
    return out.reshape(1, S, D)
```

```python
import functools
import math

import jax
import jax.numpy as jnp
import numpy as np
from jax import lax
from jax.experimental import pallas as pl
from jax.experimental.pallas import tpu as pltpu

F32, BF16, U32, I32 = jnp.float32, jnp.bfloat16, jnp.uint32, jnp.int32

S, D, H, DH, F = 2048, 640, 32, 20, 1728
W, DIL = 8, 2
NT = D // 128
TILES = [slice(c * 128, (c + 1) * 128) for c in range(NT)]
HALO = 16
T = 256
NB = S // T
RA, RL = 8, 16
LOG2E = math.log2(math.e)
EPS_BF16 = float(np.asarray(1e-5, dtype=jnp.bfloat16).astype(np.float32))

CFG = dict(flags=None, lat=100, laga=4, lagl=5, aspan=(0.0, 0.5), lspan=(0.55, 0.8), M=128, quota=(0, 0.5, 1, 1, 1, 1, 1, 1, 1, 0.4), send=5, e1=(0.0, 0.4), e2=(0.4, 0.86), ksplit=3, U=2, h=128, fc=5, skip=9, split=True, nlong=1,
           last=(256,), marks=False)

NN_DIMS = (((1,), (0,)), ((), ()))
NT_DIMS = (((1,), (1,)), ((), ()))


def _rb(v):
    return v.astype(BF16).astype(F32)


def _ds(r0, n, align=8):
    return pl.ds(r0 if isinstance(r0, int) else pl.multiple_of(r0, align), n)


def _regroup(src, dst, cols):
    for j in range(DH // 2):
        for g in range(2):
            a = src[pl.ds(g * 160 + j, 8, stride=DH), :]
            b = src[pl.ds(g * 160 + DH // 2 + j, 8, stride=DH), :]
            row = j * H + 8 * g
            dst[row:row + 8, cols] = (a & jnp.uint32(0xFFFF)) | (b << 16)
            dst[row + H // 2:row + H // 2 + 8, cols] = (a >> 16) | (b & jnp.uint32(0xFFFF0000))


def _const(val, gate, rows):
    if gate is None:
        return val
    c = pltpu.bitcast(gate | np.float32(val).view(np.uint32), F32)
    return jnp.concatenate([c] * (rows // 8), axis=0)


def _layernorm(x, gate):
    tot = x[:, :128] if gate is None else x[:, :128] + _const(0.0, gate, x.shape[0])
    for c in range(1, NT):
        tot = tot + x[:, c * 128:(c + 1) * 128]
    mean = jnp.sum(tot, axis=-1, keepdims=True) * (1.0 / D)
    xc = x - mean
    var = jnp.sum(xc * xc, axis=-1, keepdims=True) * (1.0 / D)
    sd = _rb(jnp.sqrt(_rb(_rb(var) + EPS_BF16)))
    return (_rb(x - _rb(mean)) * (1.0 / sd)).astype(BF16)


def _silu(z):
    h = 0.5 * z
    return h * jnp.tanh(h) + h


def _tiles(lhs, rhs, dims, finish):
    acc = []

    def step(k, parts=1):
        a, b = lhs(TILES[k]), rhs(TILES[k])
        n = a.shape[0] // parts
        y = jnp.concatenate([lax.dot_general(a[i * n:(i + 1) * n], b, dims, preferred_element_type=F32)
                             for i in range(parts)], axis=0)
        acc.append(y if k == 0 else acc.pop() + y)
        if k == NT - 1:
            finish(acc.pop())
        return y

    return [functools.partial(step, k) for k in range(NT)]


def _timed(steps, rows, extra=None):
    left = len(steps) % 4
    if left in (1, 2) and CFG["split"]:
        steps = steps[:-left] + [functools.partial(step, parts=4 // left) for step in steps[-left:]]
    groups, t = [], 0
    for j in range(0, len(steps), 4):
        short = extra(j // 4) if extra else []
        t += CFG["fc"] * len(short)
        groups.append((t, rows, short + steps[j:j + 4]))
        t += rows
    return groups


def _kernel(x_hbm, wqkv_hbm, wo_hbm, wr_hbm, wg_hbm, wu_hbm, wd_hbm, out_hbm,
            x_v, wqkv_v, wo_v, wg_v, wu_v, wd_v, tmp_v, wp_v, wop_v,
            xn_v, qkv_v, o_v, s_v, out_v, wr_v, r_v, xs_v, fix_v, wr1_v, sem_in, sem_out, sem_fix):
    KS = CFG["ksplit"]
    sems = iter(range(sem_in.shape[0]))

    def copy_in(src, dst):
        return pltpu.make_async_copy(src, dst, sem_in.at[next(sems)])

    def x_copy(lo, hi):
        return copy_in(x_hbm.at[lo:hi, :], x_v.at[lo:hi, :])

    def w_copy(m, lo, hi):
        return copy_in(wqkv_hbm.at[lo * 128:hi * 128, m * D:(m + 1) * D], wqkv_v.at[m, lo * 128:hi * 128, :])

    cr = copy_in(wr_hbm, wr1_v)
    cx0, cx1, cx2, cx3 = x_copy(0, T), x_copy(T, 2 * T), x_copy(2 * T, (2 + CFG['U']) * T), x_copy((2 + CFG['U']) * T, S)
    cka, ckb, cv, cq = w_copy(1, 0, KS), w_copy(1, KS, NT), w_copy(2, 0, NT), w_copy(0, 0, NT)
    cwo = [copy_in(wo_hbm.at[:, c * 128:(c + 1) * 128], wo_v.at[c]) for c in range(NT)]
    cg, cu, cd = copy_in(wg_hbm, wg_v), copy_in(wu_hbm, wu_v), copy_in(wd_hbm, wd_v)

    def out_copy(i, r0, n):
        return pltpu.make_async_copy(out_v.at[_ds(r0, n, 16), :], out_hbm.at[_ds(r0, n, 16), :], sem_out.at[i])

    lane = lax.broadcasted_iota(I32, (8, 128), 1)
    sub = lax.broadcasted_iota(I32, (8, 128), 0)

    def prep_qkv(m, lo, hi):
        for c in range(lo, hi):
            tmp_v[m, c] = pltpu.bitcast(wqkv_v[m, c * 128:(c + 1) * 128, :].T, U32)
        for c in range(lo, hi):
            _regroup(tmp_v.at[m, c], wp_v.at[m], slice(c * 128, (c + 1) * 128))

    def prep_wo():
        for c in range(NT):
            _regroup(wo_v.bitcast(U32).at[c], wop_v, slice(c * 128, (c + 1) * 128))

    def ln_rows(x, xn_out, row, slot, scores, gate):
        xn = _layernorm(x[row:row + RL, :].astype(F32), gate)
        xn_out[row // 2:(row + RL) // 2, :] = pltpu.bitcast(xn, U32)
        r = jnp.sum(xn.astype(F32) * wr_v[...], axis=-1, keepdims=True)
        for i in range(RL // 8):
            scores = jnp.where(lane == slot + i, jnp.broadcast_to(r[8 * i:8 * i + 8], (8, 128)), scores)
        return scores

    def proj(xn, qkv, r0, n, mats=(1, 2, 0)):
        def finish(m, c, y):
            qkv[m * NT + c, HALO + r0:HALO + r0 + n, :] = y
            if m > 0 and r0 == 0:
                qkv[m * NT + c, 0:HALO, :] = jnp.broadcast_to(y[0:1], (HALO, 128))

        return [step for m in mats for c in range(NT) for step in _tiles(
            lambda k: pltpu.bitcast(xn[r0 // 2:(r0 + n) // 2, k], BF16),
            lambda k, m=m, c=c: pltpu.bitcast(wp_v[m, c * 64:(c + 1) * 64, k], BF16),
            NT_DIMS, functools.partial(finish, m, c))]

    held = {}

    def attn_rows(qkv, o, off, start, gate):
        scale = _const(DH ** -0.5 * LOG2E, gate, RA)
        q = [qkv[c, HALO + off:HALO + off + RA, :] * scale for c in range(NT)]
        lg = []
        for w in range(W):
            lo = HALO + off - DIL * w
            p = q[0] * qkv[NT, lo:lo + RA, :]
            for c in range(1, NT):
                p = p + q[c] * qkv[NT + c, lo:lo + RA, :]
            p = p + pltpu.roll(p, 64, 1)
            p = p + pltpu.roll(p, 32, 1)
            if start is not None and off < DIL * w:
                p = jnp.where(sub >= DIL * w - off - start, p, -1e9 * LOG2E)
            lg.append(p)
        mx = lg[0]
        for w in range(1, W):
            mx = jnp.maximum(mx, lg[w])
        e = [jnp.exp2(l - mx) for l in lg]
        den = e[0]
        for w in range(1, W):
            den = den + e[w]
        inv = pl.reciprocal(den, full_range=False)
        fin = None
        for c in range(NT):
            acc = e[0] * qkv[2 * NT + c, HALO + off:HALO + off + RA, :]
            for w in range(1, W):
                lo = HALO + off - DIL * w
                acc = acc + e[w] * qkv[2 * NT + c, lo:lo + RA, :]
            res = acc * inv
            bits = pltpu.bitcast(res, U32)
            fin = bits if fin is None else fin | bits
            if off % 16 == 0:
                held[c] = res
            else:
                pair = jnp.concatenate([held.pop(c), res], axis=0).astype(BF16)
                o[off // 2 - 4:off // 2 + 4, c * 128:(c + 1) * 128] = pltpu.bitcast(pair, U32)
        return fin

    def out_rows(o, xn, x, s, out, r0, n):
        def finish(cols, y):
            s[r0:r0 + n, cols] = y
            g = _silu(pltpu.bitcast(xn[r0 // 2:(r0 + n) // 2, cols], BF16).astype(F32))
            out[r0:r0 + n, cols] = (x[r0:r0 + n, cols].astype(F32) + y * g).astype(BF16)

        return [step for cols in TILES for step in _tiles(
            lambda k: pltpu.bitcast(o[r0 // 2:(r0 + n) // 2, k], BF16),
            lambda k, cols=cols: pltpu.bitcast(wop_v[k.start // 2:k.stop // 2, cols], BF16),
            NN_DIMS, functools.partial(finish, cols))]

    def group(idx):
        return pl.multiple_of((idx >> 4) << 4, 16)

    def normed(idx):
        return pltpu.bitcast(xn_v[_ds((idx >> 4) << 3, 8), :], BF16).astype(F32)

    def route():
        imin = jnp.int32(-2 ** 31)
        r = r_v[0]
        for b in range(1, NB):
            if b % 4 == 0:
                first, r = r, r_v[b]
            else:
                r = jnp.where(lane >= b % 4 * 32, pltpu.roll(r_v[b], b % 4 * 32, 1), r)
        comb, vals = [], []
        for i, r in enumerate((first, r)):
            r = _rb(r) + 0.0
            bits = pltpu.bitcast(r, I32)
            key = jnp.where(bits < 0, bits ^ jnp.int32(0x7FFFFFFF), bits) >> 16
            key = jnp.where(r != r, jnp.int32(-2 ** 15), key)
            comb.append(key * S + (S - 1 - i * 1024 - lane * 8 - sub))
            vals.append(r)
        row = lax.broadcasted_iota(I32, (16, D), 0)
        xs = jnp.zeros((16, D), F32)
        sel = []
        for i in range(2):
            best = jnp.max(jnp.maximum(comb[0], comb[1]))
            rv = jnp.where(comb[0] == best, vals[0], jnp.where(comb[1] == best, vals[1], 0.0))
            comb = [jnp.where(cmb == best, imin, cmb) for cmb in comb]
            idx = (S - 1) - (best & (S - 1))
            one = jnp.sum(jnp.where(row == (idx & 15), normed(idx), 0.0), axis=0, keepdims=True)
            xs = jnp.where(row == i, one, xs)
            sel.append((idx, jnp.sum(rv, keepdims=True)))
        xs_v[...] = xs.astype(BF16)
        return sel

    def ffn():
        chunks = [slice(lo, min(lo + 128, F)) for lo in range(0, F, 128)]
        pre, hid, y = {}, {}, [0.0] * NT

        def up(w, j):
            return _tiles(lambda k: xs_v[:, k], lambda k: w[chunks[j], k], NT_DIMS, pre.setdefault(j, []).append)

        def down(j, c):
            if c == 0:
                g, u = pre[j]
                hid[j] = (g * jax.nn.sigmoid(g) * u).astype(BF16)
            y[c] = y[c] + jnp.dot(hid[j], wd_v[chunks[j], TILES[c]], preferred_element_type=F32)

        steps = []
        for j in range(len(chunks) + 1):
            if j < len(chunks):
                steps += up(wg_v, j) + up(wu_v, j)
            if j > 0:
                steps += [functools.partial(down, j - 1, c) for c in range(NT)]
        return steps, y

    def routed_gates(sel, y):
        row = lax.broadcasted_iota(I32, (16, D), 0)
        ys = [y[i:i + 1, :] * jax.nn.sigmoid(rv) for i, (_, rv) in enumerate(sel)]
        gates = []
        for idx, _ in sel:
            upd = jnp.zeros((16, D), F32)
            for (other, _), yo in zip(sel, ys):
                upd = jnp.where(row == other - group(idx), yo, upd)
            gates.append(_silu(normed(idx) + upd))
        return gates

    def run(dots, attn=(), ln=()):
        tasks = []
        for kind, jobs, step in (("a", attn, RA), ("l", ln, RL)):
            for k, job in enumerate(jobs):
                lo, hi = job[-1]
                tasks += [(lo + (hi - lo) * r / T, kind, k, r) for r in range(0, T, step)]
        tasks.sort()
        done = {"a": [], "l": []}
        pos = 0
        for j in range(-1, len(dots)):
            y = [step() for step in dots[j][2]][-1] if j >= 0 else None
            while pos < len(tasks):
                u, kind, k, off = tasks[pos]
                t = int(u * (dots[-1][0] + dots[-1][1])) - CFG["lat"] if dots else 0
                if j + 1 < len(dots) and t >= dots[j + 1][0]:
                    break
                pos += 1
                lag = CFG["lag" + kind]
                bits = done[kind][-lag] if dots and len(done[kind]) >= lag else None
                if y is not None:
                    g = min(t - dots[j][0], dots[j][1] - 8) // 8
                    mine = pltpu.bitcast(y[8 * g:8 * g + 8], U32)
                    bits = mine if bits is None else bits | mine
                gate = None if bits is None else (bits >> 31) >> 1
                if kind == "a":
                    qkv, o, first, start, _ = attn[k]
                    done[kind].append(attn_rows(qkv, o, first + off, start, gate))
                else:
                    x, xn, first, blk, _ = ln[k]
                    if off == 0:
                        scores = jnp.zeros((8, 128), F32)
                    scores = ln_rows(x, xn, first + off, off // 8, scores, gate)
                    done[kind].append(pltpu.bitcast(scores, U32))
                    if off == T - RL:
                        r_v[blk] = scores

    scope = [None]

    def mark(name):
        if not CFG.get("marks"):
            return
        if scope[0] is not None:
            scope[0].__exit__(None, None, None)
            scope[0] = None
        if name:
            scope[0] = jax.named_scope(name)
            scope[0].__enter__()

    mark("m00_start")
    for c in (cr, cx0, cka, ckb, cv, cq, cx1, *cwo, cx2, cx3, cg, cu, cd):
        c.start()
    cr.wait()
    cx0.wait()
    mark("m01_ln0")
    wr_v[...] = jnp.broadcast_to(wr1_v[...].astype(F32).reshape(1, D), (RL, D))
    run([], ln=[(x_v, xn_v, 0, 0, (0, 0))])
    mark("m02_prepka")
    cka.wait()
    prep_qkv(1, 0, KS)
    mark("m03_prepkb")
    ckb.wait()
    prep_qkv(1, KS, NT)
    h = T // 2
    run(_timed(proj(xn_v, qkv_v, 0, h, (1,)), h))
    mark("m04_kb")
    cv.wait()
    prep_qkv(2, 0, NT)
    run(_timed(proj(xn_v, qkv_v, h, h, (1,)) + proj(xn_v, qkv_v, 0, h, (2,)), h))
    mark("m06_vb")
    cq.wait()
    run(_timed(proj(xn_v, qkv_v, h, h, (2,)), h))
    prep_qkv(0, 0, NT)
    mark("m07_q")
    cx1.wait()
    run(_timed(proj(xn_v, qkv_v, 0, T, (0,)), T), ln=[(x_v, xn_v, T, 1, (0.0, 0.6))])
    mark("m08_wo")
    for c in cwo:
        c.wait()
    prep_wo()
    cx2.wait()
    mark("m11_loop")

    U = CFG["U"]

    def main(i, carry):
        base = i * (U * T)
        qkv = qkv_v.at[:, _ds(base, HALO + (U + 1) * T), :]
        xn = xn_v.at[_ds(i * (U * T // 2), (U + 2) * T // 2), :]
        o = o_v.at[_ds(i * (U * T // 2), U * T // 2), :]
        x = x_v.at[_ds(base, (U + 2) * T, 16), :]
        s, out = [ref.at[_ds(base, U * T, 16), :] for ref in (s_v, out_v)]
        dots, attn, ln = [], [], []
        for k in range(U):
            dots += proj(xn, qkv, (k + 1) * T, T) + out_rows(o, xn, x, s, out, k * T, T)
            attn.append((qkv, o, k * T, base, [(k + f) / U for f in CFG["aspan"]]))
            ln.append((x, xn, (k + 2) * T, i * U + k + 2, [(k + f) / U for f in CFG["lspan"]]))
        run(_timed(dots, T), attn, ln)
        out_copy(i, base, U * T).start()

        pl.when(i == 0)(cx3.wait)

        return carry

    lax.fori_loop(0, (NB - 2) // U, main, 0)

    mark("m12_ffn")
    cg.wait()
    cu.wait()
    cd.wait()
    sel = route()
    steps, routed = ffn()
    last = S - T
    M = CFG["M"]
    mixed = [f for r in range(last, S, M) for f in proj(xn_v, qkv_v, r, M)]
    mixed += [f for r in range(last - T, S, M) for f in out_rows(o_v, xn_v, x_v, s_v, out_v, r, M)]
    skip = CFG["skip"]
    dots = _timed(mixed, M, lambda j: steps[4 * (j - skip):4 * (j - skip + 1)] if j >= skip else [])
    dots[-CFG["send"]][2].insert(0, out_copy(NB - 2, last - T, 2 * T - M).start)
    run(dots, [(qkv_v, o_v, last - T, None, CFG["e1"]), (qkv_v, o_v, last, None, CFG["e2"])])

    for i, ((idx, _), g) in enumerate(zip(sel, routed_gates(sel, jnp.concatenate(routed, axis=1)))):
        rows = pl.ds(group(idx), 16)
        fix_v[i] = (x_v[rows, :].astype(F32) + s_v[rows, :] * g).astype(BF16)
    mark("m16_tail")
    out_copy(NB - 1, S - M, M).start()
    tiles = [group(idx) for idx, _ in sel]
    wanted = [True, tiles[1] != tiles[0]]
    fixes = [pltpu.make_async_copy(fix_v.at[i], out_hbm.at[pl.ds(g, 16), :], sem_fix.at[i])
             for i, g in enumerate(tiles)]
    for i in range((NB - 2) // U):
        out_copy(i, i * U * T, U * T).wait()
    for lo, hi, sent in ((0, last - T, None), (last - T, S - M, out_copy(NB - 2, last - T, 2 * T - M)),
                         (S - M, S, out_copy(NB - 1, S - M, M))):
        if sent is not None:
            sent.wait()
        for fix, g, want in zip(fixes, tiles, wanted):
            pl.when((g >= lo) & (g < hi) & want)(fix.start)
    fixes[0].wait()
    pl.when(wanted[1])(fixes[1].wait)
    mark(None)


@jax.jit
def pallas_recurrent_scan__sliding_local_dilated__moe_arch_mod__prompt_kernel(A_x, A_wqkv, A_wo, B_x, B_w_r, B_w_gate, B_w_up, B_w_down):
    del B_x
    hbm = pl.BlockSpec(memory_space=pltpu.HBM)
    out = pl.pallas_call(
        _kernel,
        out_shape=jax.ShapeDtypeStruct((S, D), BF16),
        in_specs=[hbm] * 7,
        out_specs=hbm,
        scratch_shapes=[
            pltpu.VMEM((S, D), BF16),
            pltpu.VMEM((3, D, D), BF16),
            pltpu.VMEM((NT, D, 128), BF16),
            pltpu.VMEM((F, D), BF16),
            pltpu.VMEM((F, D), BF16),
            pltpu.VMEM((F, D), BF16),
            pltpu.VMEM((3, NT, D // 2, 128), U32),
            pltpu.VMEM((3, D // 2, D), U32),
            pltpu.VMEM((D // 2, D), U32),
            pltpu.VMEM((S // 2, D), U32),
            pltpu.VMEM((3 * NT + 1, HALO + S, 128), F32),
            pltpu.VMEM((S // 2, D), U32),
            pltpu.VMEM((S, D), F32),
            pltpu.VMEM((S, D), BF16),
            pltpu.VMEM((RL, D), F32),
            pltpu.VMEM((NB, 8, 128), F32),
            pltpu.VMEM((16, D), BF16),
            pltpu.VMEM((2, 16, D), BF16),
            pltpu.VMEM((D,), BF16),
            pltpu.SemaphoreType.DMA((17,)),
            pltpu.SemaphoreType.DMA((NB,)),
            pltpu.SemaphoreType.DMA((2,)),
        ],
        compiler_params=pltpu.CompilerParams(vmem_limit_bytes=100 * 2 ** 20, flags=CFG['flags']),
        name="fused",
    )(A_x.reshape(S, D), A_wqkv, A_wo, B_w_r, B_w_gate.T, B_w_up.T, B_w_down)
    return out.reshape(1, S, D)
```

```python
import functools
import math

import jax
import jax.numpy as jnp
import numpy as np
from jax import lax
from jax.experimental import pallas as pl
from jax.experimental.pallas import tpu as pltpu

F32, BF16, U32, I32 = jnp.float32, jnp.bfloat16, jnp.uint32, jnp.int32

S, D, H, DH, F = 2048, 640, 32, 20, 1728
W, DIL = 8, 2
NT = D // 128
TILES = [slice(c * 128, (c + 1) * 128) for c in range(NT)]
HALO = 16
T = 256
NB = S // T
RA, RL = 8, 16
LOG2E = math.log2(math.e)
EPS_BF16 = float(np.asarray(1e-5, dtype=jnp.bfloat16).astype(np.float32))

CFG = dict(flags=None, lat=100, laga=4, lagl=5, aspan=(0.0, 0.5), lspan=(0.55, 0.8), M=128, quota=(0, 0.5, 1, 1, 1, 1, 1, 1, 1, 0.4), cut=3, e1=(0.0, 0.4), e2=(0.4, 0.86), ksplit=3, U=2, h=128, fc=5, skip=9, split=True, nlong=1,
           last=(256,), marks=False)

NN_DIMS = (((1,), (0,)), ((), ()))
NT_DIMS = (((1,), (1,)), ((), ()))


def _rb(v):
    return v.astype(BF16).astype(F32)


def _ds(r0, n, align=8):
    return pl.ds(r0 if isinstance(r0, int) else pl.multiple_of(r0, align), n)


def _regroup(src, dst, cols):
    for j in range(DH // 2):
        for g in range(2):
            a = src[pl.ds(g * 160 + j, 8, stride=DH), :]
            b = src[pl.ds(g * 160 + DH // 2 + j, 8, stride=DH), :]
            row = j * H + 8 * g
            dst[row:row + 8, cols] = (a & jnp.uint32(0xFFFF)) | (b << 16)
            dst[row + H // 2:row + H // 2 + 8, cols] = (a >> 16) | (b & jnp.uint32(0xFFFF0000))


def _const(val, gate, rows):
    if gate is None:
        return val
    c = pltpu.bitcast(gate | np.float32(val).view(np.uint32), F32)
    return jnp.concatenate([c] * (rows // 8), axis=0)


def _layernorm(x, gate):
    tot = x[:, :128] if gate is None else x[:, :128] + _const(0.0, gate, x.shape[0])
    for c in range(1, NT):
        tot = tot + x[:, c * 128:(c + 1) * 128]
    mean = jnp.sum(tot, axis=-1, keepdims=True) * (1.0 / D)
    xc = x - mean
    var = jnp.sum(xc * xc, axis=-1, keepdims=True) * (1.0 / D)
    sd = _rb(jnp.sqrt(_rb(_rb(var) + EPS_BF16)))
    return (_rb(x - _rb(mean)) * (1.0 / sd)).astype(BF16)


def _silu(z):
    h = 0.5 * z
    return h * jnp.tanh(h) + h


def _tiles(lhs, rhs, dims, finish):
    acc = []

    def step(k, parts=1):
        a, b = lhs(TILES[k]), rhs(TILES[k])
        n = a.shape[0] // parts
        y = jnp.concatenate([lax.dot_general(a[i * n:(i + 1) * n], b, dims, preferred_element_type=F32)
                             for i in range(parts)], axis=0)
        acc.append(y if k == 0 else acc.pop() + y)
        if k == NT - 1:
            finish(acc.pop())
        return y

    return [functools.partial(step, k) for k in range(NT)]


def _timed(steps, rows, extra=None):
    left = len(steps) % 4
    if left in (1, 2) and CFG["split"]:
        steps = steps[:-left] + [functools.partial(step, parts=4 // left) for step in steps[-left:]]
    groups, t = [], 0
    for j in range(0, len(steps), 4):
        short = extra(j // 4) if extra else []
        t += CFG["fc"] * len(short)
        groups.append((t, rows, short + steps[j:j + 4]))
        t += rows
    return groups


def _kernel(x_hbm, wqkv_hbm, wo_hbm, wr_hbm, wg_hbm, wu_hbm, wd_hbm, out_hbm,
            x_v, wqkv_v, wo_v, wg_v, wu_v, wd_v, tmp_v, wp_v, wop_v,
            xn_v, qkv_v, o_v, s_v, out_v, wr_v, r_v, xs_v, fix_v, wr1_v, sem_in, sem_out, sem_fix):
    KS = CFG["ksplit"]
    sems = iter(range(sem_in.shape[0]))

    def copy_in(src, dst):
        return pltpu.make_async_copy(src, dst, sem_in.at[next(sems)])

    def x_copy(lo, hi):
        return copy_in(x_hbm.at[lo:hi, :], x_v.at[lo:hi, :])

    def w_copy(m, lo, hi):
        return copy_in(wqkv_hbm.at[lo * 128:hi * 128, m * D:(m + 1) * D], wqkv_v.at[m, lo * 128:hi * 128, :])

    cr = copy_in(wr_hbm, wr1_v)
    cx0, cx1, cx2, cx3 = x_copy(0, T), x_copy(T, 2 * T), x_copy(2 * T, (2 + CFG['U']) * T), x_copy((2 + CFG['U']) * T, S)
    cka, ckb, cv, cq = w_copy(1, 0, KS), w_copy(1, KS, NT), w_copy(2, 0, NT), w_copy(0, 0, NT)
    cwo = [copy_in(wo_hbm.at[:, c * 128:(c + 1) * 128], wo_v.at[c]) for c in range(NT)]
    cg, cu, cd = copy_in(wg_hbm, wg_v), copy_in(wu_hbm, wu_v), copy_in(wd_hbm, wd_v)

    def out_copy(i, r0, n):
        return pltpu.make_async_copy(out_v.at[_ds(r0, n, 16), :], out_hbm.at[_ds(r0, n, 16), :], sem_out.at[i])

    lane = lax.broadcasted_iota(I32, (8, 128), 1)
    sub = lax.broadcasted_iota(I32, (8, 128), 0)

    def prep_qkv(m, lo, hi):
        for c in range(lo, hi):
            tmp_v[m, c] = pltpu.bitcast(wqkv_v[m, c * 128:(c + 1) * 128, :].T, U32)
        for c in range(lo, hi):
            _regroup(tmp_v.at[m, c], wp_v.at[m], slice(c * 128, (c + 1) * 128))

    def prep_wo():
        for c in range(NT):
            _regroup(wo_v.bitcast(U32).at[c], wop_v, slice(c * 128, (c + 1) * 128))

    def ln_rows(x, xn_out, row, slot, scores, gate):
        xn = _layernorm(x[row:row + RL, :].astype(F32), gate)
        xn_out[row // 2:(row + RL) // 2, :] = pltpu.bitcast(xn, U32)
        r = jnp.sum(xn.astype(F32) * wr_v[...], axis=-1, keepdims=True)
        for i in range(RL // 8):
            scores = jnp.where(lane == slot + i, jnp.broadcast_to(r[8 * i:8 * i + 8], (8, 128)), scores)
        return scores

    def proj(xn, qkv, r0, n, mats=(1, 2, 0)):
        def finish(m, c, y):
            qkv[m * NT + c, HALO + r0:HALO + r0 + n, :] = y
            if m > 0 and r0 == 0:
                qkv[m * NT + c, 0:HALO, :] = jnp.broadcast_to(y[0:1], (HALO, 128))

        return [step for m in mats for c in range(NT) for step in _tiles(
            lambda k: pltpu.bitcast(xn[r0 // 2:(r0 + n) // 2, k], BF16),
            lambda k, m=m, c=c: pltpu.bitcast(wp_v[m, c * 64:(c + 1) * 64, k], BF16),
            NT_DIMS, functools.partial(finish, m, c))]

    held = {}

    def attn_rows(qkv, o, off, start, gate):
        scale = _const(DH ** -0.5 * LOG2E, gate, RA)
        q = [qkv[c, HALO + off:HALO + off + RA, :] * scale for c in range(NT)]
        lg = []
        for w in range(W):
            lo = HALO + off - DIL * w
            p = q[0] * qkv[NT, lo:lo + RA, :]
            for c in range(1, NT):
                p = p + q[c] * qkv[NT + c, lo:lo + RA, :]
            p = p + pltpu.roll(p, 64, 1)
            p = p + pltpu.roll(p, 32, 1)
            if start is not None and off < DIL * w:
                p = jnp.where(sub >= DIL * w - off - start, p, -1e9 * LOG2E)
            lg.append(p)
        mx = lg[0]
        for w in range(1, W):
            mx = jnp.maximum(mx, lg[w])
        e = [jnp.exp2(l - mx) for l in lg]
        den = e[0]
        for w in range(1, W):
            den = den + e[w]
        inv = pl.reciprocal(den, full_range=False)
        fin = None
        for c in range(NT):
            acc = e[0] * qkv[2 * NT + c, HALO + off:HALO + off + RA, :]
            for w in range(1, W):
                lo = HALO + off - DIL * w
                acc = acc + e[w] * qkv[2 * NT + c, lo:lo + RA, :]
            res = acc * inv
            bits = pltpu.bitcast(res, U32)
            fin = bits if fin is None else fin | bits
            if off % 16 == 0:
                held[c] = res
            else:
                pair = jnp.concatenate([held.pop(c), res], axis=0).astype(BF16)
                o[off // 2 - 4:off // 2 + 4, c * 128:(c + 1) * 128] = pltpu.bitcast(pair, U32)
        return fin

    def out_rows(o, xn, x, s, out, r0, n):
        def finish(cols, y):
            s[r0:r0 + n, cols] = y
            g = _silu(pltpu.bitcast(xn[r0 // 2:(r0 + n) // 2, cols], BF16).astype(F32))
            out[r0:r0 + n, cols] = (x[r0:r0 + n, cols].astype(F32) + y * g).astype(BF16)

        return [step for cols in TILES for step in _tiles(
            lambda k: pltpu.bitcast(o[r0 // 2:(r0 + n) // 2, k], BF16),
            lambda k, cols=cols: pltpu.bitcast(wop_v[k.start // 2:k.stop // 2, cols], BF16),
            NN_DIMS, functools.partial(finish, cols))]

    def group(idx):
        return pl.multiple_of((idx >> 4) << 4, 16)

    def normed(idx):
        return pltpu.bitcast(xn_v[_ds((idx >> 4) << 3, 8), :], BF16).astype(F32)

    def route():
        imin = jnp.int32(-2 ** 31)
        r = r_v[0]
        for b in range(1, NB):
            if b % 4 == 0:
                first, r = r, r_v[b]
            else:
                r = jnp.where(lane >= b % 4 * 32, pltpu.roll(r_v[b], b % 4 * 32, 1), r)
        comb, vals = [], []
        for i, r in enumerate((first, r)):
            r = _rb(r) + 0.0
            bits = pltpu.bitcast(r, I32)
            key = jnp.where(bits < 0, bits ^ jnp.int32(0x7FFFFFFF), bits) >> 16
            key = jnp.where(r != r, jnp.int32(-2 ** 15), key)
            comb.append(key * S + (S - 1 - i * 1024 - lane * 8 - sub))
            vals.append(r)
        row = lax.broadcasted_iota(I32, (16, D), 0)
        xs = jnp.zeros((16, D), F32)
        sel = []
        for i in range(2):
            best = jnp.max(jnp.maximum(comb[0], comb[1]))
            rv = jnp.where(comb[0] == best, vals[0], jnp.where(comb[1] == best, vals[1], 0.0))
            comb = [jnp.where(cmb == best, imin, cmb) for cmb in comb]
            idx = (S - 1) - (best & (S - 1))
            one = jnp.sum(jnp.where(row == (idx & 15), normed(idx), 0.0), axis=0, keepdims=True)
            xs = jnp.where(row == i, one, xs)
            sel.append((idx, jnp.sum(rv, keepdims=True)))
        xs_v[...] = xs.astype(BF16)
        return sel

    def ffn():
        chunks = [slice(lo, min(lo + 128, F)) for lo in range(0, F, 128)]
        pre, hid, y = {}, {}, [0.0] * NT

        def up(w, j):
            return _tiles(lambda k: xs_v[:, k], lambda k: w[chunks[j], k], NT_DIMS, pre.setdefault(j, []).append)

        def down(j, c):
            if c == 0:
                g, u = pre[j]
                hid[j] = (g * jax.nn.sigmoid(g) * u).astype(BF16)
            y[c] = y[c] + jnp.dot(hid[j], wd_v[chunks[j], TILES[c]], preferred_element_type=F32)

        steps = []
        for j in range(len(chunks) + 1):
            if j < len(chunks):
                steps += up(wg_v, j) + up(wu_v, j)
            if j > 0:
                steps += [functools.partial(down, j - 1, c) for c in range(NT)]
        return steps, y

    def routed_gates(sel, y):
        row = lax.broadcasted_iota(I32, (16, D), 0)
        ys = [y[i:i + 1, :] * jax.nn.sigmoid(rv) for i, (_, rv) in enumerate(sel)]
        gates = []
        for idx, _ in sel:
            upd = jnp.zeros((16, D), F32)
            for (other, _), yo in zip(sel, ys):
                upd = jnp.where(row == other - group(idx), yo, upd)
            gates.append(_silu(normed(idx) + upd))
        return gates

    def run(dots, attn=(), ln=()):
        tasks = []
        for kind, jobs, step in (("a", attn, RA), ("l", ln, RL)):
            for k, job in enumerate(jobs):
                lo, hi = job[-1]
                tasks += [(lo + (hi - lo) * r / T, kind, k, r) for r in range(0, T, step)]
        tasks.sort()
        done = {"a": [], "l": []}
        pos = 0
        for j in range(-1, len(dots)):
            y = [v for v in [step() for step in dots[j][2]] if v is not None][-1] if j >= 0 else None
            while pos < len(tasks):
                u, kind, k, off = tasks[pos]
                t = int(u * (dots[-1][0] + dots[-1][1])) - CFG["lat"] if dots else 0
                if j + 1 < len(dots) and t >= dots[j + 1][0]:
                    break
                pos += 1
                lag = CFG["lag" + kind]
                bits = done[kind][-lag] if dots and len(done[kind]) >= lag else None
                if y is not None:
                    g = min(t - dots[j][0], dots[j][1] - 8) // 8
                    mine = pltpu.bitcast(y[8 * g:8 * g + 8], U32)
                    bits = mine if bits is None else bits | mine
                gate = None if bits is None else (bits >> 31) >> 1
                if kind == "a":
                    qkv, o, first, start, _ = attn[k]
                    done[kind].append(attn_rows(qkv, o, first + off, start, gate))
                else:
                    x, xn, first, blk, _ = ln[k]
                    if off == 0:
                        scores = jnp.zeros((8, 128), F32)
                    scores = ln_rows(x, xn, first + off, off // 8, scores, gate)
                    done[kind].append(pltpu.bitcast(scores, U32))
                    if off == T - RL:
                        r_v[blk] = scores

    scope = [None]

    def mark(name):
        if not CFG.get("marks"):
            return
        if scope[0] is not None:
            scope[0].__exit__(None, None, None)
            scope[0] = None
        if name:
            scope[0] = jax.named_scope(name)
            scope[0].__enter__()

    mark("m00_start")
    for c in (cr, cx0, cka, ckb, cv, cq, cx1, *cwo, cx2, cx3, cg, cu, cd):
        c.start()
    cr.wait()
    cx0.wait()
    mark("m01_ln0")
    wr_v[...] = jnp.broadcast_to(wr1_v[...].astype(F32).reshape(1, D), (RL, D))
    run([], ln=[(x_v, xn_v, 0, 0, (0, 0))])
    mark("m02_prepka")
    cka.wait()
    prep_qkv(1, 0, KS)
    mark("m03_prepkb")
    ckb.wait()
    prep_qkv(1, KS, NT)
    h = T // 2
    run(_timed(proj(xn_v, qkv_v, 0, h, (1,)), h))
    mark("m04_kb")
    cv.wait()
    prep_qkv(2, 0, NT)
    run(_timed(proj(xn_v, qkv_v, h, h, (1,)) + proj(xn_v, qkv_v, 0, h, (2,)), h))
    mark("m06_vb")
    cq.wait()
    run(_timed(proj(xn_v, qkv_v, h, h, (2,)), h))
    prep_qkv(0, 0, NT)
    mark("m07_q")
    cx1.wait()
    run(_timed(proj(xn_v, qkv_v, 0, T, (0,)), T), ln=[(x_v, xn_v, T, 1, (0.0, 0.6))])
    mark("m08_wo")
    for c in cwo:
        c.wait()
    prep_wo()
    cx2.wait()
    mark("m11_loop")

    U = CFG["U"]

    def main(i, carry):
        base = i * (U * T)
        qkv = qkv_v.at[:, _ds(base, HALO + (U + 1) * T), :]
        xn = xn_v.at[_ds(i * (U * T // 2), (U + 2) * T // 2), :]
        o = o_v.at[_ds(i * (U * T // 2), U * T // 2), :]
        x = x_v.at[_ds(base, (U + 2) * T, 16), :]
        s, out = [ref.at[_ds(base, U * T, 16), :] for ref in (s_v, out_v)]
        dots, attn, ln = [], [], []
        for k in range(U):
            dots += proj(xn, qkv, (k + 1) * T, T) + out_rows(o, xn, x, s, out, k * T, T)
            attn.append((qkv, o, k * T, base, [(k + f) / U for f in CFG["aspan"]]))
            ln.append((x, xn, (k + 2) * T, i * U + k + 2, [(k + f) / U for f in CFG["lspan"]]))
        run(_timed(dots, T), attn, ln)
        out_copy(i, base, U * T).start()

        pl.when(i == 0)(cx3.wait)

        return carry

    lax.fori_loop(0, (NB - 2) // U, main, 0)

    mark("m12_ffn")
    cg.wait()
    cu.wait()
    cd.wait()
    sel = route()
    steps, routed = ffn()
    last = S - T
    M = CFG["M"]
    mixed = [f for r in range(last, S, M) for f in proj(xn_v, qkv_v, r, M)]
    cut = CFG["cut"] * 128
    sends = [(last - T, last, out_copy(NB - 2, last - T, T)), (last, S - M, out_copy(NB - 1, last, T - M))]
    ends = [pltpu.make_async_copy(out_v.at[S - M:, cols], out_hbm.at[S - M:, cols], sem_out.at[NB + i])
            for i, cols in enumerate((slice(0, cut), slice(cut, D)))]
    ready = {}
    for r in range(last - T, S, M):
        mixed += out_rows(o_v, xn_v, x_v, s_v, out_v, r, M)
        ready[r + M] = len(mixed)
    skip = CFG["skip"]
    dots = _timed(mixed, M, lambda j: steps[4 * (j - skip):4 * (j - skip + 1)] if j >= skip else [])
    for _, hi, c in sends:
        dots[ready[hi] // 4 + 2][2].append(c.start)
    dots[-1][2].append(ends[0].start)
    run(dots, [(qkv_v, o_v, last - T, None, CFG["e1"]), (qkv_v, o_v, last, None, CFG["e2"])])

    for i, ((idx, _), g) in enumerate(zip(sel, routed_gates(sel, jnp.concatenate(routed, axis=1)))):
        rows = pl.ds(group(idx), 16)
        fix_v[i] = (x_v[rows, :].astype(F32) + s_v[rows, :] * g).astype(BF16)
    mark("m16_tail")
    ends[1].start()
    tiles = [group(idx) for idx, _ in sel]
    wanted = [True, tiles[1] != tiles[0]]
    fixes = [pltpu.make_async_copy(fix_v.at[i], out_hbm.at[pl.ds(g, 16), :], sem_fix.at[i])
             for i, g in enumerate(tiles)]
    stages = [(0, last - T, [out_copy(i, i * U * T, U * T) for i in range((NB - 2) // U)])]
    stages += [(lo, hi, [c]) for lo, hi, c in sends] + [(S - M, S, ends)]
    for lo, hi, copies in stages:
        for c in copies:
            c.wait()
        for fix, g, want in zip(fixes, tiles, wanted):
            pl.when((g >= lo) & (g < hi) & want)(fix.start)
    fixes[0].wait()
    pl.when(wanted[1])(fixes[1].wait)
    mark(None)


@jax.jit
def pallas_recurrent_scan__sliding_local_dilated__moe_arch_mod__prompt_kernel(A_x, A_wqkv, A_wo, B_x, B_w_r, B_w_gate, B_w_up, B_w_down):
    del B_x
    hbm = pl.BlockSpec(memory_space=pltpu.HBM)
    out = pl.pallas_call(
        _kernel,
        out_shape=jax.ShapeDtypeStruct((S, D), BF16),
        in_specs=[hbm] * 7,
        out_specs=hbm,
        scratch_shapes=[
            pltpu.VMEM((S, D), BF16),
            pltpu.VMEM((3, D, D), BF16),
            pltpu.VMEM((NT, D, 128), BF16),
            pltpu.VMEM((F, D), BF16),
            pltpu.VMEM((F, D), BF16),
            pltpu.VMEM((F, D), BF16),
            pltpu.VMEM((3, NT, D // 2, 128), U32),
            pltpu.VMEM((3, D // 2, D), U32),
            pltpu.VMEM((D // 2, D), U32),
            pltpu.VMEM((S // 2, D), U32),
            pltpu.VMEM((3 * NT + 1, HALO + S, 128), F32),
            pltpu.VMEM((S // 2, D), U32),
            pltpu.VMEM((S, D), F32),
            pltpu.VMEM((S, D), BF16),
            pltpu.VMEM((RL, D), F32),
            pltpu.VMEM((NB, 8, 128), F32),
            pltpu.VMEM((16, D), BF16),
            pltpu.VMEM((2, 16, D), BF16),
            pltpu.VMEM((D,), BF16),
            pltpu.SemaphoreType.DMA((17,)),
            pltpu.SemaphoreType.DMA((NB + 2,)),
            pltpu.SemaphoreType.DMA((2,)),
        ],
        compiler_params=pltpu.CompilerParams(vmem_limit_bytes=100 * 2 ** 20, flags=CFG['flags']),
        name="fused",
    )(A_x.reshape(S, D), A_wqkv, A_wo, B_w_r, B_w_gate.T, B_w_up.T, B_w_down)
    return out.reshape(1, S, D)
```

```python
import functools
import math

import jax
import jax.numpy as jnp
import numpy as np
from jax import lax
from jax.experimental import pallas as pl
from jax.experimental.pallas import tpu as pltpu

F32, BF16, U32, I32 = jnp.float32, jnp.bfloat16, jnp.uint32, jnp.int32

S, D, H, DH, F = 2048, 640, 32, 20, 1728
W, DIL = 8, 2
NT = D // 128
TILES = [slice(c * 128, (c + 1) * 128) for c in range(NT)]
HALO = 16
T = 256
M = T // 2
NB = S // T
U = 2
RA, RL = 8, 16
LOG2E = math.log2(math.e)
EPS_BF16 = float(np.asarray(1e-5, dtype=jnp.bfloat16).astype(np.float32))

MXU_LATENCY = 100
IN_FLIGHT = {"attn": 4, "ln": 5}
ATTN_SPAN, LN_SPAN = (0.0, 0.5), (0.52, 0.86)

NN_DIMS = (((1,), (0,)), ((), ()))
NT_DIMS = (((1,), (1,)), ((), ()))


def _bf16_round(v):
    return v.astype(BF16).astype(F32)


def _regroup(src, dst, cols):
    for j in range(DH // 2):
        for g in range(2):
            even = src[pl.ds(g * 160 + j, 8, stride=DH), :]
            odd = src[pl.ds(g * 160 + DH // 2 + j, 8, stride=DH), :]
            row = j * H + 8 * g
            dst[row:row + 8, cols] = (even & np.uint32(0xFFFF)) | (odd << 16)
            dst[row + H // 2:row + H // 2 + 8, cols] = (even >> 16) | (odd & np.uint32(0xFFFF0000))


def _const(val, gate, rows):
    if gate is None:
        return val
    c = pltpu.bitcast(gate | np.float32(val).view(np.uint32), F32)
    return jnp.concatenate([c] * (rows // 8), axis=0)


def _layernorm(x, gate):
    tot = x[:, TILES[0]] if gate is None else x[:, TILES[0]] + _const(0.0, gate, x.shape[0])
    for cols in TILES[1:]:
        tot = tot + x[:, cols]
    mean = jnp.sum(tot, axis=-1, keepdims=True) * (1.0 / D)
    xc = x - mean
    var = jnp.sum(xc * xc, axis=-1, keepdims=True) * (1.0 / D)
    sd = _bf16_round(jnp.sqrt(_bf16_round(_bf16_round(var) + EPS_BF16)))
    return (_bf16_round(x - _bf16_round(mean)) * (1.0 / sd)).astype(BF16)


def _silu(z):
    h = 0.5 * z
    return h * jnp.tanh(h) + h


def _tiles(lhs, rhs, dims, finish):
    acc = []

    def step(k, parts=1):
        a, b = lhs(TILES[k]), rhs(TILES[k])
        n = a.shape[0] // parts
        y = jnp.concatenate([lax.dot_general(a[i * n:(i + 1) * n], b, dims, preferred_element_type=F32)
                             for i in range(parts)], axis=0)
        acc.append(y if k == 0 else acc.pop() + y)
        if k == NT - 1:
            finish(acc.pop())
        return y

    return [functools.partial(step, k) for k in range(NT)]


def _rounds(steps, rows, extra=None):
    left = len(steps) % 4
    if left in (1, 2):
        steps = steps[:-left] + [functools.partial(step, parts=4 // left) for step in steps[-left:]]
    rounds, t = [], 0
    for j in range(0, len(steps), 4):
        short = extra(j // 4) if extra else []
        t += 5 * len(short)
        rounds.append((t, rows, short + steps[j:j + 4]))
        t += rows
    return rounds


def _kernel(x_hbm, wqkv_hbm, wo_hbm, wr_hbm, wg_hbm, wu_hbm, wd_hbm, out_hbm,
            x_v, wqkv_v, wo_v, wg_v, wu_v, wd_v, tmp_v, wp_v, wop_v,
            xn_v, qkv_v, o_v, s_v, out_v, wr_v, r_v, xs_v, fix_v, wr1_v, sem_in, sem_out, sem_fix):
    sems = iter(range(sem_in.shape[0]))

    def copy_in(src, dst):
        return pltpu.make_async_copy(src, dst, sem_in.at[next(sems)])

    def x_copy(lo, hi):
        return copy_in(x_hbm.at[lo:hi, :], x_v.at[lo:hi, :])

    def w_copy(m, lo, hi):
        return copy_in(wqkv_hbm.at[lo * 128:hi * 128, m * D:(m + 1) * D], wqkv_v.at[m, lo * 128:hi * 128, :])

    def out_copy(i, rows, cols=slice(None)):
        return pltpu.make_async_copy(out_v.at[rows, cols], out_hbm.at[rows, cols], sem_out.at[i])

    get_wr = copy_in(wr_hbm, wr1_v)
    get_x = [x_copy(0, T), x_copy(T, 2 * T), x_copy(2 * T, (U + 2) * T), x_copy((U + 2) * T, S)]
    get_wk = [w_copy(1, 0, 3), w_copy(1, 3, NT)]
    get_wv, get_wq = w_copy(2, 0, NT), w_copy(0, 0, NT)
    get_wo = [copy_in(wo_hbm.at[:, cols], wo_v.at[c, :D]) for c, cols in enumerate(TILES)]
    get_ffn = [copy_in(wg_hbm, wg_v), copy_in(wu_hbm, wu_v), copy_in(wd_hbm, wd_v)]

    lane = lax.broadcasted_iota(I32, (8, 128), 1)
    sub = lax.broadcasted_iota(I32, (8, 128), 0)

    def prep_qkv(m, lo, hi):
        for c in range(lo, hi):
            tmp_v[m, c, :D // 2] = pltpu.bitcast(wqkv_v[m, TILES[c], :].T, U32)
        for c in range(lo, hi):
            _regroup(tmp_v.at[m, c], wp_v.at[m], TILES[c])

    def ln_rows(x, xn_out, row, slot, scores, gate):
        xn = _layernorm(x[row:row + RL, :].astype(F32), gate)
        xn_out[row // 2:(row + RL) // 2, :] = pltpu.bitcast(xn, U32)
        r = jnp.sum(xn.astype(F32) * wr_v[...], axis=-1, keepdims=True)
        for i in range(RL // 8):
            scores = jnp.where(lane == slot + i, jnp.broadcast_to(r[8 * i:8 * i + 8], (8, 128)), scores)
        return scores

    def proj(xn, qkv, r0, n, mats=(1, 2, 0)):
        def finish(m, c, y):
            qkv[m * NT + c, HALO + r0:HALO + r0 + n, :] = y
            if m > 0 and r0 == 0:
                qkv[m * NT + c, 0:HALO, :] = jnp.broadcast_to(y[0:1], (HALO, 128))

        return [step for m in mats for c in range(NT) for step in _tiles(
            lambda k: pltpu.bitcast(xn[r0 // 2:(r0 + n) // 2, k], BF16),
            lambda k, m=m, c=c: pltpu.bitcast(wp_v[m, c * 64:(c + 1) * 64, k], BF16),
            NT_DIMS, functools.partial(finish, m, c))]

    held = {}

    def attn_rows(qkv, o, row, start, gate):
        def window(plane, w):
            return qkv[plane, pl.ds(HALO + row - DIL * w, RA), :]

        scale = _const(DH ** -0.5 * LOG2E, gate, RA)
        q = [window(c, 0) * scale for c in range(NT)]
        logits = []
        for w in range(W):
            p = q[0] * window(NT, w)
            for c in range(1, NT):
                p = p + q[c] * window(NT + c, w)
            p = p + pltpu.roll(p, 64, 1)
            p = p + pltpu.roll(p, 32, 1)
            if start is not None and row < DIL * w:
                p = jnp.where(sub >= DIL * w - row - start, p, -1e9 * LOG2E)
            logits.append(p)
        top = functools.reduce(jnp.maximum, logits)
        e = [jnp.exp2(p - top) for p in logits]
        inv = pl.reciprocal(functools.reduce(jnp.add, e), full_range=False)
        done = []
        for c in range(NT):
            acc = e[0] * window(2 * NT + c, 0)
            for w in range(1, W):
                acc = acc + e[w] * window(2 * NT + c, w)
            res = acc * inv
            done.append(pltpu.bitcast(res, U32))
            if row % 16 == 0:
                held[c] = res
            else:
                pair = jnp.concatenate([held.pop(c), res], axis=0).astype(BF16)
                o[row // 2 - 4:row // 2 + 4, TILES[c]] = pltpu.bitcast(pair, U32)
        return functools.reduce(jnp.bitwise_or, done)

    def out_rows(o, xn, x, s, out, r0, n):
        def finish(cols, y):
            s[r0:r0 + n, cols] = y
            g = _silu(pltpu.bitcast(xn[r0 // 2:(r0 + n) // 2, cols], BF16).astype(F32))
            out[r0:r0 + n, cols] = (x[r0:r0 + n, cols].astype(F32) + y * g).astype(BF16)

        return [step for cols in TILES for step in _tiles(
            lambda k: pltpu.bitcast(o[r0 // 2:(r0 + n) // 2, k], BF16),
            lambda k, cols=cols: pltpu.bitcast(wop_v[k.start // 2:k.stop // 2, cols], BF16),
            NN_DIMS, functools.partial(finish, cols))]

    def tile_of(idx):
        return pl.multiple_of((idx >> 4) << 4, 16)

    def normed_tile(idx):
        return pltpu.bitcast(xn_v[pl.ds(pl.multiple_of((idx >> 4) << 3, 8), 8), :], BF16).astype(F32)

    def route():
        keys, vals = [], []
        for half in range(NB // 4):
            r = r_v[4 * half]
            for b in range(1, 4):
                r = jnp.where(lane >= 32 * b, pltpu.roll(r_v[4 * half + b], 32 * b, 1), r)
            r = _bf16_round(r) + 0.0
            bits = pltpu.bitcast(r, I32)
            rank = jnp.where(bits < 0, bits ^ np.int32(0x7FFFFFFF), bits) >> 16
            rank = jnp.where(r != r, np.int32(-2 ** 15), rank)
            keys.append(rank * S + (S - 1 - half * 1024 - lane * 8 - sub))
            vals.append(r)
        row = lax.broadcasted_iota(I32, (16, D), 0)
        xs = jnp.zeros((16, D), F32)
        sel = []
        for i in range(2):
            best = jnp.max(jnp.maximum(keys[0], keys[1]))
            score = jnp.where(keys[0] == best, vals[0], jnp.where(keys[1] == best, vals[1], 0.0))
            keys = [jnp.where(key == best, np.int32(-2 ** 31), key) for key in keys]
            idx = (S - 1) - (best & (S - 1))
            picked = jnp.sum(jnp.where(row == (idx & 15), normed_tile(idx), 0.0), axis=0, keepdims=True)
            xs = jnp.where(row == i, picked, xs)
            sel.append((idx, jnp.sum(score, keepdims=True)))
        xs_v[...] = xs.astype(BF16)
        return sel

    def ffn():
        chunks = [slice(lo, min(lo + 128, F)) for lo in range(0, F, 128)]
        pre, hid, y = {}, {}, [0.0] * NT

        def up(w, j):
            return _tiles(lambda k: xs_v[:, k], lambda k: w[chunks[j], k], NT_DIMS, pre.setdefault(j, []).append)

        def down(j, c):
            if c == 0:
                g, u = pre[j]
                hid[j] = (g * jax.nn.sigmoid(g) * u).astype(BF16)
            y[c] = y[c] + jnp.dot(hid[j], wd_v[chunks[j], TILES[c]], preferred_element_type=F32)

        steps = []
        for j in range(len(chunks) + 1):
            if j < len(chunks):
                steps += up(wg_v, j) + up(wu_v, j)
            if j > 0:
                steps += [functools.partial(down, j - 1, c) for c in range(NT)]
        return steps, y

    def run(rounds, attn=(), ln=()):
        tasks = []
        for kind, jobs, step in (("attn", attn, RA), ("ln", ln, RL)):
            for k, job in enumerate(jobs):
                lo, hi = job[-1]
                tasks += [(lo + (hi - lo) * r / T, kind, k, r) for r in range(0, T, step)]
        tasks.sort()
        done = {"attn": [], "ln": []}
        pos = 0
        for j in range(-1, len(rounds)):
            y = [v for v in [call() for call in rounds[j][2]] if v is not None][-1] if j >= 0 else None
            while pos < len(tasks):
                frac, kind, k, off = tasks[pos]
                t = int(frac * (rounds[-1][0] + rounds[-1][1])) - MXU_LATENCY if rounds else 0
                if j + 1 < len(rounds) and t >= rounds[j + 1][0]:
                    break
                pos += 1
                lag = IN_FLIGHT[kind]
                bits = done[kind][-lag] if rounds and len(done[kind]) >= lag else None
                if y is not None:
                    g = min(t - rounds[j][0], rounds[j][1] - 8) // 8
                    mine = pltpu.bitcast(y[8 * g:8 * g + 8], U32)
                    bits = mine if bits is None else bits | mine
                gate = None if bits is None else (bits >> 31) >> 1
                if kind == "attn":
                    qkv, o, first, start, _ = attn[k]
                    done[kind].append(attn_rows(qkv, o, first + off, start, gate))
                else:
                    x, xn, first, block, _ = ln[k]
                    if off == 0:
                        scores = jnp.zeros((8, 128), F32)
                    scores = ln_rows(x, xn, first + off, off // 8, scores, gate)
                    done[kind].append(pltpu.bitcast(scores, U32))
                    if off == T - RL:
                        r_v[block] = scores

    for c in (get_wr, get_x[0], *get_wk, get_wv, get_wq, get_x[1], *get_wo, get_x[2], get_x[3], *get_ffn):
        c.start()
    get_wr.wait()
    get_x[0].wait()
    wr_v[...] = jnp.broadcast_to(wr1_v[...].astype(F32).reshape(1, D), (RL, D))
    run([], ln=[(x_v, xn_v, 0, 0, (0.0, 0.0))])
    get_wk[0].wait()
    prep_qkv(1, 0, 3)
    get_wk[1].wait()
    prep_qkv(1, 3, NT)
    run(_rounds(proj(xn_v, qkv_v, 0, M, (1,)), M))
    get_wv.wait()
    prep_qkv(2, 0, NT)
    run(_rounds(proj(xn_v, qkv_v, M, M, (1,)) + proj(xn_v, qkv_v, 0, M, (2,)), M))
    get_wq.wait()
    run(_rounds(proj(xn_v, qkv_v, M, M, (2,)), M))
    prep_qkv(0, 0, NT)
    get_x[1].wait()
    run(_rounds(proj(xn_v, qkv_v, 0, T, (0,)), T), ln=[(x_v, xn_v, T, 1, (0.0, 0.6))])
    for c in get_wo:
        c.wait()
    for c in range(NT):
        _regroup(wo_v.bitcast(U32).at[c], wop_v, TILES[c])
    get_x[2].wait()

    def trip(i, carry):
        base = pl.multiple_of(i * (U * T), T)
        pairs = pl.multiple_of(i * (U * M), M)
        qkv = qkv_v.at[:, pl.ds(base, HALO + (U + 1) * T), :]
        xn = xn_v.at[pl.ds(pairs, (U + 2) * M), :]
        o = o_v.at[pl.ds(pairs, U * M), :]
        x = x_v.at[pl.ds(base, (U + 2) * T), :]
        s, out = [ref.at[pl.ds(base, U * T), :] for ref in (s_v, out_v)]
        steps, attn, ln = [], [], []
        for k in range(U):
            steps += proj(xn, qkv, (k + 1) * T, T) + out_rows(o, xn, x, s, out, k * T, T)
            attn.append((qkv, o, k * T, base, [(k + f) / U for f in ATTN_SPAN]))
            ln.append((x, xn, (k + 2) * T, i * U + k + 2, [(k + f) / U for f in LN_SPAN]))
        run(_rounds(steps, T), attn, ln)
        out_copy(i, pl.ds(base, U * T)).start()
        pl.when(i == 0)(get_x[3].wait)
        return carry

    trips = (NB - 2) // U
    lax.fori_loop(0, trips, trip, 0)

    for c in get_ffn:
        c.wait()
    sel = route()
    small, routed = ffn()
    last = S - T
    steps = [step for r in range(last, S, M) for step in proj(xn_v, qkv_v, r, M)]
    issued = {}
    for r in range(last - T, S, M):
        steps += out_rows(o_v, xn_v, x_v, s_v, out_v, r, M)
        issued[r + M] = len(steps)
    rounds = _rounds(steps, M, lambda j: small[4 * (j - 9):4 * (j - 8)] if j >= 9 else [])
    assert len(small) <= 4 * (len(rounds) - 9)
    stages = [(0, last - T, [out_copy(i, pl.ds(i * U * T, U * T)) for i in range(trips)])]
    for i, (lo, hi) in enumerate(((last - T, last), (last, S - M))):
        stages.append((lo, hi, [out_copy(trips + i, slice(lo, hi))]))
        rounds[issued[hi] // 4 + 2][2].append(stages[-1][2][0].start)
    left, right = [out_copy(trips + 2 + i, slice(S - M, S), cols)
                   for i, cols in enumerate((slice(0, 3 * 128), slice(3 * 128, D)))]
    stages.append((S - M, S, [left, right]))
    rounds[(len(steps) - 2 * NT) // 4 + 1][2].append(left.start)
    run(rounds, [(qkv_v, o_v, last - T, None, (0.0, 0.4)), (qkv_v, o_v, last, None, (0.4, 0.86))])

    y = jnp.concatenate(routed, axis=1)
    y = [y[i:i + 1, :] * jax.nn.sigmoid(score) for i, (_, score) in enumerate(sel)]
    row = lax.broadcasted_iota(I32, (16, D), 0)
    tiles = [tile_of(idx) for idx, _ in sel]
    for i, ((idx, _), tile) in enumerate(zip(sel, tiles)):
        upd = jnp.zeros((16, D), F32)
        for (other, _), y_other in zip(sel, y):
            upd = jnp.where(row == other - tile, y_other, upd)
        rows = pl.ds(tile, 16)
        fix_v[i] = (x_v[rows, :].astype(F32) + s_v[rows, :] * _silu(normed_tile(idx) + upd)).astype(BF16)
    right.start()

    fixes = [pltpu.make_async_copy(fix_v.at[i], out_hbm.at[pl.ds(tile, 16), :], sem_fix.at[i])
             for i, tile in enumerate(tiles)]
    distinct = tiles[1] != tiles[0]
    for lo, hi, copies in stages:
        for c in copies:
            c.wait()
        pl.when((tiles[0] >= lo) & (tiles[0] < hi))(fixes[0].start)
        pl.when((tiles[1] >= lo) & (tiles[1] < hi) & distinct)(fixes[1].start)
    fixes[0].wait()
    pl.when(distinct)(fixes[1].wait)


@jax.jit
def pallas_recurrent_scan__sliding_local_dilated__moe_arch_mod__prompt_kernel(
    A_x: jax.Array,
    A_wqkv: jax.Array,
    A_wo: jax.Array,
    B_x: jax.Array,
    B_w_r: jax.Array,
    B_w_gate: jax.Array,
    B_w_up: jax.Array,
    B_w_down: jax.Array,
):
    del B_x
    hbm = pl.BlockSpec(memory_space=pltpu.HBM)
    out = pl.pallas_call(
        _kernel,
        out_shape=jax.ShapeDtypeStruct((S, D), BF16),
        in_specs=[hbm] * 7,
        out_specs=hbm,
        scratch_shapes=[
            pltpu.VMEM((S, D), BF16),
            pltpu.VMEM((3, D, D), BF16),
            pltpu.VMEM((NT, D + 64, 128), BF16),
            pltpu.VMEM((F, D), BF16),
            pltpu.VMEM((F, D), BF16),
            pltpu.VMEM((F, D), BF16),
            pltpu.VMEM((3, NT, D // 2 + 32, 128), U32),
            pltpu.VMEM((3, D // 2, D), U32),
            pltpu.VMEM((D // 2, D), U32),
            pltpu.VMEM((S // 2, D), U32),
            pltpu.VMEM((3 * NT + 1, HALO + S, 128), F32),
            pltpu.VMEM((S // 2, D), U32),
            pltpu.VMEM((S, D), F32),
            pltpu.VMEM((S, D), BF16),
            pltpu.VMEM((RL, D), F32),
            pltpu.VMEM((NB, 8, 128), F32),
            pltpu.VMEM((16, D), BF16),
            pltpu.VMEM((2, 16, D), BF16),
            pltpu.VMEM((D,), BF16),
            pltpu.SemaphoreType.DMA((17,)),
            pltpu.SemaphoreType.DMA(((NB - 2) // U + 4,)),
            pltpu.SemaphoreType.DMA((2,)),
        ],
        compiler_params=pltpu.CompilerParams(vmem_limit_bytes=64 * 2 ** 20),
        name="fused",
    )(A_x.reshape(S, D), A_wqkv, A_wo, B_w_r, B_w_gate.T, B_w_up.T, B_w_down)
    return out.reshape(1, S, D)
```

```python
import functools
import math

import jax
import jax.numpy as jnp
import numpy as np
from jax import lax
from jax.experimental import pallas as pl
from jax.experimental.pallas import tpu as pltpu

F32, BF16, U32, I32 = jnp.float32, jnp.bfloat16, jnp.uint32, jnp.int32

S, D, H, DH, F = 2048, 640, 32, 20, 1728
W, DIL = 8, 2
NT = D // 128
TILES = [slice(c * 128, (c + 1) * 128) for c in range(NT)]
HALO = 16
T = 256
M = T // 2
NB = S // T
U = 2
RA, RL = 8, 16
LOG2E = math.log2(math.e)
EPS_BF16 = float(np.asarray(1e-5, dtype=jnp.bfloat16).astype(np.float32))

MXU_LATENCY = 100
IN_FLIGHT = {"attn": 4, "ln": 5}
ATTN_SPAN, LN_SPAN = (0.0, 0.5), (0.52, 0.86)

NN_DIMS = (((1,), (0,)), ((), ()))
NT_DIMS = (((1,), (1,)), ((), ()))


def _bf16_round(v):
    return v.astype(BF16).astype(F32)


def _regroup(src, dst, cols):
    for j in range(DH // 2):
        for g in range(2):
            even = src[pl.ds(g * 160 + j, 8, stride=DH), :]
            odd = src[pl.ds(g * 160 + DH // 2 + j, 8, stride=DH), :]
            row = j * H + 8 * g
            dst[row:row + 8, cols] = (even & np.uint32(0xFFFF)) | (odd << 16)
            dst[row + H // 2:row + H // 2 + 8, cols] = (even >> 16) | (odd & np.uint32(0xFFFF0000))


def _const(val, gate, rows):
    if gate is None:
        return val
    c = pltpu.bitcast(gate | np.float32(val).view(np.uint32), F32)
    return jnp.concatenate([c] * (rows // 8), axis=0)


def _layernorm(x, gate):
    tot = x[:, TILES[0]] if gate is None else x[:, TILES[0]] + _const(0.0, gate, x.shape[0])
    for cols in TILES[1:]:
        tot = tot + x[:, cols]
    mean = jnp.sum(tot, axis=-1, keepdims=True) * (1.0 / D)
    xc = x - mean
    var = jnp.sum(xc * xc, axis=-1, keepdims=True) * (1.0 / D)
    sd = _bf16_round(jnp.sqrt(_bf16_round(_bf16_round(var) + EPS_BF16)))
    return (_bf16_round(x - _bf16_round(mean)) * (1.0 / sd)).astype(BF16)


def _silu(z):
    h = 0.5 * z
    return h * jnp.tanh(h) + h


def _tiles(lhs, rhs, dims, finish, ks=range(NT)):
    acc = []

    def step(k, parts=1):
        a, b = lhs(TILES[k]), rhs(TILES[k])
        n = a.shape[0] // parts
        y = jnp.concatenate([lax.dot_general(a[i * n:(i + 1) * n], b, dims, preferred_element_type=F32)
                             for i in range(parts)], axis=0)
        acc.append(acc.pop() + y if acc else y)
        if k == ks[-1]:
            finish(acc.pop())
        return y

    return [functools.partial(step, k) for k in ks]


def _rounds(steps, rows, extra=None):
    left = len(steps) % 4
    if left in (1, 2):
        steps = steps[:-left] + [functools.partial(step, parts=4 // left) for step in steps[-left:]]
    rounds, t = [], 0
    for j in range(0, len(steps), 4):
        short = extra(j // 4) if extra else []
        t += 3 * len(short)
        rounds.append((t, rows, short + steps[j:j + 4]))
        t += rows
    return rounds


def _kernel(x_hbm, wqkv_hbm, wo_hbm, wr_hbm, wg_hbm, wu_hbm, wd_hbm, out_hbm,
            x_v, wqkv_v, wo_v, wg_v, wu_v, wd_v, tmp_v, wp_v, wop_v,
            xn_v, qkv_v, o_v, s_v, out_v, wr_v, r_v, xs_v, fix_v, wr1_v, sem_in, sem_out, sem_fix):
    sems = iter(range(sem_in.shape[0]))

    def copy_in(src, dst):
        return pltpu.make_async_copy(src, dst, sem_in.at[next(sems)])

    def x_copy(lo, hi):
        return copy_in(x_hbm.at[lo:hi, :], x_v.at[lo:hi, :])

    def out_copy(i, rows, cols=slice(None)):
        return pltpu.make_async_copy(out_v.at[rows, cols], out_hbm.at[rows, cols], sem_out.at[i])

    get_wr = copy_in(wr_hbm, wr1_v)
    get_x = [x_copy(0, T), x_copy(T, 2 * T), x_copy(2 * T, (U + 2) * T), x_copy((U + 2) * T, S)]
    get_w = [copy_in(wqkv_hbm.at[rows, :], wqkv_v.at[rows, :]) for rows in TILES]
    get_wo = copy_in(wo_hbm, wo_v)
    get_ffn = [copy_in(wg_hbm, wg_v), copy_in(wu_hbm, wu_v), copy_in(wd_hbm, wd_v)]

    lane = lax.broadcasted_iota(I32, (8, 128), 1)
    sub = lax.broadcasted_iota(I32, (8, 128), 0)

    written = dict(xn=0, qkv=0, o=0)

    def after(name, rows, value):
        assert rows <= written[name], name
        return value

    def prep_qkv(k):
        for m in range(3):
            tmp_v[m, k, :D // 2] = pltpu.bitcast(wqkv_v[TILES[k], m * D:(m + 1) * D].T, U32)
        for m in range(3):
            _regroup(tmp_v.at[m, k], wp_v.at[m], TILES[k])

    def ln_rows(x, xn_out, row, slot, scores, gate):
        xn = _layernorm(x[row:row + RL, :].astype(F32), gate)
        xn_out[row // 2:(row + RL) // 2, :] = pltpu.bitcast(xn, U32)
        written["xn"] = row + RL
        r = jnp.sum(xn.astype(F32) * wr_v[...], axis=-1, keepdims=True)
        for i in range(RL // 8):
            scores = jnp.where(lane == slot + i, jnp.broadcast_to(r[8 * i:8 * i + 8], (8, 128)), scores)
        return scores

    def proj(xn, qkv, r0, n, ks=range(NT)):
        def finish(m, c, y):
            rows = slice(HALO + r0, HALO + r0 + n)
            if ks[0] > 0:
                y = qkv[m * NT + c, rows, :] + y
            qkv[m * NT + c, rows, :] = y
            if (m, c, ks[-1]) == (0, NT - 1, NT - 1):
                written["qkv"] = r0 + n
            if m > 0 and r0 == 0 and ks[-1] == NT - 1:
                qkv[m * NT + c, 0:HALO, :] = jnp.broadcast_to(y[0:1], (HALO, 128))

        return [step for m in (1, 2, 0) for c in range(NT) for step in _tiles(
            lambda k: after("xn", r0 + n, pltpu.bitcast(xn[r0 // 2:(r0 + n) // 2, k], BF16)),
            lambda k, m=m, c=c: pltpu.bitcast(wp_v[m, c * 64:(c + 1) * 64, k], BF16),
            NT_DIMS, functools.partial(finish, m, c), ks)]

    held = {}

    def attn_rows(qkv, o, row, start, gate):
        def window(plane, w):
            return after("qkv", row + RA, qkv[plane, pl.ds(HALO + row - DIL * w, RA), :])

        scale = _const(DH ** -0.5 * LOG2E, gate, RA)
        q = [window(c, 0) * scale for c in range(NT)]
        logits = []
        for w in range(W):
            p = q[0] * window(NT, w)
            for c in range(1, NT):
                p = p + q[c] * window(NT + c, w)
            p = p + pltpu.roll(p, 64, 1)
            p = p + pltpu.roll(p, 32, 1)
            if start is not None and row < DIL * w:
                p = jnp.where(sub >= DIL * w - row - start, p, -1e9 * LOG2E)
            logits.append(p)
        top = functools.reduce(jnp.maximum, logits)
        e = [jnp.exp2(p - top) for p in logits]
        inv = pl.reciprocal(functools.reduce(jnp.add, e), full_range=False)
        done = []
        for c in range(NT):
            acc = e[0] * window(2 * NT + c, 0)
            for w in range(1, W):
                acc = acc + e[w] * window(2 * NT + c, w)
            res = acc * inv
            done.append(pltpu.bitcast(res, U32))
            if row % 16 == 0:
                held[c] = res
            else:
                pair = jnp.concatenate([held.pop(c), res], axis=0).astype(BF16)
                o[row // 2 - 4:row // 2 + 4, TILES[c]] = pltpu.bitcast(pair, U32)
                written["o"] = row + RA
        return functools.reduce(jnp.bitwise_or, done)

    def out_rows(o, xn, x, s, out, r0, n):
        def finish(cols, y):
            s[r0:r0 + n, cols] = y
            g = _silu(pltpu.bitcast(xn[r0 // 2:(r0 + n) // 2, cols], BF16).astype(F32))
            out[r0:r0 + n, cols] = (x[r0:r0 + n, cols].astype(F32) + y * g).astype(BF16)

        return [step for cols in TILES for step in _tiles(
            lambda k: after("o", r0 + n, pltpu.bitcast(o[r0 // 2:(r0 + n) // 2, k], BF16)),
            lambda k, cols=cols: pltpu.bitcast(wop_v[k.start // 2:k.stop // 2, cols], BF16),
            NN_DIMS, functools.partial(finish, cols))]

    def tile_of(idx):
        return pl.multiple_of((idx >> 4) << 4, 16)

    def normed_tile(idx):
        return pltpu.bitcast(xn_v[pl.ds(pl.multiple_of((idx >> 4) << 3, 8), 8), :], BF16).astype(F32)

    def route():
        keys, vals = [], []
        for half in range(NB // 4):
            r = r_v[4 * half]
            for b in range(1, 4):
                r = jnp.where(lane >= 32 * b, pltpu.roll(r_v[4 * half + b], 32 * b, 1), r)
            r = _bf16_round(r) + 0.0
            bits = pltpu.bitcast(r, I32)
            rank = jnp.where(bits < 0, bits ^ np.int32(0x7FFFFFFF), bits) >> 16
            rank = jnp.where(r != r, np.int32(-2 ** 15), rank)
            keys.append(rank * S + (S - 1 - half * 1024 - lane * 8 - sub))
            vals.append(r)
        row = lax.broadcasted_iota(I32, (16, D), 0)
        xs = jnp.zeros((8, D), F32)
        sel = []
        for i in range(2):
            best = jnp.max(jnp.maximum(keys[0], keys[1]))
            score = jnp.where(keys[0] == best, vals[0], jnp.where(keys[1] == best, vals[1], 0.0))
            keys = [jnp.where(key == best, np.int32(-2 ** 31), key) for key in keys]
            idx = (S - 1) - (best & (S - 1))
            picked = jnp.sum(jnp.where(row == (idx & 15), normed_tile(idx), 0.0), axis=0, keepdims=True)
            xs = jnp.where(row[:8] == i, picked, xs)
            sel.append((idx, jnp.sum(score, keepdims=True)))
        xs_v[...] = xs
        return sel

    def ffn():
        chunks = [slice(lo, min(lo + 128, F)) for lo in range(0, F, 128)]
        pre, hid, y = {}, {}, [0.0] * NT

        def up(w, j):
            return _tiles(lambda k: xs_v[:, k], lambda k: w[chunks[j], k], NT_DIMS, pre.setdefault(j, []).append)

        def down(j, c):
            if c == 0:
                g, u = pre[j]
                hid[j] = _bf16_round(g * jax.nn.sigmoid(g) * u)
            y[c] = y[c] + lax.dot_general(hid[j], wd_v[chunks[j], TILES[c]], NN_DIMS, preferred_element_type=F32)

        steps = []
        for j in range(len(chunks) + 1):
            if j < len(chunks):
                steps += up(wg_v, j) + up(wu_v, j)
            if j > 0:
                steps += [functools.partial(down, j - 1, c) for c in range(NT)]
        return steps, y

    def run(rounds, attn=(), ln=()):
        tasks = []
        for kind, jobs, step in (("attn", attn, RA), ("ln", ln, RL)):
            for k, job in enumerate(jobs):
                lo, hi = job[-1]
                tasks += [(lo + (hi - lo) * r / T, kind, k, r) for r in range(0, T, step)]
        tasks.sort()
        done = {"attn": [], "ln": []}
        pos = 0
        for j in range(-1, len(rounds)):
            y = [v for v in [call() for call in rounds[j][2]] if v is not None][-1] if j >= 0 else None
            while pos < len(tasks):
                frac, kind, k, off = tasks[pos]
                t = int(frac * (rounds[-1][0] + rounds[-1][1])) - MXU_LATENCY if rounds else 0
                if j + 1 < len(rounds) and t >= rounds[j + 1][0]:
                    break
                pos += 1
                lag = IN_FLIGHT[kind]
                bits = done[kind][-lag] if rounds and len(done[kind]) >= lag else None
                if y is not None:
                    g = min(t - rounds[j][0], rounds[j][1] - 8) // 8
                    mine = pltpu.bitcast(y[8 * g:8 * g + 8], U32)
                    bits = mine if bits is None else bits | mine
                gate = None if bits is None else (bits >> 31) >> 1
                if kind == "attn":
                    qkv, o, first, start, _ = attn[k]
                    done[kind].append(attn_rows(qkv, o, first + off, start, gate))
                else:
                    x, xn, first, block, _ = ln[k]
                    if off == 0:
                        scores = jnp.zeros((8, 128), F32)
                    scores = ln_rows(x, xn, first + off, off // 8, scores, gate)
                    done[kind].append(pltpu.bitcast(scores, U32))
                    if off == T - RL:
                        r_v[block] = scores

    for c in (get_wr, get_x[0], *get_w, get_x[1], get_wo, get_x[2], get_x[3], *get_ffn):
        c.start()
    get_wr.wait()
    get_x[0].wait()
    wr_v[...] = jnp.broadcast_to(wr1_v[...].astype(F32).reshape(1, D), (RL, D))
    run([], ln=[(x_v, xn_v, 0, 0, (0.0, 0.0))])
    get_w[0].wait()
    prep_qkv(0)
    for k in range(3):
        get_w[k + 1].wait()
        run(_rounds(proj(xn_v, qkv_v, 0, T, [k]), T))
        prep_qkv(k + 1)
    get_w[4].wait()
    get_x[1].wait()
    prep_qkv(4)
    n = 12
    steps = proj(xn_v, qkv_v, 0, T, [3])[:n] + proj(xn_v, qkv_v, 0, T, [3, 4])[2 * n:] + proj(xn_v, qkv_v, 0, T, [4])[:n]
    run(_rounds(steps, T), ln=[(x_v, xn_v, T, 1, (0.0, 0.55))])
    get_wo.wait()
    for c in range(NT):
        tmp_v[3, c, :D // 2] = pltpu.bitcast(wo_v[:, TILES[c]], U32)
    for c in range(NT):
        _regroup(tmp_v.at[3, c], wop_v, TILES[c])
    get_x[2].wait()

    def trip(i, carry):
        base = pl.multiple_of(i * (U * T), T)
        pairs = pl.multiple_of(i * (U * M), M)
        qkv = qkv_v.at[:, pl.ds(base, HALO + (U + 1) * T), :]
        xn = xn_v.at[pl.ds(pairs, (U + 2) * M), :]
        o = o_v.at[pl.ds(pairs, U * M), :]
        x = x_v.at[pl.ds(base, (U + 2) * T), :]
        s, out = [ref.at[pl.ds(base, U * T), :] for ref in (s_v, out_v)]
        assert written == dict(xn=2 * T, qkv=T, o=0)
        steps, attn, ln = [], [], []
        for k in range(U):
            steps += proj(xn, qkv, (k + 1) * T, T) + out_rows(o, xn, x, s, out, k * T, T)
            attn.append((qkv, o, k * T, base, [(k + f) / U for f in ATTN_SPAN]))
            ln.append((x, xn, (k + 2) * T, i * U + k + 2, [(k + f) / U for f in LN_SPAN]))
        run(_rounds(steps, T), attn, ln)
        assert written == dict(xn=(U + 2) * T, qkv=(U + 1) * T, o=U * T)
        out_copy(i, pl.ds(base, U * T)).start()
        pl.when(i == 0)(get_x[3].wait)
        return carry

    trips = (NB - 2) // U
    lax.fori_loop(0, trips, trip, 0)

    for c in get_ffn:
        c.wait()
    sel = route()
    small, routed = ffn()
    last = S - T
    written.update(xn=S, qkv=last, o=last - T)
    steps = [step for r in range(last, S, M) for step in proj(xn_v, qkv_v, r, M)]
    issued = {}
    for r in range(last - T, S, M):
        steps += out_rows(o_v, xn_v, x_v, s_v, out_v, r, M)
        issued[r + M] = len(steps)
    rounds = _rounds(steps, M, lambda j: small[4 * (j - 9):4 * (j - 8)] if j >= 9 else [])
    assert len(small) <= 4 * (len(rounds) - 9)
    stages = [(0, last - T, [out_copy(i, pl.ds(i * U * T, U * T)) for i in range(trips)])]
    for i, (lo, hi) in enumerate(((last - T, last), (last, S - M))):
        stages.append((lo, hi, [out_copy(trips + i, slice(lo, hi))]))
        rounds[issued[hi] // 4 + 2][2].append(stages[-1][2][0].start)
    left, right = [out_copy(trips + 2 + i, slice(S - M, S), cols)
                   for i, cols in enumerate((slice(0, 3 * 128), slice(3 * 128, D)))]
    stages.append((S - M, S, [left, right]))
    rounds[(len(steps) - 2 * NT) // 4 + 1][2].append(left.start)
    run(rounds, [(qkv_v, o_v, last - T, None, (0.05, 0.4)), (qkv_v, o_v, last, None, (0.42, 0.86))])

    y = jnp.concatenate(routed, axis=1)
    y = [y[i:i + 1, :] * jax.nn.sigmoid(score) for i, (_, score) in enumerate(sel)]
    row = lax.broadcasted_iota(I32, (16, D), 0)
    tiles = [tile_of(idx) for idx, _ in sel]
    for i, ((idx, _), tile) in enumerate(zip(sel, tiles)):
        upd = jnp.zeros((16, D), F32)
        for (other, _), y_other in zip(sel, y):
            upd = jnp.where(row == other - tile, y_other, upd)
        rows = pl.ds(tile, 16)
        fix_v[i] = (x_v[rows, :].astype(F32) + s_v[rows, :] * _silu(normed_tile(idx) + upd)).astype(BF16)
    right.start()

    fixes = [pltpu.make_async_copy(fix_v.at[i], out_hbm.at[pl.ds(tile, 16), :], sem_fix.at[i])
             for i, tile in enumerate(tiles)]
    distinct = tiles[1] != tiles[0]
    for lo, hi, copies in stages:
        for c in copies:
            c.wait()
        pl.when((tiles[0] >= lo) & (tiles[0] < hi))(fixes[0].start)
        pl.when((tiles[1] >= lo) & (tiles[1] < hi) & distinct)(fixes[1].start)
    fixes[0].wait()
    pl.when(distinct)(fixes[1].wait)


@jax.jit
def pallas_recurrent_scan__sliding_local_dilated__moe_arch_mod__prompt_kernel(
    A_x: jax.Array,
    A_wqkv: jax.Array,
    A_wo: jax.Array,
    B_x: jax.Array,
    B_w_r: jax.Array,
    B_w_gate: jax.Array,
    B_w_up: jax.Array,
    B_w_down: jax.Array,
):
    del B_x
    hbm = pl.BlockSpec(memory_space=pltpu.HBM)
    out = pl.pallas_call(
        _kernel,
        out_shape=jax.ShapeDtypeStruct((S, D), BF16),
        in_specs=[hbm] * 7,
        out_specs=hbm,
        scratch_shapes=[
            pltpu.VMEM((S, D), BF16),
            pltpu.VMEM((D, 3 * D), BF16),
            pltpu.VMEM((D, D), BF16),
            pltpu.VMEM((F, D), BF16),
            pltpu.VMEM((F, D), BF16),
            pltpu.VMEM((F, D), BF16),
            pltpu.VMEM((4, NT, D // 2 + 32, 128), U32),
            pltpu.VMEM((3, D // 2, D), U32),
            pltpu.VMEM((D // 2, D), U32),
            pltpu.VMEM((S // 2, D), U32),
            pltpu.VMEM((3 * NT + 1, HALO + S, 128), F32),
            pltpu.VMEM((S // 2, D), U32),
            pltpu.VMEM((S, D), F32),
            pltpu.VMEM((S, D), BF16),
            pltpu.VMEM((RL, D), F32),
            pltpu.VMEM((NB, 8, 128), F32),
            pltpu.VMEM((8, D), F32),
            pltpu.VMEM((2, 16, D), BF16),
            pltpu.VMEM((D,), BF16),
            pltpu.SemaphoreType.DMA((14,)),
            pltpu.SemaphoreType.DMA(((NB - 2) // U + 4,)),
            pltpu.SemaphoreType.DMA((2,)),
        ],
        compiler_params=pltpu.CompilerParams(vmem_limit_bytes=64 * 2 ** 20),
        name="fused",
    )(A_x.reshape(S, D), A_wqkv, A_wo, B_w_r, B_w_gate.T, B_w_up.T, B_w_down)
    return out.reshape(1, S, D)
```

```python
import functools
import math

import jax
import jax.numpy as jnp
import numpy as np
from jax import lax
from jax.experimental import pallas as pl
from jax.experimental.pallas import tpu as pltpu

F32, BF16, U32, I32 = jnp.float32, jnp.bfloat16, jnp.uint32, jnp.int32

S, D, H, DH, F = 2048, 640, 32, 20, 1728
W, DIL = 8, 2
NT = D // 128
TILES = [slice(c * 128, (c + 1) * 128) for c in range(NT)]
HALO = 16
T = 256
M = T // 2
NB = S // T
U = 2
RA, RL = 8, 16
LOG2E = math.log2(math.e)
EPS_BF16 = float(np.asarray(1e-5, dtype=jnp.bfloat16).astype(np.float32))

MXU_LATENCY = 100
IN_FLIGHT = {"attn": 4, "ln": 5}
ATTN_SPAN, LN_SPAN = (0.0, 0.5), (0.52, 0.86)

NN_DIMS = (((1,), (0,)), ((), ()))
NT_DIMS = (((1,), (1,)), ((), ()))


def _bf16_round(v):
    return v.astype(BF16).astype(F32)


def _regroup(src, dst, cols):
    for j in range(DH // 2):
        for g in range(2):
            even = src[pl.ds(g * 160 + j, 8, stride=DH), :]
            odd = src[pl.ds(g * 160 + DH // 2 + j, 8, stride=DH), :]
            row = j * H + 8 * g
            dst[row:row + 8, cols] = (even & np.uint32(0xFFFF)) | (odd << 16)
            dst[row + H // 2:row + H // 2 + 8, cols] = (even >> 16) | (odd & np.uint32(0xFFFF0000))


def _const(val, gate, rows):
    if gate is None:
        return val
    c = pltpu.bitcast(gate | np.float32(val).view(np.uint32), F32)
    return jnp.concatenate([c] * (rows // 8), axis=0)


def _layernorm(x, gate):
    tot = x[:, TILES[0]] if gate is None else x[:, TILES[0]] + _const(0.0, gate, x.shape[0])
    for cols in TILES[1:]:
        tot = tot + x[:, cols]
    mean = jnp.sum(tot, axis=-1, keepdims=True) * (1.0 / D)
    xc = x - mean
    var = jnp.sum(xc * xc, axis=-1, keepdims=True) * (1.0 / D)
    sd = _bf16_round(jnp.sqrt(_bf16_round(_bf16_round(var) + EPS_BF16)))
    return (_bf16_round(x - _bf16_round(mean)) * (1.0 / sd)).astype(BF16)


def _silu(z):
    h = 0.5 * z
    return h * jnp.tanh(h) + h


def _tiles(lhs, rhs, dims, finish, ks=range(NT)):
    acc = []

    def step(k, parts=1):
        a, b = lhs(TILES[k]), rhs(TILES[k])
        n = a.shape[0] // parts
        y = jnp.concatenate([lax.dot_general(a[i * n:(i + 1) * n], b, dims, preferred_element_type=F32)
                             for i in range(parts)], axis=0)
        acc.append(acc.pop() + y if acc else y)
        if k == ks[-1]:
            finish(acc.pop())
        return y

    return [functools.partial(step, k) for k in ks]


def _rounds(steps, rows, extra=None):
    left = len(steps) % 4
    if left in (1, 2):
        steps = steps[:-left] + [functools.partial(step, parts=4 // left) for step in steps[-left:]]
    rounds, t = [], 0
    for j in range(0, len(steps), 4):
        short = extra(j // 4) if extra else []
        t += 3 * len(short)
        rounds.append((t, rows, short + steps[j:j + 4]))
        t += rows
    return rounds


def _kernel(*refs):
    pl.run_scoped(functools.partial(_body, *refs), pltpu.SemaphoreType.DMA((14,)),
                  pltpu.SemaphoreType.DMA(((NB - 2) // U + 4,)), pltpu.SemaphoreType.DMA((2,)))


def _body(x_hbm, wqkv_hbm, wo_hbm, wr_hbm, wg_hbm, wu_hbm, wd_hbm, out_hbm,
          x_v, wqkv_v, wo_v, wg_v, wu_v, wd_v, tmp_v, wp_v, wop_v,
          xn_v, qkv_v, o_v, s_v, out_v, wr_v, r_v, xs_v, fix_v, wr1_v, sem_in, sem_out, sem_fix):
    sems = iter(range(sem_in.shape[0]))

    def copy_in(src, dst):
        return pltpu.make_async_copy(src, dst, sem_in.at[next(sems)])

    def x_copy(lo, hi):
        return copy_in(x_hbm.at[lo:hi, :], x_v.at[lo:hi, :])

    def out_copy(i, rows, cols=slice(None)):
        return pltpu.make_async_copy(out_v.at[rows, cols], out_hbm.at[rows, cols], sem_out.at[i])

    get_wr = copy_in(wr_hbm, wr1_v)
    get_x = [x_copy(0, T), x_copy(T, 2 * T), x_copy(2 * T, (U + 2) * T), x_copy((U + 2) * T, S)]
    get_w = [copy_in(wqkv_hbm.at[rows, :], wqkv_v.at[rows, :]) for rows in TILES]
    get_wo = copy_in(wo_hbm, wo_v)
    get_ffn = [copy_in(wg_hbm, wg_v), copy_in(wu_hbm, wu_v), copy_in(wd_hbm, wd_v)]

    lane = lax.broadcasted_iota(I32, (8, 128), 1)
    sub = lax.broadcasted_iota(I32, (8, 128), 0)

    written = dict(xn=0, qkv=0, o=0)

    def after(name, rows, value):
        assert rows <= written[name], name
        return value

    def prep_qkv(k):
        for m in range(3):
            tmp_v[m, k, :D // 2] = pltpu.bitcast(wqkv_v[TILES[k], m * D:(m + 1) * D].T, U32)
        for m in range(3):
            _regroup(tmp_v.at[m, k], wp_v.at[m], TILES[k])

    def ln_rows(x, xn_out, row, slot, scores, gate):
        xn = _layernorm(x[row:row + RL, :].astype(F32), gate)
        xn_out[row // 2:(row + RL) // 2, :] = pltpu.bitcast(xn, U32)
        written["xn"] = row + RL
        r = jnp.sum(xn.astype(F32) * wr_v[...], axis=-1, keepdims=True)
        for i in range(RL // 8):
            scores = jnp.where(lane == slot + i, jnp.broadcast_to(r[8 * i:8 * i + 8], (8, 128)), scores)
        return scores

    def proj(xn, qkv, r0, n, ks=range(NT)):
        def finish(m, c, y):
            rows = slice(HALO + r0, HALO + r0 + n)
            if ks[0] > 0:
                y = qkv[m * NT + c, rows, :] + y
            qkv[m * NT + c, rows, :] = y
            if (m, c, ks[-1]) == (0, NT - 1, NT - 1):
                written["qkv"] = r0 + n
            if m > 0 and r0 == 0 and ks[-1] == NT - 1:
                qkv[m * NT + c, 0:HALO, :] = jnp.broadcast_to(y[0:1], (HALO, 128))

        return [step for m in (1, 2, 0) for c in range(NT) for step in _tiles(
            lambda k: after("xn", r0 + n, pltpu.bitcast(xn[r0 // 2:(r0 + n) // 2, k], BF16)),
            lambda k, m=m, c=c: pltpu.bitcast(wp_v[m, c * 64:(c + 1) * 64, k], BF16),
            NT_DIMS, functools.partial(finish, m, c), ks)]

    held = {}

    def attn_rows(qkv, o, row, start, gate):
        def window(plane, w):
            return after("qkv", row + RA, qkv[plane, pl.ds(HALO + row - DIL * w, RA), :])

        scale = _const(DH ** -0.5 * LOG2E, gate, RA)
        q = [window(c, 0) * scale for c in range(NT)]
        logits = []
        for w in range(W):
            p = q[0] * window(NT, w)
            for c in range(1, NT):
                p = p + q[c] * window(NT + c, w)
            p = p + pltpu.roll(p, 64, 1)
            p = p + pltpu.roll(p, 32, 1)
            if start is not None and row < DIL * w:
                p = jnp.where(sub >= DIL * w - row - start, p, -1e9 * LOG2E)
            logits.append(p)
        top = functools.reduce(jnp.maximum, logits)
        e = [jnp.exp2(p - top) for p in logits]
        inv = pl.reciprocal(functools.reduce(jnp.add, e), full_range=False)
        done = []
        for c in range(NT):
            acc = e[0] * window(2 * NT + c, 0)
            for w in range(1, W):
                acc = acc + e[w] * window(2 * NT + c, w)
            res = acc * inv
            done.append(pltpu.bitcast(res, U32))
            if row % 16 == 0:
                held[c] = res
            else:
                pair = jnp.concatenate([held.pop(c), res], axis=0).astype(BF16)
                o[row // 2 - 4:row // 2 + 4, TILES[c]] = pltpu.bitcast(pair, U32)
                written["o"] = row + RA
        return functools.reduce(jnp.bitwise_or, done)

    def out_rows(o, xn, x, s, out, r0, n):
        def finish(cols, y):
            s[r0:r0 + n, cols] = y
            g = _silu(pltpu.bitcast(xn[r0 // 2:(r0 + n) // 2, cols], BF16).astype(F32))
            out[r0:r0 + n, cols] = (x[r0:r0 + n, cols].astype(F32) + y * g).astype(BF16)

        return [step for cols in TILES for step in _tiles(
            lambda k: after("o", r0 + n, pltpu.bitcast(o[r0 // 2:(r0 + n) // 2, k], BF16)),
            lambda k, cols=cols: pltpu.bitcast(wop_v[k.start // 2:k.stop // 2, cols], BF16),
            NN_DIMS, functools.partial(finish, cols))]

    def tile_of(idx):
        return pl.multiple_of((idx >> 4) << 4, 16)

    def normed_tile(idx):
        return pltpu.bitcast(xn_v[pl.ds(pl.multiple_of((idx >> 4) << 3, 8), 8), :], BF16).astype(F32)

    def route():
        keys, vals = [], []
        for half in range(NB // 4):
            r = r_v[4 * half]
            for b in range(1, 4):
                r = jnp.where(lane >= 32 * b, pltpu.roll(r_v[4 * half + b], 32 * b, 1), r)
            r = _bf16_round(r) + 0.0
            bits = pltpu.bitcast(r, I32)
            rank = jnp.where(bits < 0, bits ^ np.int32(0x7FFFFFFF), bits) >> 16
            rank = jnp.where(r != r, np.int32(-2 ** 15), rank)
            keys.append(rank * S + (S - 1 - half * 1024 - lane * 8 - sub))
            vals.append(r)
        row = lax.broadcasted_iota(I32, (16, D), 0)
        xs = jnp.zeros((8, D), F32)
        sel = []
        for i in range(2):
            best = jnp.max(jnp.maximum(keys[0], keys[1]))
            score = jnp.where(keys[0] == best, vals[0], jnp.where(keys[1] == best, vals[1], 0.0))
            keys = [jnp.where(key == best, np.int32(-2 ** 31), key) for key in keys]
            idx = (S - 1) - (best & (S - 1))
            picked = jnp.sum(jnp.where(row == (idx & 15), normed_tile(idx), 0.0), axis=0, keepdims=True)
            xs = jnp.where(row[:8] == i, picked, xs)
            sel.append((idx, jnp.sum(score, keepdims=True)))
        xs_v[...] = xs
        return sel

    def ffn():
        chunks = [slice(lo, min(lo + 128, F)) for lo in range(0, F, 128)]
        pre, hid, y = {}, {}, [0.0] * NT

        def up(w, j):
            return _tiles(lambda k: xs_v[:, k], lambda k: w[chunks[j], k], NT_DIMS, pre.setdefault(j, []).append)

        def down(j, c):
            if c == 0:
                g, u = pre[j]
                hid[j] = _bf16_round(g * jax.nn.sigmoid(g) * u)
            y[c] = y[c] + lax.dot_general(hid[j], wd_v[chunks[j], TILES[c]], NN_DIMS, preferred_element_type=F32)

        steps = []
        for j in range(len(chunks) + 1):
            if j < len(chunks):
                steps += up(wg_v, j) + up(wu_v, j)
            if j > 0:
                steps += [functools.partial(down, j - 1, c) for c in range(NT)]
        return steps, y

    def run(rounds, attn=(), ln=()):
        tasks = []
        for kind, jobs, step in (("attn", attn, RA), ("ln", ln, RL)):
            for k, job in enumerate(jobs):
                lo, hi = job[-1]
                tasks += [(lo + (hi - lo) * r / T, kind, k, r) for r in range(0, T, step)]
        tasks.sort()
        done = {"attn": [], "ln": []}
        pos = 0
        for j in range(-1, len(rounds)):
            y = [v for v in [call() for call in rounds[j][2]] if v is not None][-1] if j >= 0 else None
            while pos < len(tasks):
                frac, kind, k, off = tasks[pos]
                t = int(frac * (rounds[-1][0] + rounds[-1][1])) - MXU_LATENCY if rounds else 0
                if j + 1 < len(rounds) and t >= rounds[j + 1][0]:
                    break
                pos += 1
                lag = IN_FLIGHT[kind]
                bits = done[kind][-lag] if rounds and len(done[kind]) >= lag else None
                if y is not None:
                    g = min(t - rounds[j][0], rounds[j][1] - 8) // 8
                    mine = pltpu.bitcast(y[8 * g:8 * g + 8], U32)
                    bits = mine if bits is None else bits | mine
                gate = None if bits is None else (bits >> 31) >> 1
                if kind == "attn":
                    qkv, o, first, start, _ = attn[k]
                    done[kind].append(attn_rows(qkv, o, first + off, start, gate))
                else:
                    x, xn, first, block, _ = ln[k]
                    if off == 0:
                        scores = jnp.zeros((8, 128), F32)
                    scores = ln_rows(x, xn, first + off, off // 8, scores, gate)
                    done[kind].append(pltpu.bitcast(scores, U32))
                    if off == T - RL:
                        r_v[block] = scores

    for c in (get_wr, get_x[0], *get_w, get_x[1], get_wo, get_x[2], get_x[3], *get_ffn):
        c.start()
    get_wr.wait()
    get_x[0].wait()
    wr_v[...] = jnp.broadcast_to(wr1_v[...].astype(F32).reshape(1, D), (RL, D))
    run([], ln=[(x_v, xn_v, 0, 0, (0.0, 0.0))])
    get_w[0].wait()
    prep_qkv(0)
    for k in range(3):
        get_w[k + 1].wait()
        run(_rounds(proj(xn_v, qkv_v, 0, T, [k]), T))
        prep_qkv(k + 1)
    get_w[4].wait()
    get_x[1].wait()
    prep_qkv(4)
    n = 12
    steps = proj(xn_v, qkv_v, 0, T, [3])[:n] + proj(xn_v, qkv_v, 0, T, [3, 4])[2 * n:] + proj(xn_v, qkv_v, 0, T, [4])[:n]
    run(_rounds(steps, T), ln=[(x_v, xn_v, T, 1, (0.0, 0.55))])
    get_wo.wait()
    for c in range(NT):
        tmp_v[3, c, :D // 2] = pltpu.bitcast(wo_v[:, TILES[c]], U32)
    for c in range(NT):
        _regroup(tmp_v.at[3, c], wop_v, TILES[c])
    get_x[2].wait()

    def trip(i, carry):
        base = pl.multiple_of(i * (U * T), T)
        pairs = pl.multiple_of(i * (U * M), M)
        qkv = qkv_v.at[:, pl.ds(base, HALO + (U + 1) * T), :]
        xn = xn_v.at[pl.ds(pairs, (U + 2) * M), :]
        o = o_v.at[pl.ds(pairs, U * M), :]
        x = x_v.at[pl.ds(base, (U + 2) * T), :]
        s, out = [ref.at[pl.ds(base, U * T), :] for ref in (s_v, out_v)]
        assert written == dict(xn=2 * T, qkv=T, o=0)
        steps, attn, ln = [], [], []
        for k in range(U):
            steps += proj(xn, qkv, (k + 1) * T, T) + out_rows(o, xn, x, s, out, k * T, T)
            attn.append((qkv, o, k * T, base, [(k + f) / U for f in ATTN_SPAN]))
            ln.append((x, xn, (k + 2) * T, i * U + k + 2, [(k + f) / U for f in LN_SPAN]))
        run(_rounds(steps, T), attn, ln)
        assert written == dict(xn=(U + 2) * T, qkv=(U + 1) * T, o=U * T)
        out_copy(i, pl.ds(base, U * T)).start()
        pl.when(i == 0)(get_x[3].wait)
        return carry

    trips = (NB - 2) // U
    lax.fori_loop(0, trips, trip, 0)

    for c in get_ffn:
        c.wait()
    sel = route()
    small, routed = ffn()
    last = S - T
    written.update(xn=S, qkv=last, o=last - T)
    steps = [step for r in range(last, S, M) for step in proj(xn_v, qkv_v, r, M)]
    issued = {}
    for r in range(last - T, S, M):
        steps += out_rows(o_v, xn_v, x_v, s_v, out_v, r, M)
        issued[r + M] = len(steps)
    rounds = _rounds(steps, M, lambda j: small[4 * (j - 9):4 * (j - 8)] if j >= 9 else [])
    assert len(small) <= 4 * (len(rounds) - 9)
    stages = [(0, last - T, [out_copy(i, pl.ds(i * U * T, U * T)) for i in range(trips)])]
    for i, (lo, hi) in enumerate(((last - T, last), (last, S - M))):
        stages.append((lo, hi, [out_copy(trips + i, slice(lo, hi))]))
        rounds[issued[hi] // 4 + 2][2].append(stages[-1][2][0].start)
    left, right = [out_copy(trips + 2 + i, slice(S - M, S), cols)
                   for i, cols in enumerate((slice(0, 3 * 128), slice(3 * 128, D)))]
    stages.append((S - M, S, [left, right]))
    rounds[(len(steps) - 2 * NT) // 4 + 1][2].append(left.start)
    run(rounds, [(qkv_v, o_v, last - T, None, (0.05, 0.4)), (qkv_v, o_v, last, None, (0.42, 0.86))])

    y = jnp.concatenate(routed, axis=1)
    y = [y[i:i + 1, :] * jax.nn.sigmoid(score) for i, (_, score) in enumerate(sel)]
    row = lax.broadcasted_iota(I32, (16, D), 0)
    tiles = [tile_of(idx) for idx, _ in sel]
    for i, ((idx, _), tile) in enumerate(zip(sel, tiles)):
        upd = jnp.zeros((16, D), F32)
        for (other, _), y_other in zip(sel, y):
            upd = jnp.where(row == other - tile, y_other, upd)
        rows = pl.ds(tile, 16)
        fix_v[i] = (x_v[rows, :].astype(F32) + s_v[rows, :] * _silu(normed_tile(idx) + upd)).astype(BF16)
    right.start()

    fixes = [pltpu.make_async_copy(fix_v.at[i], out_hbm.at[pl.ds(tile, 16), :], sem_fix.at[i])
             for i, tile in enumerate(tiles)]
    distinct = tiles[1] != tiles[0]
    for lo, hi, copies in stages:
        for c in copies:
            c.wait()
        pl.when((tiles[0] >= lo) & (tiles[0] < hi))(fixes[0].start)
        pl.when((tiles[1] >= lo) & (tiles[1] < hi) & distinct)(fixes[1].start)
    fixes[0].wait()
    pl.when(distinct)(fixes[1].wait)


@jax.jit
def pallas_recurrent_scan__sliding_local_dilated__moe_arch_mod__prompt_kernel(
    A_x: jax.Array,
    A_wqkv: jax.Array,
    A_wo: jax.Array,
    B_x: jax.Array,
    B_w_r: jax.Array,
    B_w_gate: jax.Array,
    B_w_up: jax.Array,
    B_w_down: jax.Array,
):
    del B_x
    hbm = pl.BlockSpec(memory_space=pltpu.HBM)
    out = pl.pallas_call(
        _kernel,
        out_shape=jax.ShapeDtypeStruct((S, D), BF16),
        in_specs=[hbm] * 7,
        out_specs=hbm,
        scratch_shapes=[
            pltpu.VMEM((S, D), BF16),
            pltpu.VMEM((D, 3 * D), BF16),
            pltpu.VMEM((D, D), BF16),
            pltpu.VMEM((F, D), BF16),
            pltpu.VMEM((F, D), BF16),
            pltpu.VMEM((F, D), BF16),
            pltpu.VMEM((4, NT, D // 2 + 32, 128), U32),
            pltpu.VMEM((3, D // 2, D), U32),
            pltpu.VMEM((D // 2, D), U32),
            pltpu.VMEM((S // 2, D), U32),
            pltpu.VMEM((3 * NT + 1, HALO + S, 128), F32),
            pltpu.VMEM((S // 2, D), U32),
            pltpu.VMEM((S, D), F32),
            pltpu.VMEM((S, D), BF16),
            pltpu.VMEM((RL, D), F32),
            pltpu.VMEM((NB, 8, 128), F32),
            pltpu.VMEM((8, D), F32),
            pltpu.VMEM((2, 16, D), BF16),
            pltpu.VMEM((D,), BF16),
        ],
        compiler_params=pltpu.CompilerParams(vmem_limit_bytes=64 * 2 ** 20),
        name="fused",
    )(A_x.reshape(S, D), A_wqkv, A_wo, B_w_r, B_w_gate.T, B_w_up.T, B_w_down)
    return out.reshape(1, S, D)
```

```python
import functools
import math

import jax
import jax.numpy as jnp
import numpy as np
from jax import lax
from jax.experimental import pallas as pl
from jax.experimental.pallas import tpu as pltpu

F32, BF16, U32, I32 = jnp.float32, jnp.bfloat16, jnp.uint32, jnp.int32

S, D, H, DH, F = 2048, 640, 32, 20, 1728
W, DIL = 8, 2
NT = D // 128
TILES = [slice(c * 128, (c + 1) * 128) for c in range(NT)]
HALO = 16
T = 256
M = T // 2
NB = S // T
U = 2
TRIPS = NB // U - 2
RA, RL = 8, 16
LOG2E = math.log2(math.e)
EPS_BF16 = float(np.asarray(1e-5, dtype=jnp.bfloat16).astype(np.float32))

MXU_LATENCY = 100
IN_FLIGHT = {"attn": 4, "ln": 5}
ATTN_SPAN, LN_SPAN = (0.0, 0.5), (0.52, 0.86)

NN_DIMS = (((1,), (0,)), ((), ()))
NT_DIMS = (((1,), (1,)), ((), ()))


def _bf16_round(v):
    return v.astype(BF16).astype(F32)


def _regroup(src, dst, cols):
    for j in range(DH // 2):
        for g in range(2):
            even = src[pl.ds(g * 160 + j, 8, stride=DH), :]
            odd = src[pl.ds(g * 160 + DH // 2 + j, 8, stride=DH), :]
            row = j * H + 8 * g
            dst[row:row + 8, cols] = (even & np.uint32(0xFFFF)) | (odd << 16)
            dst[row + H // 2:row + H // 2 + 8, cols] = (even >> 16) | (odd & np.uint32(0xFFFF0000))


def _const(val, gate, rows):
    if gate is None:
        return val
    c = pltpu.bitcast(gate | np.float32(val).view(np.uint32), F32)
    return jnp.concatenate([c] * (rows // 8), axis=0)


def _layernorm(x, gate):
    tot = x[:, TILES[0]] if gate is None else x[:, TILES[0]] + _const(0.0, gate, x.shape[0])
    for cols in TILES[1:]:
        tot = tot + x[:, cols]
    mean = jnp.sum(tot, axis=-1, keepdims=True) * (1.0 / D)
    xc = x - mean
    var = jnp.sum(xc * xc, axis=-1, keepdims=True) * (1.0 / D)
    sd = _bf16_round(jnp.sqrt(_bf16_round(_bf16_round(var) + EPS_BF16)))
    return (_bf16_round(x - _bf16_round(mean)) * (1.0 / sd)).astype(BF16)


def _silu(z):
    h = 0.5 * z
    return h * jnp.tanh(h) + h


def _tiles(lhs, rhs, dims, finish, ks=range(NT)):
    acc = []

    def step(k, parts=1):
        a, b = lhs(TILES[k]), rhs(TILES[k])
        n = a.shape[0] // parts
        y = jnp.concatenate([lax.dot_general(a[i * n:(i + 1) * n], b, dims, preferred_element_type=F32)
                             for i in range(parts)], axis=0)
        acc.append(acc.pop() + y if acc else y)
        if k == ks[-1]:
            finish(acc.pop())
        return y

    return [functools.partial(step, k) for k in ks]


def _rounds(steps, rows, extra=None):
    left = len(steps) % 4
    if left in (1, 2):
        steps = steps[:-left] + [functools.partial(step, parts=4 // left) for step in steps[-left:]]
    rounds, t = [], 0
    for j in range(0, len(steps), 4):
        short = extra(j // 4) if extra else []
        t += 3 * len(short)
        rounds.append((t, rows, short + steps[j:j + 4]))
        t += rows
    return rounds


def _kernel(*refs):
    pl.run_scoped(functools.partial(_body, *refs), pltpu.SemaphoreType.DMA((NB + NT + 5,)),
                  pltpu.SemaphoreType.DMA((TRIPS + 5,)), pltpu.SemaphoreType.DMA((2,)))


def _body(x_hbm, wqkv_hbm, wo_hbm, wr_hbm, wg_hbm, wu_hbm, wd_hbm, out_hbm,
          x_v, wqkv_v, wo_v, wg_v, wu_v, wd_v, tmp_v, wp_v, wop_v,
          xn_v, qkv_v, o_v, s_v, out_v, wr_v, r_v, xs_v, fix_v, wr1_v, sem_in, sem_out, sem_fix):
    sems = iter(range(NB, sem_in.shape[0]))

    def copy_in(src, dst):
        return pltpu.make_async_copy(src, dst, sem_in.at[next(sems)])

    def x_copy(b):
        rows = pl.ds(b * T if isinstance(b, int) else pl.multiple_of(b * T, T), T)
        return pltpu.make_async_copy(x_hbm.at[rows, :], x_v.at[rows, :], sem_in.at[b])

    def out_copy(i, rows, cols=slice(None)):
        return pltpu.make_async_copy(out_v.at[rows, cols], out_hbm.at[rows, cols], sem_out.at[i])

    get_wr = copy_in(wr_hbm, wr1_v)
    get_x = [x_copy(b) for b in range(NB)]
    get_w = [copy_in(wqkv_hbm.at[rows, :], wqkv_v.at[rows, :]) for rows in TILES]
    get_wo = copy_in(wo_hbm, wo_v.at[:D, :])
    get_ffn = [copy_in(wg_hbm, wg_v), copy_in(wu_hbm, wu_v), copy_in(wd_hbm, wd_v)]

    lane = lax.broadcasted_iota(I32, (8, 128), 1)
    sub = lax.broadcasted_iota(I32, (8, 128), 0)

    written = dict(xn=0, qkv=0, o=0)

    def after(name, rows, value):
        assert rows <= written[name], name
        return value

    def prep_qkv(k):
        for m in range(3):
            tmp_v[m, k, :D // 2] = pltpu.bitcast(wqkv_v[TILES[k], m * D:(m + 1) * D].T, U32)
        for m in range(3):
            _regroup(tmp_v.at[m, k], wp_v.at[m], TILES[k])

    def ln_rows(x, xn_out, row, slot, scores, gate):
        xn = _layernorm(x[row:row + RL, :].astype(F32), gate)
        xn_out[row // 2:(row + RL) // 2, :] = pltpu.bitcast(xn, U32)
        written["xn"] = row + RL
        r = jnp.sum(xn.astype(F32) * wr_v[...], axis=-1, keepdims=True)
        for i in range(RL // 8):
            scores = jnp.where(lane == slot + i, jnp.broadcast_to(r[8 * i:8 * i + 8], (8, 128)), scores)
        return scores

    def proj(xn, qkv, r0, n, ks=range(NT)):
        def finish(m, c, y):
            rows = slice(HALO + r0, HALO + r0 + n)
            if ks[0] > 0:
                y = qkv[m * NT + c, rows, :] + y
            qkv[m * NT + c, rows, :] = y
            if (m, c, ks[-1]) == (0, NT - 1, NT - 1):
                written["qkv"] = r0 + n
            if m > 0 and r0 == 0 and ks[-1] == NT - 1:
                qkv[m * NT + c, 0:HALO, :] = jnp.broadcast_to(y[0:1], (HALO, 128))

        return [step for m in (1, 2, 0) for c in range(NT) for step in _tiles(
            lambda k: after("xn", r0 + n, pltpu.bitcast(xn[r0 // 2:(r0 + n) // 2, k], BF16)),
            lambda k, m=m, c=c: pltpu.bitcast(wp_v[m, c * 64:(c + 1) * 64, k], BF16),
            NT_DIMS, functools.partial(finish, m, c), ks)]

    held = {}

    def attn_rows(qkv, o, row, head, gate):
        def window(plane, w):
            return after("qkv", row + RA, qkv[plane, pl.ds(HALO + row - DIL * w, RA), :])

        scale = _const(DH ** -0.5 * LOG2E, gate, RA)
        q = [window(c, 0) * scale for c in range(NT)]
        logits = []
        for w in range(W):
            p = q[0] * window(NT, w)
            for c in range(1, NT):
                p = p + q[c] * window(NT + c, w)
            p = p + pltpu.roll(p, 64, 1)
            p = p + pltpu.roll(p, 32, 1)
            if head and row < DIL * w:
                p = jnp.where(sub >= DIL * w - row, p, -1e9 * LOG2E)
            logits.append(p)
        top = functools.reduce(jnp.maximum, logits)
        e = [jnp.exp2(p - top) for p in logits]
        inv = pl.reciprocal(functools.reduce(jnp.add, e), full_range=False)
        done = []
        for c in range(NT):
            acc = e[0] * window(2 * NT + c, 0)
            for w in range(1, W):
                acc = acc + e[w] * window(2 * NT + c, w)
            res = acc * inv
            done.append(pltpu.bitcast(res, U32))
            if row % 16 == 0:
                held[c] = res
            else:
                pair = jnp.concatenate([held.pop(c), res], axis=0).astype(BF16)
                o[row // 2 - 4:row // 2 + 4, TILES[c]] = pltpu.bitcast(pair, U32)
                written["o"] = row + RA
        return functools.reduce(jnp.bitwise_or, done)

    def out_rows(o, xn, x, s, out, r0, n):
        def finish(cols, y):
            s[r0:r0 + n, cols] = y
            g = _silu(pltpu.bitcast(xn[r0 // 2:(r0 + n) // 2, cols], BF16).astype(F32))
            out[r0:r0 + n, cols] = (x[r0:r0 + n, cols].astype(F32) + y * g).astype(BF16)

        return [step for cols in TILES for step in _tiles(
            lambda k: after("o", r0 + n, pltpu.bitcast(o[r0 // 2:(r0 + n) // 2, k], BF16)),
            lambda k, cols=cols: pltpu.bitcast(wop_v[k.start // 2:k.stop // 2, cols], BF16),
            NN_DIMS, functools.partial(finish, cols))]

    def tile_of(idx):
        return pl.multiple_of((idx >> 4) << 4, 16)

    def normed_tile(idx):
        return pltpu.bitcast(xn_v[pl.ds(pl.multiple_of((idx >> 4) << 3, 8), 8), :], BF16).astype(F32)

    def route():
        keys, vals = [], []
        for half in range(NB // 4):
            r = r_v[4 * half]
            for b in range(1, 4):
                r = jnp.where(lane >= 32 * b, pltpu.roll(r_v[4 * half + b], 32 * b, 1), r)
            r = _bf16_round(r) + 0.0
            bits = pltpu.bitcast(r, I32)
            rank = jnp.where(bits < 0, bits ^ np.int32(0x7FFFFFFF), bits) >> 16
            rank = jnp.where(r != r, np.int32(-2 ** 15), rank)
            keys.append(rank * S + (S - 1 - half * 1024 - lane * 8 - sub))
            vals.append(r)
        row = lax.broadcasted_iota(I32, (16, D), 0)
        xs = jnp.zeros((8, D), F32)
        sel = []
        for i in range(2):
            best = jnp.max(jnp.maximum(keys[0], keys[1]))
            score = jnp.where(keys[0] == best, vals[0], jnp.where(keys[1] == best, vals[1], 0.0))
            keys = [jnp.where(key == best, np.int32(-2 ** 31), key) for key in keys]
            idx = (S - 1) - (best & (S - 1))
            picked = jnp.sum(jnp.where(row == (idx & 15), normed_tile(idx), 0.0), axis=0, keepdims=True)
            xs = jnp.where(row[:8] == i, picked, xs)
            sel.append((idx, jnp.sum(score, keepdims=True)))
        xs_v[...] = xs
        return sel

    def ffn():
        chunks = [slice(lo, min(lo + 128, F)) for lo in range(0, F, 128)]
        pre, hid, y = {}, {}, [0.0] * NT

        def up(w, j):
            return _tiles(lambda k: xs_v[:, k], lambda k: w[chunks[j], k], NT_DIMS, pre.setdefault(j, []).append)

        def down(j, c):
            if c == 0:
                g, u = pre[j]
                hid[j] = _bf16_round(g * jax.nn.sigmoid(g) * u)
            y[c] = y[c] + lax.dot_general(hid[j], wd_v[chunks[j], TILES[c]], NN_DIMS, preferred_element_type=F32)

        steps = []
        for j in range(len(chunks) + 1):
            if j < len(chunks):
                steps += up(wg_v, j) + up(wu_v, j)
            if j > 0:
                steps += [functools.partial(down, j - 1, c) for c in range(NT)]
        return steps, y

    latest = [None]

    def wait_after(copy, buf, g):
        buf[buf.shape[0] - 8:, TILES[0]] = latest[0][8 * g:8 * g + 8].astype(BF16)
        copy.wait()

    def run(rounds, attn=(), ln=()):
        tasks = []
        for kind, jobs, step in (("attn", attn, RA), ("ln", ln, RL)):
            for k, job in enumerate(jobs):
                lo, hi = job[-1]
                tasks += [(lo + (hi - lo) * r / T, kind, k, r) for r in range(0, T, step)]
        tasks.sort()
        done = {"attn": [], "ln": []}
        pos = 0
        for j in range(-1, len(rounds)):
            for call in rounds[j][2] if j >= 0 else ():
                v = call()
                latest[0] = latest[0] if v is None else v
            y = latest[0] if j >= 0 else None
            while pos < len(tasks):
                frac, kind, k, off = tasks[pos]
                t = int(frac * (rounds[-1][0] + rounds[-1][1])) - MXU_LATENCY if rounds else 0
                if j + 1 < len(rounds) and t >= rounds[j + 1][0]:
                    break
                pos += 1
                lag = IN_FLIGHT[kind]
                bits = done[kind][-lag] if rounds and len(done[kind]) >= lag else None
                if y is not None:
                    g = min(t - rounds[j][0], rounds[j][1] - 8) // 8
                    mine = pltpu.bitcast(y[8 * g:8 * g + 8], U32)
                    bits = mine if bits is None else bits | mine
                gate = None if bits is None else (bits >> 31) >> 1
                if kind == "attn":
                    qkv, o, first, head, _ = attn[k]
                    done[kind].append(attn_rows(qkv, o, first + off, head, gate))
                else:
                    x, xn, first, block, _ = ln[k]
                    if off == 0:
                        scores = jnp.zeros((8, 128), F32)
                    scores = ln_rows(x, xn, first + off, off // 8, scores, gate)
                    done[kind].append(pltpu.bitcast(scores, U32))
                    if off == T - RL:
                        r_v[block] = latest[0] = scores

    for c in (get_wr, get_x[0], *get_w, get_x[1], get_wo, *get_x[2:], *get_ffn):
        c.start()
    get_wr.wait()
    get_x[0].wait()
    wr_v[...] = jnp.broadcast_to(wr1_v[...].astype(F32).reshape(1, D), (RL, D))
    run([], ln=[(x_v, xn_v, 0, 0, (0.0, 0.0))])
    wait_after(get_w[0], wqkv_v, 0)
    prep_qkv(0)
    for k in range(NT):
        rounds = _rounds(proj(xn_v, qkv_v, 0, T, [k]), T)
        if k + 1 < NT:
            rounds[1][2].append(functools.partial(wait_after, get_w[k + 1], wqkv_v, 8))
            rounds[1][2].append(functools.partial(prep_qkv, k + 1))
        else:
            rounds[0][2].append(functools.partial(wait_after, get_x[1], x_v, 0))
        run(rounds)
    run([], ln=[(x_v, xn_v, T, 1, (0.0, 0.0))])

    def prep_wo():
        for c, cols in enumerate(TILES):
            tmp_v[3, c, :D // 2] = pltpu.bitcast(wo_v[:D, cols], U32)
            _regroup(tmp_v.at[3, c], wop_v, cols)

    def blocks(qkv, xn, o, x, s, out, block, head=False):
        assert written == dict(xn=2 * T, qkv=T, o=0)
        steps, attn, ln = [], [], []
        for k in range(U):
            steps += proj(xn, qkv, (k + 1) * T, T) + out_rows(o, xn, x, s, out, k * T, T)
            attn.append((qkv, o, k * T, head, [(k + f) / U for f in ATTN_SPAN]))
            ln.append((x, xn, (k + 2) * T, block + k + 2, [(k + f) / U for f in LN_SPAN]))
        rounds = _rounds(steps, T)
        if head:
            rounds[4][2].extend([functools.partial(wait_after, get_wo, wo_v, 0), prep_wo])
        for k in range(U):
            rounds[k * len(rounds) // U + 8][2].append(functools.partial(wait_after, x_copy(block + k + 2), x_v, 0))
        run(rounds, attn, ln)
        assert written == dict(xn=(U + 2) * T, qkv=(U + 1) * T, o=U * T)
        written.update(xn=2 * T, qkv=T, o=0)

    def trip(i, carry):
        base = pl.multiple_of(i * (U * T), T)
        pairs = pl.multiple_of(i * (U * M), M)
        blocks(qkv_v.at[:, pl.ds(base, HALO + (U + 1) * T), :], xn_v.at[pl.ds(pairs, (U + 2) * M), :],
               o_v.at[pl.ds(pairs, U * M), :], x_v.at[pl.ds(base, (U + 2) * T), :],
               s_v.at[pl.ds(base, U * T), :], out_v.at[pl.ds(base, U * T), :], i * U)
        out_copy(i, pl.ds(base, U * T)).start()
        return carry

    sent = [out_copy(i, pl.ds(i * U * T, U * T)) for i in range(TRIPS + 1)]
    blocks(qkv_v, xn_v, o_v, x_v, s_v, out_v, 0, head=True)
    sent[0].start()
    lax.fori_loop(1, TRIPS + 1, trip, 0)

    for c in get_ffn:
        c.wait()
    sel = route()
    small, routed = ffn()
    last = S - T
    written.update(xn=S, qkv=last, o=last - T)
    steps = [step for r in range(last, S, M) for step in proj(xn_v, qkv_v, r, M)]
    issued = {}
    for r in range(last - T, S, M):
        steps += out_rows(o_v, xn_v, x_v, s_v, out_v, r, M)
        issued[r + M] = len(steps)
    rounds = _rounds(steps, M, lambda j: small[4 * (j - 9):4 * (j - 8)] if j >= 9 else [])
    assert len(small) <= 4 * (len(rounds) - 9)
    stages = [(0, last - T, sent)]
    for i, (lo, hi) in enumerate(((last - T, last), (last, S - M))):
        stages.append((lo, hi, [out_copy(TRIPS + 1 + i, slice(lo, hi))]))
        rounds[issued[hi] // 4 + 2][2].append(stages[-1][2][0].start)
    left, right = [out_copy(TRIPS + 3 + i, slice(S - M, S), cols)
                   for i, cols in enumerate((slice(0, 3 * 128), slice(3 * 128, D)))]
    stages.append((S - M, S, [left, right]))
    rounds[(len(steps) - 2 * NT) // 4 + 1][2].append(left.start)
    run(rounds, [(qkv_v, o_v, last - T, False, (0.05, 0.4)), (qkv_v, o_v, last, False, (0.42, 0.86))])

    y = jnp.concatenate(routed, axis=1)
    y = [y[i:i + 1, :] * jax.nn.sigmoid(score) for i, (_, score) in enumerate(sel)]
    row = lax.broadcasted_iota(I32, (16, D), 0)
    tiles = [tile_of(idx) for idx, _ in sel]
    for i, ((idx, _), tile) in enumerate(zip(sel, tiles)):
        upd = jnp.zeros((16, D), F32)
        for (other, _), y_other in zip(sel, y):
            upd = jnp.where(row == other - tile, y_other, upd)
        rows = pl.ds(tile, 16)
        fix_v[i] = (x_v[rows, :].astype(F32) + s_v[rows, :] * _silu(normed_tile(idx) + upd)).astype(BF16)
    right.start()

    fixes = [pltpu.make_async_copy(fix_v.at[i], out_hbm.at[pl.ds(tile, 16), :], sem_fix.at[i])
             for i, tile in enumerate(tiles)]
    distinct = tiles[1] != tiles[0]
    for lo, hi, copies in stages:
        for c in copies:
            c.wait()
        pl.when((tiles[0] >= lo) & (tiles[0] < hi))(fixes[0].start)
        pl.when((tiles[1] >= lo) & (tiles[1] < hi) & distinct)(fixes[1].start)
    fixes[0].wait()
    pl.when(distinct)(fixes[1].wait)


@jax.jit
def pallas_recurrent_scan__sliding_local_dilated__moe_arch_mod__prompt_kernel(
    A_x: jax.Array,
    A_wqkv: jax.Array,
    A_wo: jax.Array,
    B_x: jax.Array,
    B_w_r: jax.Array,
    B_w_gate: jax.Array,
    B_w_up: jax.Array,
    B_w_down: jax.Array,
):
    del B_x
    hbm = pl.BlockSpec(memory_space=pltpu.HBM)
    out = pl.pallas_call(
        _kernel,
        out_shape=jax.ShapeDtypeStruct((S, D), BF16),
        in_specs=[hbm] * 7,
        out_specs=hbm,
        scratch_shapes=[
            pltpu.VMEM((S + 64, D), BF16),
            pltpu.VMEM((D + 64, 3 * D), BF16),
            pltpu.VMEM((D + 64, D), BF16),
            pltpu.VMEM((F, D), BF16),
            pltpu.VMEM((F, D), BF16),
            pltpu.VMEM((F, D), BF16),
            pltpu.VMEM((4, NT, D // 2 + 32, 128), U32),
            pltpu.VMEM((3, D // 2, D), U32),
            pltpu.VMEM((D // 2, D), U32),
            pltpu.VMEM((S // 2, D), U32),
            pltpu.VMEM((3 * NT + 1, HALO + S, 128), F32),
            pltpu.VMEM((S // 2, D), U32),
            pltpu.VMEM((S, D), F32),
            pltpu.VMEM((S, D), BF16),
            pltpu.VMEM((RL, D), F32),
            pltpu.VMEM((NB, 8, 128), F32),
            pltpu.VMEM((8, D), F32),
            pltpu.VMEM((2, 16, D), BF16),
            pltpu.VMEM((D,), BF16),
        ],
        compiler_params=pltpu.CompilerParams(vmem_limit_bytes=64 * 2 ** 20,
                                             flags={"XLA_TPU_RESCHEDULE_DMA_DONES": True}),
        name="fused",
    )(A_x.reshape(S, D), A_wqkv, A_wo, B_w_r, B_w_gate.T, B_w_up.T, B_w_down)
    return out.reshape(1, S, D)
```
